```python
import jax
import jax.numpy as jnp

def _softmax(x, axis=-1):
    return jax.nn.softmax(x, axis=axis)

def _gelu(x):
    return jax.nn.gelu(x, approximate=True)

def _silu(x):
    return jax.nn.silu(x)

def _sigmoid(x):
    return jax.nn.sigmoid(x)

def _layernorm(x, axis=-1, eps=1e-05):
    m = jnp.mean(x, axis=axis, keepdims=True)
    v = jnp.var(x, axis=axis, keepdims=True)
    return (x - m) / jnp.sqrt(v + eps)

def _scatter_add(tgt, idx, src, axis=0):
    return tgt.at[idx].add(src)

def _segment_sum(src, seg, n):
    return jax.ops.segment_sum(src, seg, n)

class _Rng:

    def __init__(self, key):
        self._k = key

    def _next(self):
        self._k, sub = jax.random.split(self._k)
        return sub

    def normal(self, shape):
        return jax.random.normal(self._next(), shape, dtype=jnp.bfloat16)

    def randint(self, lo, hi, shape):
        return jax.random.randint(self._next(), shape, lo, hi, dtype=jnp.int32)

    def uniform(self, shape, lo=0.0, hi=1.0):
        return jax.random.uniform(self._next(), shape, jnp.bfloat16, lo, hi)

    def permutation(self, n):
        return jax.random.permutation(self._next(), n)
kernel_name = 'interleave_layers__memory_aug_recurrent_mem_tr__glu_gated_swiglu__prompt'

def setup_inputs():
    _rng = _Rng(jax.random.key(int.from_bytes(__import__("os").urandom(4), "little")))
    _w = lambda a: (lambda t: t.astype(jnp.bfloat16) if jnp.issubdtype(t.dtype, jnp.floating) else t)(jnp.asarray(a))

    def _A_setup():
        B, S, Dm = (1, 2048, 576)
        H, Dh = (32, 128)
        M, seg = (8, 32)
        seg = min(seg, S)
        S = S // seg * seg
        return {'x': _w((lambda *s: _rng.normal(s) * 0.05)(B, S, Dm)), 'mem0': _w((lambda *s: _rng.normal(s) * 0.05)(B, M, Dm)), 'Wq': _w((lambda *s: _rng.normal(s) * 0.05)(Dm, H, Dh) * Dm ** (-0.5)), 'Wk': _w((lambda *s: _rng.normal(s) * 0.05)(Dm, H, Dh) * Dm ** (-0.5)), 'Wv': _w((lambda *s: _rng.normal(s) * 0.05)(Dm, H, Dh) * Dm ** (-0.5)), 'Wo': _w((lambda *s: _rng.normal(s) * 0.05)(H, Dh, Dm) * (H * Dh) ** (-0.5)), 'seg_len': seg}
    _A_in = _A_setup()

    def _B_setup():
        B, S, D, F = (1, 2048, 576, 4608)
        return {'x': _w((lambda *s: _rng.normal(s) * 0.05)(B, S, D)), 'w1': _w((lambda *s: _rng.normal(s) * 0.05)(D, F) * (2.0 / D) ** 0.5), 'w3': _w((lambda *s: _rng.normal(s) * 0.05)(D, F) * (2.0 / D) ** 0.5), 'w2': _w((lambda *s: _rng.normal(s) * 0.05)(F, D) * (2.0 / F) ** 0.5)}
    _B_in = _B_setup()
    return {'A_x': _A_in['x'], 'A_mem0': _A_in['mem0'], 'A_Wq': _A_in['Wq'], 'A_Wk': _A_in['Wk'], 'A_Wv': _A_in['Wv'], 'A_Wo': _A_in['Wo'], 'A_seg_len': _A_in['seg_len'], 'B_x': _B_in['x'], 'B_w1': _B_in['w1'], 'B_w3': _B_in['w3'], 'B_w2': _B_in['w2']}

def reference(A_x, A_mem0, A_Wq, A_Wk, A_Wv, A_Wo, A_seg_len, B_x, B_w1, B_w3, B_w2):

    def _A_ref(x, mem0, Wq, Wk, Wv, Wo, seg_len):
        B, S, Dm = x.shape
        H, Dh = (Wq.shape[1], Wq.shape[2])
        M = mem0.shape[1]
        scale = Dh ** (-0.5)
        n_seg = S // seg_len
        L = M + seg_len
        idx = jnp.arange(L)
        mask = (idx[:, None] < M) | (idx[:, None] >= idx[None, :])
        mem = mem0
        outs = []
        for s in range(n_seg):
            xs = x[:, s * seg_len:(s + 1) * seg_len, :].copy()
            h = jnp.concatenate([mem, xs], axis=1)
            q = jnp.einsum('btd,dhe->bhte', h, Wq)
            k = jnp.einsum('btd,dhe->bhte', h, Wk)
            v = jnp.einsum('btd,dhe->bhte', h, Wv)
            scores = jnp.einsum('bhqe,bhke->bhqk', q, k) * scale
            scores = jnp.where(mask[None, None], scores, -1000000000.0)
            p = _softmax(scores, axis=-1)
            o = jnp.einsum('bhqk,bhke->bhqe', p, v)
            o = jnp.einsum('bhte,hed->btd', o, Wo)
            mem = o[:, :M, :].copy()
            outs.append(o[:, M:, :])
        return jnp.concatenate(outs, axis=1)

    def _B_ref(x, w1, w3, w2):
        gate = jnp.einsum('bsd,df->bsf', x, w1)
        up = jnp.einsum('bsd,df->bsf', x, w3)
        h = _silu(gate) * up
        out = jnp.einsum('bsf,fd->bsd', h, w2)
        return out
    x = A_x
    x = x + _A_ref(_layernorm(x, axis=-1), A_mem0, A_Wq, A_Wk, A_Wv, A_Wo, A_seg_len)
    x = x + _B_ref(_layernorm(x, axis=-1), B_w1, B_w3, B_w2)
    x = x + _A_ref(_layernorm(x, axis=-1), A_mem0, A_Wq, A_Wk, A_Wv, A_Wo, A_seg_len)
    x = x + _B_ref(_layernorm(x, axis=-1), B_w1, B_w3, B_w2)
    return x
```

```python
import jax
import jax.numpy as jnp
from jax import lax
import jax.experimental.pallas as pl
import jax.experimental.pallas.tpu as pltpu

SEG = 32
EPS = 1e-5
MASK_FILL = -1000000000.0
F_CHUNK = 512
BF16 = jnp.bfloat16
F32 = jnp.float32
NT_DIMS = (((1,), (1,)), ((), ()))


def _layernorm(x):
    inv_n = 1.0 / x.shape[-1]
    c = x - jnp.sum(x, axis=-1, keepdims=True) * inv_n
    v = jnp.sum(c * c, axis=-1, keepdims=True) * inv_n
    return c * lax.rsqrt(v + EPS)


def _kernel(xt_hbm, mem0_ref, wq_hbm, wk_hbm, wv_hbm, wot_hbm, w1_hbm, w3_hbm, w2t_hbm,
            out_ref,
            xt_v, xs, stage, wqkv, wot, w1, w3, w2t,
            h_a, res_a, y_b, o_scr, g_scr, zs, sems, *, n_heads, d_head, n_mem):
    d_model, seq = xt_v.shape
    n_seg = seq // SEG
    d_ff = w1.shape[1]
    rows = 2 * SEG + 2 * n_mem
    scale = d_head ** -0.5

    cp_x = pltpu.make_async_copy(xt_hbm, xt_v, sems.at[0])
    cp_qkv = [pltpu.make_async_copy(w, stage.at[i], sems.at[1 + i])
              for i, w in enumerate((wq_hbm, wk_hbm, wv_hbm))]
    cp_wo = [pltpu.make_async_copy(wot_hbm.at[h], wot.at[:, pl.ds(h * d_head, d_head)], sems.at[4])
             for h in range(n_heads)]
    cp_ff = [pltpu.make_async_copy(s, d, sems.at[5 + i])
             for i, (s, d) in enumerate(((w1_hbm, w1), (w3_hbm, w3), (w2t_hbm, w2t)))]
    cp_x.start()
    for cp in cp_qkv + cp_wo + cp_ff:
        cp.start()

    cp_x.wait()
    for c in range(seq // 128):
        xs[c * 128:(c + 1) * 128, :] = xt_v[:, c * 128:(c + 1) * 128].astype(F32).T

    pairs = n_heads // 2
    for i in range(3):
        cp_qkv[i].wait()
        words = stage.at[i].bitcast(jnp.uint32)
        for j in range(pairs):
            w = words[pl.ds(j, d_model, stride=pairs), :]
            lo = pltpu.bitcast(w << 16, F32).astype(BF16)
            hi = pltpu.bitcast(w & jnp.uint32(0xFFFF0000), F32).astype(BF16)
            c0 = (2 * j * 3 + i) * d_head
            c1 = ((2 * j + 1) * 3 + i) * d_head
            wqkv[:, c0:c0 + d_head] = lo
            wqkv[:, c1:c1 + d_head] = hi

    mem0 = mem0_ref[...].astype(F32)
    x0 = xs[0:SEG, :]
    res_a[0:SEG, :] = x0
    res_a[SEG:2 * SEG, :] = jnp.zeros((SEG, d_model), F32)
    h_a[0:SEG, :] = _layernorm(x0).astype(BF16)
    h_a[SEG:2 * SEG, :] = jnp.zeros((SEG, d_model), BF16)
    h_a[2 * SEG:rows, :] = jnp.concatenate([mem0, mem0], axis=0).astype(BF16)
    y_b[...] = jnp.zeros(y_b.shape, F32)

    for cp in cp_wo + cp_ff:
        cp.wait()

    def step(t, carry):
        r = lax.broadcasted_iota(jnp.int32, (rows, rows), 0)
        c = lax.broadcasted_iota(jnp.int32, (rows, rows), 1)
        r_mem, c_mem = r >= 2 * SEG, c >= 2 * SEG
        r_layer = jnp.where(r_mem, (r - 2 * SEG) // n_mem, r // SEG)
        c_layer = jnp.where(c_mem, (c - 2 * SEG) // n_mem, c // SEG)
        same = r_layer == c_layer
        visible = same & (r_mem | c_mem | (c <= r))
        fill = jnp.where(same, MASK_FILL, -jnp.inf).astype(F32)

        y_prev = y_b[...]
        h_b = _layernorm(y_prev).astype(BF16)

        ha = h_a[...]
        for h in range(n_heads):
            qkv = jnp.dot(ha, wqkv[:, 3 * h * d_head:3 * (h + 1) * d_head],
                          preferred_element_type=F32).astype(BF16)
            q, k, v = (qkv[:, i * d_head:(i + 1) * d_head] for i in range(3))
            s = lax.dot_general(q, k, NT_DIMS, preferred_element_type=F32) * scale
            s = jnp.where(visible, s, fill)
            e = jnp.exp(s - jnp.max(s, axis=-1, keepdims=True))
            inv = 1.0 / jnp.sum(e, axis=-1, keepdims=True)
            o = jnp.dot(e.astype(BF16), v, preferred_element_type=F32) * inv
            o_scr[:, h * d_head:(h + 1) * d_head] = o.astype(BF16)

        for f in range(d_ff // F_CHUNK):
            cols = slice(f * F_CHUNK, (f + 1) * F_CHUNK)
            gate = jnp.dot(h_b, w1[:, cols], preferred_element_type=F32)
            up = jnp.dot(h_b, w3[:, cols], preferred_element_type=F32)
            g_scr[:, cols] = (gate * jax.nn.sigmoid(gate) * up).astype(BF16)

        z = y_prev + lax.dot_general(g_scr[...], w2t[...], NT_DIMS, preferred_element_type=F32)
        att = lax.dot_general(o_scr[...], wot[...], NT_DIMS, preferred_element_type=F32)

        y_b[...] = res_a[...] + att[0:2 * SEG]
        mem2 = jnp.where(t >= 2, att[2 * SEG + n_mem:rows], mem0)
        h_a[2 * SEG:rows, :] = jnp.concatenate(
            [att[2 * SEG:2 * SEG + n_mem], mem2], axis=0).astype(BF16)

        nxt = pl.multiple_of(jnp.minimum(t + 1, n_seg - 1) * SEG, SEG)
        x_next = xs[pl.ds(nxt, SEG), :]
        res_a[0:SEG, :] = x_next
        h_a[0:SEG, :] = _layernorm(x_next).astype(BF16)
        res_a[SEG:2 * SEG, :] = z[0:SEG]
        h_a[SEG:2 * SEG, :] = _layernorm(z[0:SEG]).astype(BF16)
        done = pl.multiple_of(jnp.maximum(t - 3, 0) * SEG, SEG)
        zs[pl.ds(done, SEG), :] = z[SEG:2 * SEG]
        return carry

    lax.fori_loop(0, n_seg + 3, step, 0)

    for c in range(seq // 128):
        out_ref[:, c * 128:(c + 1) * 128] = zs[c * 128:(c + 1) * 128, :].T.astype(out_ref.dtype)


@jax.jit
def pallas_interleave_layers__memory_aug_recurrent_mem_tr__glu_gated_swiglu__prompt_kernel(
    A_x, A_mem0, A_Wq, A_Wk, A_Wv, A_Wo, A_seg_len, B_x, B_w1, B_w3, B_w2,
):
    del A_seg_len, B_x
    batch, seq, d_model = A_x.shape
    _, n_heads, d_head = A_Wq.shape
    n_mem = A_mem0.shape[1]
    d_ff = B_w1.shape[1]
    assert batch == 1 and seq % 128 == 0 and d_ff % F_CHUNK == 0
    rows = 2 * SEG + 2 * n_mem

    def kernel(*refs):
        _kernel(*refs, n_heads=n_heads, d_head=d_head, n_mem=n_mem)

    hbm = pl.BlockSpec(memory_space=pl.ANY)
    vmem = pl.BlockSpec(memory_space=pltpu.VMEM)
    out_t = pl.pallas_call(
        kernel,
        out_shape=jax.ShapeDtypeStruct((d_model, seq), A_x.dtype),
        in_specs=[hbm, vmem, hbm, hbm, hbm, hbm, hbm, hbm, hbm],
        out_specs=vmem,
        scratch_shapes=[
            pltpu.VMEM((d_model, seq), BF16),
            pltpu.VMEM((seq, d_model), F32),
            pltpu.VMEM((3, d_model * n_heads, d_head), BF16),
            pltpu.VMEM((d_model, 3 * n_heads * d_head), BF16),
            pltpu.VMEM((d_model, n_heads * d_head), BF16),
            pltpu.VMEM((d_model, d_ff), BF16),
            pltpu.VMEM((d_model, d_ff), BF16),
            pltpu.VMEM((d_model, d_ff), BF16),
            pltpu.VMEM((rows, d_model), BF16),
            pltpu.VMEM((2 * SEG, d_model), F32),
            pltpu.VMEM((2 * SEG, d_model), F32),
            pltpu.VMEM((rows, n_heads * d_head), BF16),
            pltpu.VMEM((2 * SEG, d_ff), BF16),
            pltpu.VMEM((seq, d_model), F32),
            pltpu.SemaphoreType.DMA((8,)),
        ],
        compiler_params=pltpu.CompilerParams(vmem_limit_bytes=110 * 1024 * 1024),
    )(
        A_x[0].T,
        A_mem0[0],
        A_Wq.reshape(d_model * n_heads, d_head),
        A_Wk.reshape(d_model * n_heads, d_head),
        A_Wv.reshape(d_model * n_heads, d_head),
        jnp.transpose(A_Wo, (0, 2, 1)),
        B_w1,
        B_w3,
        B_w2.T,
    )
    return out_t.T[None]
```

```python
import functools

import jax
import jax.numpy as jnp
from jax import lax
import jax.experimental.pallas as pl
import jax.experimental.pallas.tpu as pltpu

SEG = 32
EPS = 1e-5
MASK_FILL = -1000000000.0
F_CHUNK = 512
LANES = 128
LAG = 4
STAGE_LAG = 3
BF16 = jnp.bfloat16
F32 = jnp.float32
NT_DIMS = (((1,), (1,)), ((), ()))


def _layernorm(x):
    inv_n = 1.0 / x.shape[-1]
    c = x - jnp.sum(x, axis=-1, keepdims=True) * inv_n
    v = jnp.sum(c * c, axis=-1, keepdims=True) * inv_n
    return c * lax.rsqrt(v + EPS)


def _attention_mask(n_x, n_mem):
    rows = n_x + 2 * n_mem
    r = lax.broadcasted_iota(jnp.int32, (rows, rows), 0)
    c = lax.broadcasted_iota(jnp.int32, (rows, rows), 1)
    r_mem, c_mem = r >= n_x, c >= n_x
    r_stream = jnp.where(r_mem, (r - n_x) // n_mem, r // SEG)
    c_stream = jnp.where(c_mem, (c - n_x) // n_mem, c // SEG)
    same = r_stream == c_stream
    visible = same & (r_mem | c_mem | (c <= r))
    fill = jnp.where(same, MASK_FILL, -jnp.inf).astype(F32)
    return visible, fill


def _kernel(xt_hbm, mem0_ref, wq_hbm, wk_hbm, wv_hbm, wot_hbm, w1_hbm, w3_hbm, w2t_hbm,
            out_hbm,
            xt_v, stage, wqkv, wot, w1, w3, w2t,
            acts, ys, h_a, qkv_scr, p_scr, o_scr, g_scr, out_v, sems, out_sems,
            *, n_heads, d_head, n_mem):
    d_model, seq = xt_v.shape
    n_seg = seq // SEG
    n_chunks = seq // LANES
    segs_per_chunk = LANES // SEG
    n_f = w1.shape[1] // F_CHUNK
    scale = d_head ** -0.5

    def seg_rows(base, s):
        return pl.ds(pl.multiple_of(base + s * SEG, SEG), SEG)

    def mixer_stages(h, n_x):
        rows = n_x + 2 * n_mem
        visible, fill = _attention_mask(n_x, n_mem)

        def project(i):
            cols = slice(3 * i * d_head, 3 * (i + 1) * d_head)
            qkv_scr[0:rows, cols] = jnp.dot(h, wqkv[:, cols], preferred_element_type=F32).astype(BF16)

        def scores(i):
            q = qkv_scr[0:rows, 3 * i * d_head:(3 * i + 1) * d_head]
            k = qkv_scr[0:rows, (3 * i + 1) * d_head:(3 * i + 2) * d_head]
            s = lax.dot_general(q, k, NT_DIMS, preferred_element_type=F32) * scale
            s = jnp.where(visible, s, fill)
            e = jnp.exp(s - jnp.max(s, axis=-1, keepdims=True))
            p = e * (1.0 / jnp.sum(e, axis=-1, keepdims=True))
            p_scr[i, 0:rows, 0:rows] = p.astype(BF16)

        def mix(i):
            v = qkv_scr[0:rows, (3 * i + 2) * d_head:(3 * i + 3) * d_head]
            o = jnp.dot(p_scr[i, 0:rows, 0:rows], v, preferred_element_type=F32)
            o_scr[0:rows, i * d_head:(i + 1) * d_head] = o.astype(BF16)

        def output():
            return lax.dot_general(o_scr[0:rows, :], wot[...], NT_DIMS, preferred_element_type=F32)

        return project, scores, mix, output

    def ffn_stages(rows0, rows1):
        y = jnp.concatenate([ys[rows0, :], ys[rows1, :]], axis=0)
        h = _layernorm(y).astype(BF16)

        def hidden(f):
            cols = slice(f * F_CHUNK, (f + 1) * F_CHUNK)
            gate = jnp.dot(h, w1[:, cols], preferred_element_type=F32)
            up = jnp.dot(h, w3[:, cols], preferred_element_type=F32)
            g_scr[:, cols] = (gate * jax.nn.sigmoid(gate) * up).astype(BF16)

        def output():
            return y + lax.dot_general(g_scr[...], w2t[...], NT_DIMS, preferred_element_type=F32)

        return hidden, output

    def emit(matmul_work, scores, mix):
        for i in range(max(len(matmul_work), n_heads + 2 * STAGE_LAG)):
            if i < len(matmul_work):
                matmul_work[i]()
            if 0 <= i - STAGE_LAG < n_heads:
                scores(i - STAGE_LAG)
            if 0 <= i - 2 * STAGE_LAG < n_heads:
                mix(i - 2 * STAGE_LAG)

    def mixer_only(layer, s, mem):
        x = acts[seg_rows(layer * seq, s), :]
        tail = jnp.concatenate([mem, jnp.zeros_like(mem)], axis=0)
        h = jnp.concatenate([_layernorm(x).astype(BF16), tail.astype(BF16)], axis=0)
        project, scores, mix, output = mixer_stages(h, SEG)
        emit([functools.partial(project, i) for i in range(n_heads)], scores, mix)
        att = output()
        ys[seg_rows(layer * seq, s), :] = x + att[0:SEG]
        return att[SEG:SEG + n_mem]

    def ffn_only(off0, off1):
        hidden, output = ffn_stages(seg_rows(off0, 0), seg_rows(off1, 0))
        for f in range(n_f):
            hidden(f)
        z = output()
        acts[seg_rows(seq + off0, 0), :] = z[0:SEG]
        acts[seg_rows(seq + off1, 0), :] = z[SEG:2 * SEG]

    def stage_tokens(t):
        h_a[0:SEG, :] = _layernorm(acts[seg_rows(0, t), :]).astype(BF16)
        h_a[SEG:2 * SEG, :] = _layernorm(acts[seg_rows(seq, t - LAG), :]).astype(BF16)

    def transpose_out(c):
        rows = pl.ds(pl.multiple_of(2 * seq + c * LANES, LANES), LANES)
        out_v[c] = acts[rows, :].T.astype(out_v.dtype)

    def out_copy(c):
        return pltpu.make_async_copy(out_v.at[c], out_hbm.at[:, pl.ds(c * LANES, LANES)], out_sems.at[c])

    cp_x = pltpu.make_async_copy(xt_hbm, xt_v, sems.at[0])
    cp_qkv = [pltpu.make_async_copy(w, stage.at[i], sems.at[1 + i])
              for i, w in enumerate((wq_hbm, wk_hbm, wv_hbm))]
    cp_wo = [pltpu.make_async_copy(wot_hbm.at[i], wot.at[:, pl.ds(i * d_head, d_head)], sems.at[4])
             for i in range(n_heads)]
    cp_ff = [pltpu.make_async_copy(s, d, sems.at[5 + i])
             for i, (s, d) in enumerate(((w1_hbm, w1), (w3_hbm, w3), (w2t_hbm, w2t)))]

    cp_x.start()
    cp_qkv[0].start()
    cp_x.wait()
    cp_qkv[1].start()
    for c in range(n_chunks):
        acts[c * LANES:(c + 1) * LANES, :] = xt_v[:, c * LANES:(c + 1) * LANES].astype(F32).T
    acts[2 * seq:2 * seq + LANES, :] = jnp.zeros((LANES, d_model), F32)

    pairs = n_heads // 2
    for i in range(3):
        cp_qkv[i].wait()
        if i == 0:
            cp_qkv[2].start()
        elif i == 1:
            for cp in cp_wo:
                cp.start()
        words = stage.at[i].bitcast(jnp.uint32)
        for j in range(pairs):
            w = words[pl.ds(j, d_model, stride=pairs), :]
            c0 = (2 * j * 3 + i) * d_head
            c1 = ((2 * j + 1) * 3 + i) * d_head
            wqkv[:, c0:c0 + d_head] = pltpu.bitcast(w << 16, F32).astype(BF16)
            wqkv[:, c1:c1 + d_head] = pltpu.bitcast(w & jnp.uint32(0xFFFF0000), F32).astype(BF16)
    for cp in cp_ff:
        cp.start()
    for cp in cp_wo:
        cp.wait()

    mem0 = mem0_ref[...].astype(F32)
    mem1 = lax.fori_loop(0, LAG, functools.partial(mixer_only, 0), mem0)
    for cp in cp_ff:
        cp.wait()
    ffn_only(0, SEG)
    stage_tokens(LAG)
    h_a[2 * SEG:, :] = jnp.concatenate([mem1, mem0], axis=0).astype(BF16)

    def step(t, carry):
        off0 = (t - 1) * SEG
        off1 = jnp.where(t == LAG, (LAG - 2) * SEG, seq + (t - LAG - 1) * SEG)
        hidden, ffn_output = ffn_stages(seg_rows(off0, 0), seg_rows(off1, 0))
        project, scores, mix, mixer_output = mixer_stages(h_a[...], 2 * SEG)
        emit([functools.partial(project, i) for i in range(n_heads)]
             + [functools.partial(hidden, f) for f in range(n_f)], scores, mix)
        transpose_out(jnp.maximum(t - LAG - 1 - segs_per_chunk, 0) // segs_per_chunk)
        stage_tokens(jnp.minimum(t + 1, n_seg - 1))
        z = ffn_output()
        att = mixer_output()
        acts[seg_rows(seq + off0, 0), :] = z[0:SEG]
        acts[seg_rows(seq + off1, 0), :] = z[SEG:2 * SEG]
        h_a[2 * SEG:, :] = att[2 * SEG:].astype(BF16)
        ys[seg_rows(0, t), :] = acts[seg_rows(0, t), :] + att[0:SEG]
        ys[seg_rows(seq, t - LAG), :] = acts[seg_rows(seq, t - LAG), :] + att[SEG:2 * SEG]
        return carry

    lax.fori_loop(LAG, n_seg, step, 0)

    done = (n_seg - 1 - LAG - 1 - segs_per_chunk) // segs_per_chunk + 1
    for c in range(done):
        out_copy(c).start()
    ffn_only((n_seg - 1) * SEG, seq + (n_seg - LAG - 1) * SEG)
    mem2 = h_a[2 * SEG:, :].astype(F32)[n_mem:]
    lax.fori_loop(n_seg - LAG, n_seg, functools.partial(mixer_only, 1), mem2)

    def ffn_tail(j, carry):
        off = seq + (n_seg - LAG + 2 * j) * SEG
        ffn_only(off, off + SEG)
        return carry

    lax.fori_loop(0, LAG // 2, ffn_tail, 0)
    for c in range(done, n_chunks):
        transpose_out(c)
        out_copy(c).start()
    for c in range(n_chunks):
        out_copy(c).wait()


@jax.jit
def pallas_interleave_layers__memory_aug_recurrent_mem_tr__glu_gated_swiglu__prompt_kernel(
    A_x, A_mem0, A_Wq, A_Wk, A_Wv, A_Wo, A_seg_len, B_x, B_w1, B_w3, B_w2,
):
    del A_seg_len, B_x
    batch, seq, d_model = A_x.shape
    _, n_heads, d_head = A_Wq.shape
    n_mem = A_mem0.shape[1]
    d_ff = B_w1.shape[1]
    assert batch == 1 and seq % 128 == 0 and d_ff % F_CHUNK == 0
    rows = 2 * SEG + 2 * n_mem

    def kernel(*refs):
        _kernel(*refs, n_heads=n_heads, d_head=d_head, n_mem=n_mem)

    hbm = pl.BlockSpec(memory_space=pl.ANY)
    vmem = pl.BlockSpec(memory_space=pltpu.VMEM)
    out_t = pl.pallas_call(
        kernel,
        out_shape=jax.ShapeDtypeStruct((d_model, seq), A_x.dtype),
        in_specs=[hbm, vmem, hbm, hbm, hbm, hbm, hbm, hbm, hbm],
        out_specs=hbm,
        scratch_shapes=[
            pltpu.VMEM((d_model, seq), BF16),
            pltpu.VMEM((3, d_model * n_heads, d_head), BF16),
            pltpu.VMEM((d_model, 3 * n_heads * d_head), BF16),
            pltpu.VMEM((d_model, n_heads * d_head), BF16),
            pltpu.VMEM((d_model, d_ff), BF16),
            pltpu.VMEM((d_model, d_ff), BF16),
            pltpu.VMEM((d_model, d_ff), BF16),
            pltpu.VMEM((3 * seq, d_model), F32),
            pltpu.VMEM((2 * seq, d_model), F32),
            pltpu.VMEM((rows, d_model), BF16),
            pltpu.VMEM((rows, 3 * n_heads * d_head), BF16),
            pltpu.VMEM((n_heads, rows, rows), BF16),
            pltpu.VMEM((rows, n_heads * d_head), BF16),
            pltpu.VMEM((2 * SEG, d_ff), BF16),
            pltpu.VMEM((seq // LANES, d_model, LANES), A_x.dtype),
            pltpu.SemaphoreType.DMA((8,)),
            pltpu.SemaphoreType.DMA((seq // LANES,)),
        ],
        compiler_params=pltpu.CompilerParams(vmem_limit_bytes=110 * 1024 * 1024),
    )(
        A_x[0].T,
        A_mem0[0],
        A_Wq.reshape(d_model * n_heads, d_head),
        A_Wk.reshape(d_model * n_heads, d_head),
        A_Wv.reshape(d_model * n_heads, d_head),
        jnp.transpose(A_Wo, (0, 2, 1)),
        B_w1,
        B_w3,
        B_w2.T,
    )
    return out_t.T[None]
```

```python
import functools

import jax
import jax.numpy as jnp
from jax import lax
import jax.experimental.pallas as pl
import jax.experimental.pallas.tpu as pltpu

SEG = 32
EPS = 1e-5
MASK_FILL = -1000000000.0
F_CHUNK = 512
LANES = 128
LAG = 4
STAGE_LAG = 5
BF16 = jnp.bfloat16
F32 = jnp.float32
NT_DIMS = (((1,), (1,)), ((), ()))


def _layernorm(x):
    inv_n = 1.0 / x.shape[-1]
    c = x - jnp.sum(x, axis=-1, keepdims=True) * inv_n
    v = jnp.sum(c * c, axis=-1, keepdims=True) * inv_n
    return c * lax.rsqrt(v + EPS)


def _attention_mask(n_x, n_mem):
    rows = n_x + 2 * n_mem
    r = lax.broadcasted_iota(jnp.int32, (rows, rows), 0)
    c = lax.broadcasted_iota(jnp.int32, (rows, rows), 1)
    r_mem, c_mem = r >= n_x, c >= n_x
    r_stream = jnp.where(r_mem, (r - n_x) // n_mem, r // SEG)
    c_stream = jnp.where(c_mem, (c - n_x) // n_mem, c // SEG)
    same = r_stream == c_stream
    visible = same & (r_mem | c_mem | (c <= r))
    fill = jnp.where(same, MASK_FILL, -jnp.inf).astype(F32)
    return visible, fill


def _kernel(xt_hbm, mem0_ref, wq_hbm, wk_hbm, wv_hbm, wot_hbm, w1_hbm, w3_hbm, w2t_hbm,
            out_hbm,
            xt_v, stage, wqkv, wot, w1, w3, w2t,
            acts, ys, h_a, qkv_scr, p_scr, o_scr, g_scr, out_v, sems, out_sems,
            *, n_heads, d_head, n_mem):
    d_model, seq = xt_v.shape
    n_seg = seq // SEG
    n_chunks = seq // LANES
    segs_per_chunk = LANES // SEG
    n_f = w1.shape[1] // F_CHUNK
    scale = d_head ** -0.5

    def seg_rows(base, s):
        return pl.ds(pl.multiple_of(base + s * SEG, SEG), SEG)

    def mixer_stages(h, n_x):
        rows = n_x + 2 * n_mem
        visible, fill = _attention_mask(n_x, n_mem)

        def project(i):
            cols = slice(3 * i * d_head, 3 * (i + 1) * d_head)
            qkv_scr[0:rows, cols] = jnp.dot(h, wqkv[:, cols], preferred_element_type=F32).astype(BF16)

        def scores(i):
            q = qkv_scr[0:rows, 3 * i * d_head:(3 * i + 1) * d_head]
            k = qkv_scr[0:rows, (3 * i + 1) * d_head:(3 * i + 2) * d_head]
            s = lax.dot_general(q, k, NT_DIMS, preferred_element_type=F32) * scale
            s = jnp.where(visible, s, fill)
            e = jnp.exp(s - jnp.max(s, axis=-1, keepdims=True))
            p = e * (1.0 / jnp.sum(e, axis=-1, keepdims=True))
            p_scr[i, 0:rows, 0:rows] = p.astype(BF16)

        def mix(i):
            v = qkv_scr[0:rows, (3 * i + 2) * d_head:(3 * i + 3) * d_head]
            o = jnp.dot(p_scr[i, 0:rows, 0:rows], v, preferred_element_type=F32)
            o_scr[0:rows, i * d_head:(i + 1) * d_head] = o.astype(BF16)

        def output():
            return lax.dot_general(o_scr[0:rows, :], wot[...], NT_DIMS, preferred_element_type=F32)

        return project, scores, mix, output

    def ffn_stages(rows0, rows1):
        y = jnp.concatenate([ys[rows0, :], ys[rows1, :]], axis=0)
        h = _layernorm(y).astype(BF16)

        def hidden(f):
            cols = slice(f * F_CHUNK, (f + 1) * F_CHUNK)
            gate = jnp.dot(h, w1[:, cols], preferred_element_type=F32)
            up = jnp.dot(h, w3[:, cols], preferred_element_type=F32)
            g_scr[:, cols] = (gate * jax.nn.sigmoid(gate) * up).astype(BF16)

        def output():
            return y + lax.dot_general(g_scr[...], w2t[...], NT_DIMS, preferred_element_type=F32)

        return hidden, output

    def emit(matmul_work, scores, mix):
        for i in range(max(len(matmul_work), n_heads + 2 * STAGE_LAG)):
            if i < len(matmul_work):
                matmul_work[i]()
            if 0 <= i - STAGE_LAG < n_heads:
                scores(i - STAGE_LAG)
            if 0 <= i - 2 * STAGE_LAG < n_heads:
                mix(i - 2 * STAGE_LAG)

    def mixer_only(layer, s, mem):
        x = acts[seg_rows(layer * seq, s), :]
        tail = jnp.concatenate([mem, jnp.zeros_like(mem)], axis=0)
        h = jnp.concatenate([_layernorm(x).astype(BF16), tail.astype(BF16)], axis=0)
        project, scores, mix, output = mixer_stages(h, SEG)
        emit([functools.partial(project, i) for i in range(n_heads)], scores, mix)
        att = output()
        ys[seg_rows(layer * seq, s), :] = x + att[0:SEG]
        return att[SEG:SEG + n_mem]

    def ffn_only(off0, off1):
        hidden, output = ffn_stages(seg_rows(off0, 0), seg_rows(off1, 0))
        for f in range(n_f):
            hidden(f)
        z = output()
        acts[seg_rows(seq + off0, 0), :] = z[0:SEG]
        acts[seg_rows(seq + off1, 0), :] = z[SEG:2 * SEG]

    def stage_tokens(t):
        h_a[0:SEG, :] = _layernorm(acts[seg_rows(0, t), :]).astype(BF16)
        h_a[SEG:2 * SEG, :] = _layernorm(acts[seg_rows(seq, t - LAG), :]).astype(BF16)

    def transpose_out(c):
        rows = pl.ds(pl.multiple_of(2 * seq + c * LANES, LANES), LANES)
        out_v[c] = acts[rows, :].T.astype(out_v.dtype)

    def out_copy(c):
        return pltpu.make_async_copy(out_v.at[c], out_hbm.at[:, pl.ds(c * LANES, LANES)], out_sems.at[c])

    cp_x0 = pltpu.make_async_copy(xt_hbm.at[:, 0:LANES], xt_v.at[:, 0:LANES], sems.at[8])
    cp_x = pltpu.make_async_copy(xt_hbm.at[:, LANES:], xt_v.at[:, LANES:], sems.at[0])
    cp_qkv = [pltpu.make_async_copy(w, stage.at[i], sems.at[1 + i])
              for i, w in enumerate((wq_hbm, wk_hbm, wv_hbm))]
    cp_wo = [pltpu.make_async_copy(wot_hbm.at[i], wot.at[:, pl.ds(i * d_head, d_head)], sems.at[4])
             for i in range(n_heads)]
    cp_ff = [pltpu.make_async_copy(s, d, sems.at[5 + i])
             for i, (s, d) in enumerate(((w1_hbm, w1), (w3_hbm, w3), (w2t_hbm, w2t)))]

    def transpose_in(c):
        acts[c * LANES:(c + 1) * LANES, :] = xt_v[:, c * LANES:(c + 1) * LANES].astype(F32).T

    cp_x0.start()
    cp_qkv[0].start()
    cp_qkv[1].start()
    cp_x0.wait()
    transpose_in(0)
    acts[2 * seq:2 * seq + LANES, :] = jnp.zeros((LANES, d_model), F32)

    pairs = n_heads // 2
    for i in range(3):
        cp_qkv[i].wait()
        if i == 0:
            cp_qkv[2].start()
        elif i == 1:
            for cp in cp_wo:
                cp.start()
        words = stage.at[i].bitcast(jnp.uint32)
        for j in range(pairs):
            w = words[pl.ds(j, d_model, stride=pairs), :]
            c0 = (2 * j * 3 + i) * d_head
            c1 = ((2 * j + 1) * 3 + i) * d_head
            wqkv[:, c0:c0 + d_head] = pltpu.bitcast(w << 16, F32).astype(BF16)
            wqkv[:, c1:c1 + d_head] = pltpu.bitcast(w & jnp.uint32(0xFFFF0000), F32).astype(BF16)
    for cp in cp_ff:
        cp.start()
    cp_x.start()
    for cp in cp_wo:
        cp.wait()

    def step(t, carry):
        off0 = (t - 1) * SEG
        off1 = jnp.where(t == LAG, (LAG - 2) * SEG, seq + (t - LAG - 1) * SEG)
        hidden, ffn_output = ffn_stages(seg_rows(off0, 0), seg_rows(off1, 0))
        project, scores, mix, mixer_output = mixer_stages(h_a[...], 2 * SEG)
        emit([functools.partial(project, i) for i in range(n_heads)]
             + [functools.partial(hidden, f) for f in range(n_f)], scores, mix)
        transpose_out(jnp.maximum(t - LAG - 1 - segs_per_chunk, 0) // segs_per_chunk)
        stage_tokens(jnp.minimum(t + 1, n_seg - 1))
        z = ffn_output()
        att = mixer_output()
        acts[seg_rows(seq + off0, 0), :] = z[0:SEG]
        acts[seg_rows(seq + off1, 0), :] = z[SEG:2 * SEG]
        h_a[2 * SEG:, :] = att[2 * SEG:].astype(BF16)
        ys[seg_rows(0, t), :] = acts[seg_rows(0, t), :] + att[0:SEG]
        ys[seg_rows(seq, t - LAG), :] = acts[seg_rows(seq, t - LAG), :] + att[SEG:2 * SEG]
        return carry

    done = (n_seg - 1 - LAG - 1 - segs_per_chunk) // segs_per_chunk + 1
    mem0 = mem0_ref[...].astype(F32)
    h_a[2 * SEG:, :] = jnp.concatenate([mem0, mem0], axis=0).astype(BF16)

    def schedule_round(r, carry):
        layer = r // 2
        first = layer * (n_seg - LAG)
        count = jnp.where(r % 2 == 0, LAG, 0)
        mems = h_a[2 * SEG:, :].astype(F32)
        mem = jnp.where(layer == 0, mems[:n_mem], mems[n_mem:])
        mem = lax.fori_loop(first, first + count, functools.partial(mixer_only, layer), mem)

        @pl.when(r == 0)
        def _():
            for cp in cp_ff:
                cp.wait()
            cp_x.wait()
            for c in range(1, n_chunks):
                transpose_in(c)

        @pl.when(r == 1)
        def _():
            for c in range(done):
                out_copy(c).start()

        tail = seq + (n_seg - LAG + 2 * (r - 2)) * SEG
        off0 = jnp.where(r == 0, 0, jnp.where(r == 1, (n_seg - 1) * SEG, tail))
        off1 = jnp.where(r == 1, seq + (n_seg - LAG - 1) * SEG, off0 + SEG)
        ffn_only(off0, off1)

        @pl.when(r == 0)
        def _():
            stage_tokens(LAG)
            h_a[2 * SEG:, :] = jnp.concatenate([mem, mem0], axis=0).astype(BF16)
            lax.fori_loop(LAG, n_seg, step, 0)

        return carry

    lax.fori_loop(0, 2 + LAG // 2, schedule_round, 0)
    for c in range(done, n_chunks):
        transpose_out(c)
        out_copy(c).start()
    for c in range(n_chunks):
        out_copy(c).wait()


@jax.jit
def pallas_interleave_layers__memory_aug_recurrent_mem_tr__glu_gated_swiglu__prompt_kernel(
    A_x, A_mem0, A_Wq, A_Wk, A_Wv, A_Wo, A_seg_len, B_x, B_w1, B_w3, B_w2,
):
    del A_seg_len, B_x
    batch, seq, d_model = A_x.shape
    _, n_heads, d_head = A_Wq.shape
    n_mem = A_mem0.shape[1]
    d_ff = B_w1.shape[1]
    assert batch == 1 and seq % 128 == 0 and d_ff % F_CHUNK == 0
    rows = 2 * SEG + 2 * n_mem

    def kernel(*refs):
        _kernel(*refs, n_heads=n_heads, d_head=d_head, n_mem=n_mem)

    hbm = pl.BlockSpec(memory_space=pl.ANY)
    vmem = pl.BlockSpec(memory_space=pltpu.VMEM)
    out_t = pl.pallas_call(
        kernel,
        out_shape=jax.ShapeDtypeStruct((d_model, seq), A_x.dtype),
        in_specs=[hbm, vmem, hbm, hbm, hbm, hbm, hbm, hbm, hbm],
        out_specs=hbm,
        scratch_shapes=[
            pltpu.VMEM((d_model, seq), BF16),
            pltpu.VMEM((3, d_model * n_heads, d_head), BF16),
            pltpu.VMEM((d_model, 3 * n_heads * d_head), BF16),
            pltpu.VMEM((d_model, n_heads * d_head), BF16),
            pltpu.VMEM((d_model, d_ff), BF16),
            pltpu.VMEM((d_model, d_ff), BF16),
            pltpu.VMEM((d_model, d_ff), BF16),
            pltpu.VMEM((3 * seq, d_model), F32),
            pltpu.VMEM((2 * seq, d_model), F32),
            pltpu.VMEM((rows, d_model), BF16),
            pltpu.VMEM((rows, 3 * n_heads * d_head), BF16),
            pltpu.VMEM((n_heads, rows, rows), BF16),
            pltpu.VMEM((rows, n_heads * d_head), BF16),
            pltpu.VMEM((2 * SEG, d_ff), BF16),
            pltpu.VMEM((seq // LANES, d_model, LANES), A_x.dtype),
            pltpu.SemaphoreType.DMA((9,)),
            pltpu.SemaphoreType.DMA((seq // LANES,)),
        ],
        compiler_params=pltpu.CompilerParams(vmem_limit_bytes=110 * 1024 * 1024),
    )(
        A_x[0].T,
        A_mem0[0],
        A_Wq.reshape(d_model * n_heads, d_head),
        A_Wk.reshape(d_model * n_heads, d_head),
        A_Wv.reshape(d_model * n_heads, d_head),
        jnp.transpose(A_Wo, (0, 2, 1)),
        B_w1,
        B_w3,
        B_w2.T,
    )
    return out_t.T[None]
```

```python
import functools

import jax
import jax.numpy as jnp
from jax import lax
import jax.experimental.pallas as pl
import jax.experimental.pallas.tpu as pltpu

SEG = 32
EPS = 1e-5
MASK_FILL = -1000000000.0
F_CHUNK = 128
LANES = 128
LAG = 4
K_BLOCK = 256
PLAIN_CHUNK = 256
SUM_ROWS = 32
STAGE_LAG = 5
BF16 = jnp.bfloat16
F32 = jnp.float32
NT_DIMS = (((1,), (1,)), ((), ()))


def _layernorm(x):
    inv_n = 1.0 / x.shape[-1]
    c = x - jnp.sum(x, axis=-1, keepdims=True) * inv_n
    v = jnp.sum(c * c, axis=-1, keepdims=True) * inv_n
    return c * lax.rsqrt(v + EPS)


def _attention_mask(n_x, n_mem):
    rows = n_x + 2 * n_mem
    r = lax.broadcasted_iota(jnp.int32, (rows, rows), 0)
    c = lax.broadcasted_iota(jnp.int32, (rows, rows), 1)
    r_mem, c_mem = r >= n_x, c >= n_x
    r_stream = jnp.where(r_mem, (r - n_x) // n_mem, r // SEG)
    c_stream = jnp.where(c_mem, (c - n_x) // n_mem, c // SEG)
    same = r_stream == c_stream
    visible = same & (r_mem | c_mem | (c <= r))
    fill = jnp.where(same, MASK_FILL, -jnp.inf).astype(F32)
    return visible, fill


def _kernel(xt_hbm, mem0_ref, wq_hbm, wk_hbm, wv_hbm, wot_hbm, w1_hbm, w3_hbm, w2t_hbm,
            out_hbm,
            xt_v, stage, wqkv, wot, w1, w3, w2t, w_sums,
            acts, ys, h_a, qkv_scr, p_scr, o_scr, g_scr, acc_t, out_v, sems, out_sems,
            *, n_heads, d_head, n_mem):
    d_model, seq = xt_v.shape
    n_seg = seq // SEG
    n_chunks = seq // LANES
    segs_per_chunk = LANES // SEG
    f_half = w1.shape[2]
    k_lo, k_hi, k_rest = slice(0, K_BLOCK), slice(K_BLOCK, 2 * K_BLOCK), slice(2 * K_BLOCK, d_model)
    scale = d_head ** -0.5

    def seg_rows(base, s):
        return pl.ds(pl.multiple_of(base + s * SEG, SEG), SEG)

    def pair_rows(start):
        return pl.ds(pl.multiple_of(start, 2 * SEG), 2 * SEG)

    def mixer_stages(h, n_x):
        rows = n_x + 2 * n_mem
        visible, fill = _attention_mask(n_x, n_mem)

        def project(i):
            cols = slice(3 * i * d_head, 3 * (i + 1) * d_head)
            qkv_scr[0:rows, cols] = jnp.dot(h, wqkv[:, cols], preferred_element_type=F32).astype(BF16)

        def scores(i):
            q = qkv_scr[0:rows, 3 * i * d_head:(3 * i + 1) * d_head]
            k = qkv_scr[0:rows, (3 * i + 1) * d_head:(3 * i + 2) * d_head]
            s = lax.dot_general(q, k, NT_DIMS, preferred_element_type=F32) * scale
            s = jnp.where(visible, s, fill)
            e = jnp.exp(s - jnp.max(s, axis=-1, keepdims=True))
            p = e * (1.0 / jnp.sum(e, axis=-1, keepdims=True))
            p_scr[i, 0:rows, 0:rows] = p.astype(BF16)

        def mix(i):
            v = qkv_scr[0:rows, (3 * i + 2) * d_head:(3 * i + 3) * d_head]
            o = jnp.dot(p_scr[i, 0:rows, 0:rows], v, preferred_element_type=F32)
            o_scr[0:rows, i * d_head:(i + 1) * d_head] = o.astype(BF16)

        def output(lo=0, hi=n_heads):
            cols = slice(lo * d_head, hi * d_head)
            return lax.dot_general(o_scr[0:rows, cols], wot[:, cols], NT_DIMS, preferred_element_type=F32)

        return project, scores, mix, output

    def dot(a, b):
        return jnp.dot(a, b, preferred_element_type=F32)

    def swiglu(gate, up):
        return (gate * jax.nn.sigmoid(gate) * up).astype(BF16)

    def ffn_stages(half, src0, src1, dst0, dst1):
        y = jnp.concatenate([ys[pair_rows(src0), :], ys[pair_rows(src1), :]], axis=0)
        h = _layernorm(y)
        top, bot = slice(0, 2 * SEG), slice(2 * SEG, 4 * SEG)
        a11, a12, a21, a22 = h[top, k_lo], h[top, k_hi], h[bot, k_lo], h[bot, k_hi]
        l1, l2, l3, l4, l5, l6, l7 = (
            a.astype(BF16) for a in (a11 + a22, a21 + a22, a11, a22, a11 + a12, a21 - a11, a12 - a22))
        rest = h[:, k_rest].astype(BF16)

        def hidden(f):
            cols = slice(f * F_CHUNK, (f + 1) * F_CHUNK)
            gate_rest = dot(rest, w1[half, k_rest, cols])
            up_rest = dot(rest, w3[half, k_rest, cols])
            m1 = dot(l1, w_sums[half, 0, :, cols])
            m2 = dot(l2, w1[half, k_lo, cols])
            m3 = dot(l3, w_sums[half, 1, :, cols])
            m4 = dot(l4, w_sums[half, 2, :, cols])
            m5 = dot(l5, w3[half, k_hi, cols])
            m6 = dot(l6, w_sums[half, 3, :, cols])
            m7 = dot(l7, w_sums[half, 4, :, cols])
            g_scr[top, cols] = swiglu(gate_rest[top] + m1 + m4 - m5 + m7, up_rest[top] + m3 + m5)
            g_scr[bot, cols] = swiglu(gate_rest[bot] + m2 + m4, up_rest[bot] + m1 - m2 + m3 + m6)

        def output():
            part = lax.dot_general(w2t[half], g_scr[...], NT_DIMS, preferred_element_type=F32)
            total = part + jnp.where(half == 1, acc_t[...], 0.0)
            acc_t[...] = total
            z = y + total.T
            acts[pair_rows(dst0), :] = z[top]
            acts[pair_rows(dst1), :] = z[bot]

        return [functools.partial(hidden, f) for f in range(f_half // F_CHUNK)], output

    def first_ffn():
        y = ys[0:2 * SEG, :]
        h = _layernorm(y).astype(BF16)
        z = y
        for half in range(2):
            for f in range(f_half // PLAIN_CHUNK):
                cols = slice(f * PLAIN_CHUNK, (f + 1) * PLAIN_CHUNK)
                rows = slice(half * 2 * SEG, (half + 1) * 2 * SEG)
                g_scr[rows, cols] = swiglu(dot(h, w1[half, :, cols]), dot(h, w3[half, :, cols]))
        for half in range(2):
            rows = slice(half * 2 * SEG, (half + 1) * 2 * SEG)
            z = z + lax.dot_general(g_scr[rows, :], w2t[half], NT_DIMS, preferred_element_type=F32)
        acts[seq:seq + 2 * SEG, :] = z

    def form_weight_sums(i, carry):
        per_half = K_BLOCK // SUM_ROWS
        half = i // per_half
        r0 = pl.multiple_of((i % per_half) * SUM_ROWS, SUM_ROWS)
        lo, hi = pl.ds(r0, SUM_ROWS), pl.ds(r0 + K_BLOCK, SUM_ROWS)
        for c in range(f_half // LANES):
            cols = slice(c * LANES, (c + 1) * LANES)
            b11, b21 = w1[half, lo, cols].astype(F32), w1[half, hi, cols].astype(F32)
            b12, b22 = w3[half, lo, cols].astype(F32), w3[half, hi, cols].astype(F32)
            for k, b in enumerate((b11 + b22, b12 - b22, b21 - b11, b11 + b12, b21 + b22)):
                w_sums[half, k, lo, cols] = b.astype(BF16)
        return carry

    def emit(matmul_work, scores, mix):
        for i in range(max(len(matmul_work), n_heads + 2 * STAGE_LAG)):
            if i < len(matmul_work):
                matmul_work[i]()
            if 0 <= i - STAGE_LAG < n_heads:
                scores(i - STAGE_LAG)
            if 0 <= i - 2 * STAGE_LAG < n_heads:
                mix(i - 2 * STAGE_LAG)

    def mixer_only(layer, s, mem):
        x = acts[seg_rows(layer * seq, s), :]
        tail = jnp.concatenate([mem, jnp.zeros_like(mem)], axis=0)
        h = jnp.concatenate([_layernorm(x).astype(BF16), tail.astype(BF16)], axis=0)
        project, scores, mix, output = mixer_stages(h, SEG)
        parts = []
        bounds = [0] + [n_heads - STAGE_LAG - k * STAGE_LAG // 1 for k in range(1, -1, -1)]
        emit([functools.partial(project, i) for i in range(n_heads)]
             + [lambda lo=lo, hi=hi: parts.append(output(lo, hi)) for lo, hi in [(0, n_heads - 2 * STAGE_LAG)]], scores, mix)
        att = parts[0] + output(n_heads - 2 * STAGE_LAG, n_heads)
        ys[seg_rows(layer * seq, s), :] = x + att[0:SEG]
        return att[SEG:SEG + n_mem]

    def stage_tokens(t):
        h_a[0:SEG, :] = _layernorm(acts[seg_rows(0, t), :]).astype(BF16)
        h_a[SEG:2 * SEG, :] = _layernorm(acts[seg_rows(seq, t - LAG), :]).astype(BF16)

    def transpose_out(c):
        rows = pl.ds(pl.multiple_of(2 * seq + c * LANES, LANES), LANES)
        out_v[c] = acts[rows, :].T.astype(out_v.dtype)

    def out_copy(c):
        return pltpu.make_async_copy(out_v.at[c], out_hbm.at[:, pl.ds(c * LANES, LANES)], out_sems.at[c])

    cp_x0 = pltpu.make_async_copy(xt_hbm.at[:, 0:LANES], xt_v.at[:, 0:LANES], sems.at[8])
    cp_x = pltpu.make_async_copy(xt_hbm.at[:, LANES:], xt_v.at[:, LANES:], sems.at[0])
    cp_qkv = [pltpu.make_async_copy(w, stage.at[i], sems.at[1 + i])
              for i, w in enumerate((wq_hbm, wk_hbm, wv_hbm))]
    cp_wo = [pltpu.make_async_copy(wot_hbm.at[i], wot.at[:, pl.ds(i * d_head, d_head)], sems.at[4])
             for i in range(n_heads)]
    cp_ff = [pltpu.make_async_copy(src.at[:, pl.ds(half * f_half, f_half)], dst.at[half], sems.at[5])
             for src, dst in ((w1_hbm, w1), (w3_hbm, w3), (w2t_hbm, w2t)) for half in range(2)]

    def transpose_in(c):
        acts[c * LANES:(c + 1) * LANES, :] = xt_v[:, c * LANES:(c + 1) * LANES].astype(F32).T

    cp_x0.start()
    cp_qkv[0].start()
    cp_qkv[1].start()
    cp_x0.wait()
    transpose_in(0)
    acts[2 * seq:2 * seq + LANES, :] = jnp.zeros((LANES, d_model), F32)
    acc_t[...] = jnp.zeros(acc_t.shape, F32)

    pairs = n_heads // 2
    for i in range(3):
        cp_qkv[i].wait()
        if i == 0:
            cp_qkv[2].start()
        elif i == 1:
            for cp in cp_wo:
                cp.start()
        words = stage.at[i].bitcast(jnp.uint32)
        for j in range(pairs):
            w = words[pl.ds(j, d_model, stride=pairs), :]
            c0 = (2 * j * 3 + i) * d_head
            c1 = ((2 * j + 1) * 3 + i) * d_head
            wqkv[:, c0:c0 + d_head] = pltpu.bitcast(w << 16, F32).astype(BF16)
            wqkv[:, c1:c1 + d_head] = pltpu.bitcast(w & jnp.uint32(0xFFFF0000), F32).astype(BF16)
    for cp in cp_ff:
        cp.start()
    for cp in cp_wo:
        cp.wait()

    def step(t, carry):
        half = t % 2
        src0 = (t - half - 2) * SEG
        lagged = (t - half - LAG - 2) * SEG
        ready = lagged >= 0
        hidden, ffn_output = ffn_stages(
            half, src0, jnp.where(ready, seq + lagged, 0),
            seq + src0, jnp.where(ready, 2 * seq + lagged, 3 * seq))
        project, scores, mix, mixer_output = mixer_stages(h_a[...], 2 * SEG)
        emit([functools.partial(project, i) for i in range(n_heads)] + hidden, scores, mix)
        transpose_out(jnp.maximum(t - out_delay, 0) // segs_per_chunk)
        ffn_output()
        stage_tokens(jnp.minimum(t + 1, n_seg - 1))
        att = mixer_output()
        h_a[2 * SEG:, :] = att[2 * SEG:].astype(BF16)
        ys[seg_rows(0, t), :] = acts[seg_rows(0, t), :] + att[0:SEG]
        ys[seg_rows(seq, t - LAG), :] = acts[seg_rows(seq, t - LAG), :] + att[SEG:2 * SEG]
        return carry

    out_delay = LAG + 2 + segs_per_chunk
    done = (n_seg - 1 - out_delay) // segs_per_chunk + 1
    mem0 = mem0_ref[...].astype(F32)
    h_a[2 * SEG:, :] = jnp.concatenate([mem0, mem0], axis=0).astype(BF16)

    def schedule_round(layer, carry):
        first = layer * (n_seg - LAG)
        mem = h_a[2 * SEG:, :].astype(F32)[n_mem:]
        mem = lax.fori_loop(first, first + LAG, functools.partial(mixer_only, layer), mem)

        @pl.when(layer == 0)
        def _():
            for cp in cp_ff:
                cp.wait()
            cp_x.start()
            lax.fori_loop(0, 2 * K_BLOCK // SUM_ROWS, form_weight_sums, 0)
            first_ffn()
            cp_x.wait()
            for c in range(1, n_chunks):
                transpose_in(c)
            stage_tokens(LAG)
            h_a[2 * SEG:, :] = jnp.concatenate([mem, mem0], axis=0).astype(BF16)
            lax.fori_loop(LAG, n_seg, step, 0)
            for c in range(done):
                out_copy(c).start()

        src0 = jnp.where(layer == 0, (n_seg - 2) * SEG, seq + (n_seg - 4) * SEG)
        src1 = jnp.where(layer == 0, seq + (n_seg - LAG - 2) * SEG, seq + (n_seg - 2) * SEG)

        def ffn_half(half, inner):
            hidden, output = ffn_stages(half, src0, src1, seq + src0, seq + src1)
            for work in hidden:
                work()
            output()
            return inner

        lax.fori_loop(0, 2, ffn_half, 0)
        return carry

    lax.fori_loop(0, 2, schedule_round, 0)
    for c in range(done, n_chunks):
        transpose_out(c)
        out_copy(c).start()
    for c in range(n_chunks):
        out_copy(c).wait()


@jax.jit
def pallas_interleave_layers__memory_aug_recurrent_mem_tr__glu_gated_swiglu__prompt_kernel(
    A_x, A_mem0, A_Wq, A_Wk, A_Wv, A_Wo, A_seg_len, B_x, B_w1, B_w3, B_w2,
):
    del A_seg_len, B_x
    batch, seq, d_model = A_x.shape
    _, n_heads, d_head = A_Wq.shape
    n_mem = A_mem0.shape[1]
    d_ff = B_w1.shape[1]
    assert batch == 1 and seq % 128 == 0 and d_ff % (2 * F_CHUNK) == 0
    rows = 2 * SEG + 2 * n_mem

    def kernel(*refs):
        _kernel(*refs, n_heads=n_heads, d_head=d_head, n_mem=n_mem)

    hbm = pl.BlockSpec(memory_space=pl.ANY)
    vmem = pl.BlockSpec(memory_space=pltpu.VMEM)
    out_t = pl.pallas_call(
        kernel,
        out_shape=jax.ShapeDtypeStruct((d_model, seq), A_x.dtype),
        in_specs=[hbm, vmem, hbm, hbm, hbm, hbm, hbm, hbm, hbm],
        out_specs=hbm,
        scratch_shapes=[
            pltpu.VMEM((d_model, seq), BF16),
            pltpu.VMEM((3, d_model * n_heads, d_head), BF16),
            pltpu.VMEM((d_model, 3 * n_heads * d_head), BF16),
            pltpu.VMEM((d_model, n_heads * d_head), BF16),
            pltpu.VMEM((2, d_model, d_ff // 2), BF16),
            pltpu.VMEM((2, d_model, d_ff // 2), BF16),
            pltpu.VMEM((2, d_model, d_ff // 2), BF16),
            pltpu.VMEM((2, 5, K_BLOCK, d_ff // 2), BF16),
            pltpu.VMEM((3 * seq + 2 * SEG, d_model), F32),
            pltpu.VMEM((2 * seq, d_model), F32),
            pltpu.VMEM((rows, d_model), BF16),
            pltpu.VMEM((rows, 3 * n_heads * d_head), BF16),
            pltpu.VMEM((n_heads, rows, rows), BF16),
            pltpu.VMEM((rows, n_heads * d_head), BF16),
            pltpu.VMEM((4 * SEG, d_ff // 2), BF16),
            pltpu.VMEM((d_model, 4 * SEG), F32),
            pltpu.VMEM((seq // LANES, d_model, LANES), A_x.dtype),
            pltpu.SemaphoreType.DMA((9,)),
            pltpu.SemaphoreType.DMA((seq // LANES,)),
        ],
        compiler_params=pltpu.CompilerParams(vmem_limit_bytes=120 * 1024 * 1024),
    )(
        A_x[0].T,
        A_mem0[0],
        A_Wq.reshape(d_model * n_heads, d_head),
        A_Wk.reshape(d_model * n_heads, d_head),
        A_Wv.reshape(d_model * n_heads, d_head),
        jnp.transpose(A_Wo, (0, 2, 1)),
        B_w1,
        B_w3,
        B_w2.T,
    )
    return out_t.T[None]
```

```python
import functools

import jax
import jax.numpy as jnp
from jax import lax
import jax.experimental.pallas as pl
import jax.experimental.pallas.tpu as pltpu

SEG = 32
EPS = 1e-5
MASK_FILL = -1000000000.0
LANES = 128
LAG = 4
K_BLOCK = 256
PLAIN_CHUNK = 256
SUM_ROWS = 32
STAGE_LAG = 5
BF16 = jnp.bfloat16
F32 = jnp.float32
NT_DIMS = (((1,), (1,)), ((), ()))


def _layernorm(x):
    inv_n = 1.0 / x.shape[-1]
    c = x - jnp.sum(x, axis=-1, keepdims=True) * inv_n
    v = jnp.sum(c * c, axis=-1, keepdims=True) * inv_n
    return c * lax.rsqrt(v + EPS)


def _strassen_lhs(a11, a12, a21, a22):
    return [a.astype(BF16) for a in (a11 + a22, a21 + a22, a11, a22, a11 + a12, a21 - a11, a12 - a22)]


def _strassen_rhs_sums(b11, b12, b21, b22):
    return [b.astype(BF16) for b in (b11 + b22, b12 - b22, b21 - b11, b11 + b12, b21 + b22)]


def _strassen_out(m1, m2, m3, m4, m5, m6, m7):
    return m1 + m4 - m5 + m7, m3 + m5, m2 + m4, m1 - m2 + m3 + m6


def _attention_mask(n_x, n_mem):
    rows = n_x + 2 * n_mem
    r = lax.broadcasted_iota(jnp.int32, (rows, rows), 0)
    c = lax.broadcasted_iota(jnp.int32, (rows, rows), 1)
    r_mem, c_mem = r >= n_x, c >= n_x
    r_stream = jnp.where(r_mem, (r - n_x) // n_mem, r // SEG)
    c_stream = jnp.where(c_mem, (c - n_x) // n_mem, c // SEG)
    same = r_stream == c_stream
    visible = same & (r_mem | c_mem | (c <= r))
    fill = jnp.where(same, MASK_FILL, -jnp.inf).astype(F32)
    return visible, fill


def _kernel(xt_hbm, mem0_ref, wq_hbm, wk_hbm, wv_hbm, wot_hbm, w1_hbm, w3_hbm, w2t_hbm,
            out_hbm,
            xt_v, stage, wqkv, wot, w1, w3, w2t, up_sums, down_sums,
            acts, ys, h_a, qkv_scr, p_scr, o_scr, g_scr, g_lhs, acc, out_v, sems, out_sems,
            *, n_heads, d_head, n_mem):
    d_model, seq = xt_v.shape
    n_seg = seq // SEG
    n_chunks = seq // LANES
    segs_per_chunk = LANES // SEG
    f_half = w1.shape[2]
    f_quarter = f_half // 2
    k_lo, k_hi, k_rest = slice(0, K_BLOCK), slice(K_BLOCK, 2 * K_BLOCK), slice(2 * K_BLOCK, d_model)
    scale = d_head ** -0.5

    def seg_rows(base, s):
        return pl.ds(pl.multiple_of(base + s * SEG, SEG), SEG)

    def pair_rows(start):
        return pl.ds(pl.multiple_of(start, 2 * SEG), 2 * SEG)

    def mixer_stages(h, n_x):
        rows = n_x + 2 * n_mem
        visible, fill = _attention_mask(n_x, n_mem)

        def project(i):
            cols = slice(3 * i * d_head, 3 * (i + 1) * d_head)
            qkv_scr[0:rows, cols] = jnp.dot(h, wqkv[:, cols], preferred_element_type=F32).astype(BF16)

        def scores(i):
            q = qkv_scr[0:rows, 3 * i * d_head:(3 * i + 1) * d_head]
            k = qkv_scr[0:rows, (3 * i + 1) * d_head:(3 * i + 2) * d_head]
            s = lax.dot_general(q, k, NT_DIMS, preferred_element_type=F32) * scale
            s = jnp.where(visible, s, fill)
            e = jnp.exp(s - jnp.max(s, axis=-1, keepdims=True))
            p = e * (1.0 / jnp.sum(e, axis=-1, keepdims=True))
            p_scr[i, 0:rows, 0:rows] = p.astype(BF16)

        def mix(i):
            v = qkv_scr[0:rows, (3 * i + 2) * d_head:(3 * i + 3) * d_head]
            o = jnp.dot(p_scr[i, 0:rows, 0:rows], v, preferred_element_type=F32)
            o_scr[0:rows, i * d_head:(i + 1) * d_head] = o.astype(BF16)

        def output(lo=0, hi=n_heads):
            cols = slice(lo * d_head, hi * d_head)
            return lax.dot_general(o_scr[0:rows, cols], wot[:, cols], NT_DIMS, preferred_element_type=F32)

        return project, scores, mix, output

    def dot(a, b):
        return jnp.dot(a, b, preferred_element_type=F32)

    def dot_nt(a, b):
        return lax.dot_general(a, b, NT_DIMS, preferred_element_type=F32)

    def swiglu(gate, up):
        half_gate = 0.5 * gate
        return (half_gate + half_gate * jnp.tanh(half_gate)) * up

    def ffn_stages(half, src0, src1, dst0, dst1):
        y = jnp.concatenate([ys[pair_rows(src0), :], ys[pair_rows(src1), :]], axis=0)
        h = _layernorm(y)
        top, bot = slice(0, 2 * SEG), slice(2 * SEG, 4 * SEG)
        lhs = _strassen_lhs(h[top, k_lo], h[top, k_hi], h[bot, k_lo], h[bot, k_hi])
        rest = h[:, k_rest].astype(BF16)

        def hidden_tile(cols):
            gate_rest = dot(rest, w1[half, k_rest, cols])
            up_rest = dot(rest, w3[half, k_rest, cols])
            rhs = (up_sums[half, 0, :, cols], w1[half, k_lo, cols], up_sums[half, 1, :, cols],
                   up_sums[half, 2, :, cols], w3[half, k_hi, cols], up_sums[half, 3, :, cols],
                   up_sums[half, 4, :, cols])
            gate_top, up_top, gate_bot, up_bot = _strassen_out(*(dot(a, b) for a, b in zip(lhs, rhs)))
            g_top = swiglu(gate_top + gate_rest[top], up_top + up_rest[top])
            g_bot = swiglu(gate_bot + gate_rest[bot], up_bot + up_rest[bot])
            g_scr[top, cols] = g_top.astype(BF16)
            g_scr[bot, cols] = g_bot.astype(BF16)
            return g_top, g_bot

        def hidden(f):
            cols = slice(f * LANES, (f + 1) * LANES)
            g11, g21 = hidden_tile(cols)
            g12, g22 = hidden_tile(slice(f_quarter + f * LANES, f_quarter + (f + 1) * LANES))
            sums = _strassen_lhs(g11, g12, g21, g22)
            for k, i in enumerate((0, 1, 4, 5, 6)):
                g_lhs[k, :, cols] = sums[i]

        def output():
            f_lo, f_hi = slice(0, f_quarter), slice(f_quarter, f_half)
            g = (g_lhs[0], g_lhs[1], g_scr[top, f_lo], g_scr[bot, f_hi], g_lhs[2], g_lhs[3], g_lhs[4])
            rhs = (down_sums[half, 0], w2t[half, k_lo, f_lo], down_sums[half, 1], down_sums[half, 2],
                   w2t[half, k_hi, f_hi], down_sums[half, 3], down_sums[half, 4])
            c11, c12, c21, c22 = _strassen_out(*(dot_nt(a, b) for a, b in zip(g, rhs)))
            rest_t = dot_nt(w2t[half, k_rest, :], g_scr[...])
            rest_t = jnp.concatenate([rest_t, jnp.zeros((LANES - rest_t.shape[0], 4 * SEG), F32)], axis=0)
            part = jnp.concatenate(
                [jnp.concatenate([c11, c21], axis=0), jnp.concatenate([c12, c22], axis=0),
                 rest_t.T[:, :d_model - 2 * K_BLOCK]], axis=1)
            z = part + jnp.where(half == 1, acc[...], y)
            acc[...] = z
            acts[pair_rows(dst0), :] = z[top]
            acts[pair_rows(dst1), :] = z[bot]

        return [functools.partial(hidden, f) for f in range(f_quarter // LANES)], output

    def first_ffn():
        y = ys[0:2 * SEG, :]
        h = _layernorm(y).astype(BF16)
        z = y
        for half in range(2):
            for f in range(f_half // PLAIN_CHUNK):
                cols = slice(f * PLAIN_CHUNK, (f + 1) * PLAIN_CHUNK)
                rows = slice(half * 2 * SEG, (half + 1) * 2 * SEG)
                g_scr[rows, cols] = swiglu(dot(h, w1[half, :, cols]), dot(h, w3[half, :, cols])).astype(BF16)
        for half in range(2):
            rows = slice(half * 2 * SEG, (half + 1) * 2 * SEG)
            z = z + lax.dot_general(g_scr[rows, :], w2t[half], NT_DIMS, preferred_element_type=F32)
        acts[seq:seq + 2 * SEG, :] = z

    def form_weight_sums(i, carry):
        per_half = K_BLOCK // SUM_ROWS
        half = i // per_half
        r0 = pl.multiple_of((i % per_half) * SUM_ROWS, SUM_ROWS)
        lo, hi = pl.ds(r0, SUM_ROWS), pl.ds(r0 + K_BLOCK, SUM_ROWS)
        for c in range(f_half // LANES):
            cols = slice(c * LANES, (c + 1) * LANES)
            blocks = (w1[half, lo, cols], w3[half, lo, cols], w1[half, hi, cols], w3[half, hi, cols])
            for k, b in enumerate(_strassen_rhs_sums(*(b.astype(F32) for b in blocks))):
                up_sums[half, k, lo, cols] = b
        for c in range(f_quarter // LANES):
            cols = slice(c * LANES, (c + 1) * LANES)
            cols_hi = slice(f_quarter + c * LANES, f_quarter + (c + 1) * LANES)
            blocks = (w2t[half, lo, cols], w2t[half, hi, cols], w2t[half, lo, cols_hi], w2t[half, hi, cols_hi])
            for k, b in enumerate(_strassen_rhs_sums(*(b.astype(F32) for b in blocks))):
                down_sums[half, k, lo, cols] = b
        return carry

    def emit(matmul_work, scores, mix):
        for i in range(max(len(matmul_work), n_heads + 2 * STAGE_LAG)):
            if i < len(matmul_work):
                matmul_work[i]()
            if 0 <= i - STAGE_LAG < n_heads:
                scores(i - STAGE_LAG)
            if 0 <= i - 2 * STAGE_LAG < n_heads:
                mix(i - 2 * STAGE_LAG)

    def mixer_only(layer, s, mem):
        x = acts[seg_rows(layer * seq, s), :]
        tail = jnp.concatenate([mem, jnp.zeros_like(mem)], axis=0)
        h = jnp.concatenate([_layernorm(x).astype(BF16), tail.astype(BF16)], axis=0)
        project, scores, mix, output = mixer_stages(h, SEG)
        parts = []
        bounds = [0] + [n_heads - STAGE_LAG - k * STAGE_LAG // 1 for k in range(1, -1, -1)]
        emit([functools.partial(project, i) for i in range(n_heads)]
             + [lambda lo=lo, hi=hi: parts.append(output(lo, hi)) for lo, hi in [(0, n_heads - 2 * STAGE_LAG)]], scores, mix)
        att = parts[0] + output(n_heads - 2 * STAGE_LAG, n_heads)
        ys[seg_rows(layer * seq, s), :] = x + att[0:SEG]
        return att[SEG:SEG + n_mem]

    def stage_tokens(t):
        h_a[0:SEG, :] = _layernorm(acts[seg_rows(0, t), :]).astype(BF16)
        h_a[SEG:2 * SEG, :] = _layernorm(acts[seg_rows(seq, t - LAG), :]).astype(BF16)

    def transpose_out(c):
        rows = pl.ds(pl.multiple_of(2 * seq + c * LANES, LANES), LANES)
        out_v[c] = acts[rows, :].T.astype(out_v.dtype)

    def out_copy(c):
        return pltpu.make_async_copy(out_v.at[c], out_hbm.at[:, pl.ds(c * LANES, LANES)], out_sems.at[c])

    cp_x0 = pltpu.make_async_copy(xt_hbm.at[:, 0:LANES], xt_v.at[:, 0:LANES], sems.at[8])
    cp_x = pltpu.make_async_copy(xt_hbm.at[:, LANES:], xt_v.at[:, LANES:], sems.at[0])
    cp_qkv = [pltpu.make_async_copy(w, stage.at[i], sems.at[1 + i])
              for i, w in enumerate((wq_hbm, wk_hbm, wv_hbm))]
    cp_wo = [pltpu.make_async_copy(wot_hbm.at[i], wot.at[:, pl.ds(i * d_head, d_head)], sems.at[4])
             for i in range(n_heads)]
    cp_ff = [pltpu.make_async_copy(src.at[:, pl.ds(half * f_half, f_half)], dst.at[half], sems.at[5])
             for src, dst in ((w1_hbm, w1), (w3_hbm, w3), (w2t_hbm, w2t)) for half in range(2)]

    def transpose_in(c):
        acts[c * LANES:(c + 1) * LANES, :] = xt_v[:, c * LANES:(c + 1) * LANES].astype(F32).T

    cp_x0.start()
    cp_qkv[0].start()
    cp_qkv[1].start()
    cp_x0.wait()
    transpose_in(0)
    acts[2 * seq:2 * seq + LANES, :] = jnp.zeros((LANES, d_model), F32)
    acc[...] = jnp.zeros(acc.shape, F32)

    pairs = n_heads // 2
    for i in range(3):
        cp_qkv[i].wait()
        if i == 0:
            cp_qkv[2].start()
        elif i == 1:
            for cp in cp_wo:
                cp.start()
        words = stage.at[i].bitcast(jnp.uint32)
        for j in range(pairs):
            w = words[pl.ds(j, d_model, stride=pairs), :]
            c0 = (2 * j * 3 + i) * d_head
            c1 = ((2 * j + 1) * 3 + i) * d_head
            wqkv[:, c0:c0 + d_head] = pltpu.bitcast(w << 16, F32).astype(BF16)
            wqkv[:, c1:c1 + d_head] = pltpu.bitcast(w & jnp.uint32(0xFFFF0000), F32).astype(BF16)
    for cp in cp_ff:
        cp.start()
    for cp in cp_wo:
        cp.wait()

    def step(t, carry):
        half = t % 2
        src0 = (t - half - 2) * SEG
        lagged = (t - half - LAG - 2) * SEG
        ready = lagged >= 0
        hidden, ffn_output = ffn_stages(
            half, src0, jnp.where(ready, seq + lagged, 0),
            seq + src0, jnp.where(ready, 2 * seq + lagged, 3 * seq))
        project, scores, mix, mixer_output = mixer_stages(h_a[...], 2 * SEG)
        emit([functools.partial(project, i) for i in range(n_heads)] + hidden, scores, mix)
        transpose_out(jnp.maximum(t - out_delay, 0) // segs_per_chunk)
        ffn_output()
        stage_tokens(jnp.minimum(t + 1, n_seg - 1))
        att = mixer_output()
        h_a[2 * SEG:, :] = att[2 * SEG:].astype(BF16)
        ys[seg_rows(0, t), :] = acts[seg_rows(0, t), :] + att[0:SEG]
        ys[seg_rows(seq, t - LAG), :] = acts[seg_rows(seq, t - LAG), :] + att[SEG:2 * SEG]
        return carry

    out_delay = LAG + 2 + segs_per_chunk
    done = (n_seg - 1 - out_delay) // segs_per_chunk + 1
    mem0 = mem0_ref[...].astype(F32)
    h_a[2 * SEG:, :] = jnp.concatenate([mem0, mem0], axis=0).astype(BF16)

    def schedule_round(layer, carry):
        first = layer * (n_seg - LAG)
        mem = h_a[2 * SEG:, :].astype(F32)[n_mem:]
        mem = lax.fori_loop(first, first + LAG, functools.partial(mixer_only, layer), mem)

        @pl.when(layer == 0)
        def _():
            for cp in cp_ff:
                cp.wait()
            cp_x.start()
            lax.fori_loop(0, 2 * K_BLOCK // SUM_ROWS, form_weight_sums, 0)
            first_ffn()
            cp_x.wait()
            for c in range(1, n_chunks):
                transpose_in(c)
            stage_tokens(LAG)
            h_a[2 * SEG:, :] = jnp.concatenate([mem, mem0], axis=0).astype(BF16)
            lax.fori_loop(LAG, n_seg, step, 0)
            for c in range(done):
                out_copy(c).start()

        src0 = jnp.where(layer == 0, (n_seg - 2) * SEG, seq + (n_seg - 4) * SEG)
        src1 = jnp.where(layer == 0, seq + (n_seg - LAG - 2) * SEG, seq + (n_seg - 2) * SEG)

        def ffn_half(half, inner):
            hidden, output = ffn_stages(half, src0, src1, seq + src0, seq + src1)
            for work in hidden:
                work()
            output()
            return inner

        lax.fori_loop(0, 2, ffn_half, 0)
        return carry

    lax.fori_loop(0, 2, schedule_round, 0)
    for c in range(done, n_chunks):
        transpose_out(c)
        out_copy(c).start()
    for c in range(n_chunks):
        out_copy(c).wait()


@jax.jit
def pallas_interleave_layers__memory_aug_recurrent_mem_tr__glu_gated_swiglu__prompt_kernel(
    A_x, A_mem0, A_Wq, A_Wk, A_Wv, A_Wo, A_seg_len, B_x, B_w1, B_w3, B_w2,
):
    del A_seg_len, B_x
    batch, seq, d_model = A_x.shape
    _, n_heads, d_head = A_Wq.shape
    n_mem = A_mem0.shape[1]
    d_ff = B_w1.shape[1]
    assert batch == 1 and seq % 128 == 0 and d_ff % (4 * LANES) == 0
    rows = 2 * SEG + 2 * n_mem

    def kernel(*refs):
        _kernel(*refs, n_heads=n_heads, d_head=d_head, n_mem=n_mem)

    hbm = pl.BlockSpec(memory_space=pl.ANY)
    vmem = pl.BlockSpec(memory_space=pltpu.VMEM)
    out_t = pl.pallas_call(
        kernel,
        out_shape=jax.ShapeDtypeStruct((d_model, seq), A_x.dtype),
        in_specs=[hbm, vmem, hbm, hbm, hbm, hbm, hbm, hbm, hbm],
        out_specs=hbm,
        scratch_shapes=[
            pltpu.VMEM((d_model, seq), BF16),
            pltpu.VMEM((3, d_model * n_heads, d_head), BF16),
            pltpu.VMEM((d_model, 3 * n_heads * d_head), BF16),
            pltpu.VMEM((d_model, n_heads * d_head), BF16),
            pltpu.VMEM((2, d_model, d_ff // 2), BF16),
            pltpu.VMEM((2, d_model, d_ff // 2), BF16),
            pltpu.VMEM((2, d_model, d_ff // 2), BF16),
            pltpu.VMEM((2, 5, K_BLOCK, d_ff // 2), BF16),
            pltpu.VMEM((2, 5, K_BLOCK, d_ff // 4), BF16),
            pltpu.VMEM((3 * seq + 2 * SEG, d_model), F32),
            pltpu.VMEM((2 * seq, d_model), F32),
            pltpu.VMEM((rows, d_model), BF16),
            pltpu.VMEM((rows, 3 * n_heads * d_head), BF16),
            pltpu.VMEM((n_heads, rows, rows), BF16),
            pltpu.VMEM((rows, n_heads * d_head), BF16),
            pltpu.VMEM((4 * SEG, d_ff // 2), BF16),
            pltpu.VMEM((5, 2 * SEG, d_ff // 4), BF16),
            pltpu.VMEM((4 * SEG, d_model), F32),
            pltpu.VMEM((seq // LANES, d_model, LANES), A_x.dtype),
            pltpu.SemaphoreType.DMA((9,)),
            pltpu.SemaphoreType.DMA((seq // LANES,)),
        ],
        compiler_params=pltpu.CompilerParams(vmem_limit_bytes=126 * 1024 * 1024),
    )(
        A_x[0].T,
        A_mem0[0],
        A_Wq.reshape(d_model * n_heads, d_head),
        A_Wk.reshape(d_model * n_heads, d_head),
        A_Wv.reshape(d_model * n_heads, d_head),
        jnp.transpose(A_Wo, (0, 2, 1)),
        B_w1,
        B_w3,
        B_w2.T,
    )
    return out_t.T[None]
```

```python
import functools

import jax
import jax.numpy as jnp
from jax import lax
import jax.experimental.pallas as pl
import jax.experimental.pallas.tpu as pltpu

SEG = 32
EPS = 1e-5
MASK_FILL = -1000000000.0
LANES = 128
LAG = 4
K_BLOCK = 256
PLAIN_CHUNK = 256
SUM_ROWS = 32
STAGE_LAG = 5
BF16 = jnp.bfloat16
F32 = jnp.float32
NT_DIMS = (((1,), (1,)), ((), ()))


def _layernorm(x):
    inv_n = 1.0 / x.shape[-1]
    c = x - jnp.sum(x, axis=-1, keepdims=True) * inv_n
    v = jnp.sum(c * c, axis=-1, keepdims=True) * inv_n
    return c * lax.rsqrt(v + EPS)


def _strassen_lhs(a11, a12, a21, a22):
    return [a.astype(BF16) for a in (a11 + a22, a21 + a22, a11, a22, a11 + a12, a21 - a11, a12 - a22)]


def _strassen_rhs_sums(b11, b12, b21, b22):
    return [b.astype(BF16) for b in (b11 + b22, b12 - b22, b21 - b11, b11 + b12, b21 + b22)]


def _strassen_out(m1, m2, m3, m4, m5, m6, m7):
    return m1 + m4 - m5 + m7, m3 + m5, m2 + m4, m1 - m2 + m3 + m6


def _attention_mask(n_x, n_mem):
    rows = n_x + 2 * n_mem
    r = lax.broadcasted_iota(jnp.int32, (rows, rows), 0)
    c = lax.broadcasted_iota(jnp.int32, (rows, rows), 1)
    r_mem, c_mem = r >= n_x, c >= n_x
    r_stream = jnp.where(r_mem, (r - n_x) // n_mem, r // SEG)
    c_stream = jnp.where(c_mem, (c - n_x) // n_mem, c // SEG)
    same = r_stream == c_stream
    visible = same & (r_mem | c_mem | (c <= r))
    fill = jnp.where(same, MASK_FILL, -jnp.inf).astype(F32)
    return visible, fill


def _kernel(xt_hbm, mem0_ref, wq_hbm, wk_hbm, wv_hbm, wot_hbm, w1_hbm, w3_hbm, w2t_hbm,
            out_hbm,
            xt_v, stage, wqkv, wot, w1, w3, w2t, up_sums, down_sums,
            acts, ys, h_a, qkv_scr, p_scr, o_scr, g_scr, g_lhs, acc, out_v, sems, out_sems,
            *, n_heads, d_head, n_mem):
    d_model, seq = xt_v.shape
    n_seg = seq // SEG
    n_chunks = seq // LANES
    segs_per_chunk = LANES // SEG
    f_half = w1.shape[2]
    f_quarter = f_half // 2
    k_lo, k_hi, k_rest = slice(0, K_BLOCK), slice(K_BLOCK, 2 * K_BLOCK), slice(2 * K_BLOCK, d_model)
    scale = d_head ** -0.5

    def seg_rows(base, s):
        return pl.ds(pl.multiple_of(base + s * SEG, SEG), SEG)

    def dot(a, b):
        return jnp.dot(a, b, preferred_element_type=F32)

    def dot_nt(a, b):
        return lax.dot_general(a, b, NT_DIMS, preferred_element_type=F32)

    def trailing_features(w_t, act):
        n, rows = w_t.shape[0], act.shape[0]
        out_t = dot_nt(w_t, act)
        if rows < LANES:
            out_t = jnp.concatenate([out_t, jnp.zeros((n, LANES - rows), F32)], axis=1)
        out_t = jnp.concatenate([out_t, jnp.zeros((LANES - n, LANES), F32)], axis=0)
        return out_t.T[:rows, :n]

    def pair_rows(start):
        return pl.ds(pl.multiple_of(start, 2 * SEG), 2 * SEG)

    def mixer_stages(h, n_x):
        rows = n_x + 2 * n_mem
        visible, fill = _attention_mask(n_x, n_mem)

        def project(i):
            cols = slice(3 * i * d_head, 3 * (i + 1) * d_head)
            qkv_scr[0:rows, cols] = jnp.dot(h, wqkv[:, cols], preferred_element_type=F32).astype(BF16)

        def scores(i):
            q = qkv_scr[0:rows, 3 * i * d_head:(3 * i + 1) * d_head]
            k = qkv_scr[0:rows, (3 * i + 1) * d_head:(3 * i + 2) * d_head]
            s = lax.dot_general(q, k, NT_DIMS, preferred_element_type=F32) * scale
            s = jnp.where(visible, s, fill)
            e = jnp.exp(s - jnp.max(s, axis=-1, keepdims=True))
            p = e * (1.0 / jnp.sum(e, axis=-1, keepdims=True))
            p_scr[i, 0:rows, 0:rows] = p.astype(BF16)

        def mix(i):
            v = qkv_scr[0:rows, (3 * i + 2) * d_head:(3 * i + 3) * d_head]
            o = jnp.dot(p_scr[i, 0:rows, 0:rows], v, preferred_element_type=F32)
            o_scr[0:rows, i * d_head:(i + 1) * d_head] = o.astype(BF16)

        def output(lo=0, hi=n_heads):
            cols = slice(lo * d_head, hi * d_head)
            rest = trailing_features(wot[k_rest, cols], o_scr[0:rows, cols])
            main = dot_nt(o_scr[0:rows, cols], wot[0:2 * K_BLOCK, cols])
            return jnp.concatenate([main, rest], axis=1)

        return project, scores, mix, output

    def swiglu(gate, up):
        half_gate = 0.5 * gate
        return (half_gate + half_gate * jnp.tanh(half_gate)) * up

    def ffn_stages(half, src0, src1, dst0, dst1):
        y = jnp.concatenate([ys[pair_rows(src0), :], ys[pair_rows(src1), :]], axis=0)
        h = _layernorm(y)
        top, bot = slice(0, 2 * SEG), slice(2 * SEG, 4 * SEG)
        lhs = _strassen_lhs(h[top, k_lo], h[top, k_hi], h[bot, k_lo], h[bot, k_hi])
        rest = h[:, k_rest].astype(BF16)

        def hidden_tile(cols):
            gate_rest = dot(rest, w1[half, k_rest, cols])
            up_rest = dot(rest, w3[half, k_rest, cols])
            rhs = (up_sums[half, 0, :, cols], w1[half, k_lo, cols], up_sums[half, 1, :, cols],
                   up_sums[half, 2, :, cols], w3[half, k_hi, cols], up_sums[half, 3, :, cols],
                   up_sums[half, 4, :, cols])
            gate_top, up_top, gate_bot, up_bot = _strassen_out(*(dot(a, b) for a, b in zip(lhs, rhs)))
            g_top = swiglu(gate_top + gate_rest[top], up_top + up_rest[top])
            g_bot = swiglu(gate_bot + gate_rest[bot], up_bot + up_rest[bot])
            g_scr[top, cols] = g_top.astype(BF16)
            g_scr[bot, cols] = g_bot.astype(BF16)
            return g_top, g_bot

        def hidden(f):
            cols = slice(f * LANES, (f + 1) * LANES)
            g11, g21 = hidden_tile(cols)
            g12, g22 = hidden_tile(slice(f_quarter + f * LANES, f_quarter + (f + 1) * LANES))
            sums = _strassen_lhs(g11, g12, g21, g22)
            for k, i in enumerate((0, 1, 4, 5, 6)):
                g_lhs[k, :, cols] = sums[i]

        def output():
            f_lo, f_hi = slice(0, f_quarter), slice(f_quarter, f_half)
            g = (g_lhs[0], g_lhs[1], g_scr[top, f_lo], g_scr[bot, f_hi], g_lhs[2], g_lhs[3], g_lhs[4])
            rhs = (down_sums[half, 0], w2t[half, k_lo, f_lo], down_sums[half, 1], down_sums[half, 2],
                   w2t[half, k_hi, f_hi], down_sums[half, 3], down_sums[half, 4])
            c11, c12, c21, c22 = _strassen_out(*(dot_nt(a, b) for a, b in zip(g, rhs)))
            part = jnp.concatenate(
                [jnp.concatenate([c11, c21], axis=0), jnp.concatenate([c12, c22], axis=0),
                 trailing_features(w2t[half, k_rest, :], g_scr[...])], axis=1)
            z = part + jnp.where(half == 1, acc[...], y)
            acc[...] = z
            acts[pair_rows(dst0), :] = z[top]
            acts[pair_rows(dst1), :] = z[bot]

        return [functools.partial(hidden, f) for f in range(f_quarter // LANES)], output

    def first_ffn():
        y = ys[0:2 * SEG, :]
        h = _layernorm(y).astype(BF16)
        z = y
        for half in range(2):
            for f in range(f_half // PLAIN_CHUNK):
                cols = slice(f * PLAIN_CHUNK, (f + 1) * PLAIN_CHUNK)
                rows = slice(half * 2 * SEG, (half + 1) * 2 * SEG)
                g_scr[rows, cols] = swiglu(dot(h, w1[half, :, cols]), dot(h, w3[half, :, cols])).astype(BF16)
        for half in range(2):
            rows = slice(half * 2 * SEG, (half + 1) * 2 * SEG)
            z = z + lax.dot_general(g_scr[rows, :], w2t[half], NT_DIMS, preferred_element_type=F32)
        acts[seq:seq + 2 * SEG, :] = z

    def form_weight_sums(i, carry):
        per_half = K_BLOCK // SUM_ROWS
        half = i // per_half
        r0 = pl.multiple_of((i % per_half) * SUM_ROWS, SUM_ROWS)
        lo, hi = pl.ds(r0, SUM_ROWS), pl.ds(r0 + K_BLOCK, SUM_ROWS)
        for c in range(f_half // LANES):
            cols = slice(c * LANES, (c + 1) * LANES)
            blocks = (w1[half, lo, cols], w3[half, lo, cols], w1[half, hi, cols], w3[half, hi, cols])
            for k, b in enumerate(_strassen_rhs_sums(*(b.astype(F32) for b in blocks))):
                up_sums[half, k, lo, cols] = b
        for c in range(f_quarter // LANES):
            cols = slice(c * LANES, (c + 1) * LANES)
            cols_hi = slice(f_quarter + c * LANES, f_quarter + (c + 1) * LANES)
            blocks = (w2t[half, lo, cols], w2t[half, hi, cols], w2t[half, lo, cols_hi], w2t[half, hi, cols_hi])
            for k, b in enumerate(_strassen_rhs_sums(*(b.astype(F32) for b in blocks))):
                down_sums[half, k, lo, cols] = b
        return carry

    def emit(matmul_work, scores, mix):
        for i in range(max(len(matmul_work), n_heads + 2 * STAGE_LAG)):
            if i < len(matmul_work):
                matmul_work[i]()
            if 0 <= i - STAGE_LAG < n_heads:
                scores(i - STAGE_LAG)
            if 0 <= i - 2 * STAGE_LAG < n_heads:
                mix(i - 2 * STAGE_LAG)

    def mixer_only(layer, s, mem):
        x = acts[seg_rows(layer * seq, s), :]
        tail = jnp.concatenate([mem, jnp.zeros_like(mem)], axis=0)
        h = jnp.concatenate([_layernorm(x).astype(BF16), tail.astype(BF16)], axis=0)
        project, scores, mix, output = mixer_stages(h, SEG)
        parts = []
        bounds = [0] + [n_heads - STAGE_LAG - k * STAGE_LAG // 1 for k in range(1, -1, -1)]
        emit([functools.partial(project, i) for i in range(n_heads)]
             + [lambda lo=lo, hi=hi: parts.append(output(lo, hi)) for lo, hi in [(0, n_heads - 2 * STAGE_LAG)]], scores, mix)
        att = parts[0] + output(n_heads - 2 * STAGE_LAG, n_heads)
        ys[seg_rows(layer * seq, s), :] = x + att[0:SEG]
        return att[SEG:SEG + n_mem]

    def stage_tokens(t):
        h_a[0:SEG, :] = _layernorm(acts[seg_rows(0, t), :]).astype(BF16)
        h_a[SEG:2 * SEG, :] = _layernorm(acts[seg_rows(seq, t - LAG), :]).astype(BF16)

    def transpose_out(c):
        rows = pl.ds(pl.multiple_of(2 * seq + c * LANES, LANES), LANES)
        out_v[c] = acts[rows, :].T.astype(out_v.dtype)

    def out_copy(c):
        return pltpu.make_async_copy(out_v.at[c], out_hbm.at[:, pl.ds(c * LANES, LANES)], out_sems.at[c])

    cp_x0 = pltpu.make_async_copy(xt_hbm.at[:, 0:LANES], xt_v.at[:, 0:LANES], sems.at[8])
    cp_x = pltpu.make_async_copy(xt_hbm.at[:, LANES:], xt_v.at[:, LANES:], sems.at[0])
    cp_qkv = [pltpu.make_async_copy(w, stage.at[i], sems.at[1 + i])
              for i, w in enumerate((wq_hbm, wk_hbm, wv_hbm))]
    cp_wo = [pltpu.make_async_copy(wot_hbm.at[i], wot.at[:, pl.ds(i * d_head, d_head)], sems.at[4])
             for i in range(n_heads)]
    cp_ff = [pltpu.make_async_copy(src.at[:, pl.ds(half * f_half, f_half)], dst.at[half], sems.at[5])
             for src, dst in ((w1_hbm, w1), (w3_hbm, w3), (w2t_hbm, w2t)) for half in range(2)]

    def transpose_in(c):
        acts[c * LANES:(c + 1) * LANES, :] = xt_v[:, c * LANES:(c + 1) * LANES].astype(F32).T

    cp_x0.start()
    cp_qkv[0].start()
    cp_qkv[1].start()
    cp_x0.wait()
    transpose_in(0)
    acts[2 * seq:2 * seq + LANES, :] = jnp.zeros((LANES, d_model), F32)
    acc[...] = jnp.zeros(acc.shape, F32)

    pairs = n_heads // 2
    for i in range(3):
        cp_qkv[i].wait()
        if i == 0:
            cp_qkv[2].start()
        elif i == 1:
            for cp in cp_wo:
                cp.start()
        words = stage.at[i].bitcast(jnp.uint32)
        for j in range(pairs):
            w = words[pl.ds(j, d_model, stride=pairs), :]
            c0 = (2 * j * 3 + i) * d_head
            c1 = ((2 * j + 1) * 3 + i) * d_head
            wqkv[:, c0:c0 + d_head] = pltpu.bitcast(w << 16, F32).astype(BF16)
            wqkv[:, c1:c1 + d_head] = pltpu.bitcast(w & jnp.uint32(0xFFFF0000), F32).astype(BF16)
    for cp in cp_ff:
        cp.start()
    for cp in cp_wo:
        cp.wait()

    def step(t, carry):
        half = t % 2
        src0 = (t - half - 2) * SEG
        lagged = (t - half - LAG - 2) * SEG
        ready = lagged >= 0
        hidden, ffn_output = ffn_stages(
            half, src0, jnp.where(ready, seq + lagged, 0),
            seq + src0, jnp.where(ready, 2 * seq + lagged, 3 * seq))
        project, scores, mix, mixer_output = mixer_stages(h_a[...], 2 * SEG)
        emit([functools.partial(project, i) for i in range(n_heads)] + hidden, scores, mix)
        transpose_out(jnp.maximum(t - out_delay, 0) // segs_per_chunk)
        ffn_output()
        stage_tokens(jnp.minimum(t + 1, n_seg - 1))
        att = mixer_output()
        h_a[2 * SEG:, :] = att[2 * SEG:].astype(BF16)
        ys[seg_rows(0, t), :] = acts[seg_rows(0, t), :] + att[0:SEG]
        ys[seg_rows(seq, t - LAG), :] = acts[seg_rows(seq, t - LAG), :] + att[SEG:2 * SEG]
        return carry

    out_delay = LAG + 2 + segs_per_chunk
    done = (n_seg - 1 - out_delay) // segs_per_chunk + 1
    mem0 = mem0_ref[...].astype(F32)
    h_a[2 * SEG:, :] = jnp.concatenate([mem0, mem0], axis=0).astype(BF16)

    def schedule_round(layer, carry):
        first = layer * (n_seg - LAG)
        mem = h_a[2 * SEG:, :].astype(F32)[n_mem:]
        mem = lax.fori_loop(first, first + LAG, functools.partial(mixer_only, layer), mem)

        @pl.when(layer == 0)
        def _():
            for cp in cp_ff:
                cp.wait()
            cp_x.start()
            lax.fori_loop(0, 2 * K_BLOCK // SUM_ROWS, form_weight_sums, 0)
            first_ffn()
            cp_x.wait()
            for c in range(1, n_chunks):
                transpose_in(c)
            stage_tokens(LAG)
            h_a[2 * SEG:, :] = jnp.concatenate([mem, mem0], axis=0).astype(BF16)
            lax.fori_loop(LAG, n_seg, step, 0)
            for c in range(done):
                out_copy(c).start()

        src0 = jnp.where(layer == 0, (n_seg - 2) * SEG, seq + (n_seg - 4) * SEG)
        src1 = jnp.where(layer == 0, seq + (n_seg - LAG - 2) * SEG, seq + (n_seg - 2) * SEG)

        def ffn_half(half, inner):
            hidden, output = ffn_stages(half, src0, src1, seq + src0, seq + src1)
            for work in hidden:
                work()
            output()
            return inner

        lax.fori_loop(0, 2, ffn_half, 0)
        return carry

    lax.fori_loop(0, 2, schedule_round, 0)
    for c in range(done, n_chunks):
        transpose_out(c)
        out_copy(c).start()
    for c in range(n_chunks):
        out_copy(c).wait()


@jax.jit
def pallas_interleave_layers__memory_aug_recurrent_mem_tr__glu_gated_swiglu__prompt_kernel(
    A_x, A_mem0, A_Wq, A_Wk, A_Wv, A_Wo, A_seg_len, B_x, B_w1, B_w3, B_w2,
):
    del A_seg_len, B_x
    batch, seq, d_model = A_x.shape
    _, n_heads, d_head = A_Wq.shape
    n_mem = A_mem0.shape[1]
    d_ff = B_w1.shape[1]
    assert batch == 1 and seq % 128 == 0 and d_ff % (4 * LANES) == 0
    rows = 2 * SEG + 2 * n_mem

    def kernel(*refs):
        _kernel(*refs, n_heads=n_heads, d_head=d_head, n_mem=n_mem)

    hbm = pl.BlockSpec(memory_space=pl.ANY)
    vmem = pl.BlockSpec(memory_space=pltpu.VMEM)
    out_t = pl.pallas_call(
        kernel,
        out_shape=jax.ShapeDtypeStruct((d_model, seq), A_x.dtype),
        in_specs=[hbm, vmem, hbm, hbm, hbm, hbm, hbm, hbm, hbm],
        out_specs=hbm,
        scratch_shapes=[
            pltpu.VMEM((d_model, seq), BF16),
            pltpu.VMEM((3, d_model * n_heads, d_head), BF16),
            pltpu.VMEM((d_model, 3 * n_heads * d_head), BF16),
            pltpu.VMEM((d_model, n_heads * d_head), BF16),
            pltpu.VMEM((2, d_model, d_ff // 2), BF16),
            pltpu.VMEM((2, d_model, d_ff // 2), BF16),
            pltpu.VMEM((2, d_model, d_ff // 2), BF16),
            pltpu.VMEM((2, 5, K_BLOCK, d_ff // 2), BF16),
            pltpu.VMEM((2, 5, K_BLOCK, d_ff // 4), BF16),
            pltpu.VMEM((3 * seq + 2 * SEG, d_model), F32),
            pltpu.VMEM((2 * seq, d_model), F32),
            pltpu.VMEM((rows, d_model), BF16),
            pltpu.VMEM((rows, 3 * n_heads * d_head), BF16),
            pltpu.VMEM((n_heads, rows, rows), BF16),
            pltpu.VMEM((rows, n_heads * d_head), BF16),
            pltpu.VMEM((4 * SEG, d_ff // 2), BF16),
            pltpu.VMEM((5, 2 * SEG, d_ff // 4), BF16),
            pltpu.VMEM((4 * SEG, d_model), F32),
            pltpu.VMEM((seq // LANES, d_model, LANES), A_x.dtype),
            pltpu.SemaphoreType.DMA((9,)),
            pltpu.SemaphoreType.DMA((seq // LANES,)),
        ],
        compiler_params=pltpu.CompilerParams(vmem_limit_bytes=126 * 1024 * 1024),
    )(
        A_x[0].T,
        A_mem0[0],
        A_Wq.reshape(d_model * n_heads, d_head),
        A_Wk.reshape(d_model * n_heads, d_head),
        A_Wv.reshape(d_model * n_heads, d_head),
        jnp.transpose(A_Wo, (0, 2, 1)),
        B_w1,
        B_w3,
        B_w2.T,
    )
    return out_t.T[None]
```

```python
import functools

import jax
import jax.numpy as jnp
from jax import lax
import jax.experimental.pallas as pl
import jax.experimental.pallas.tpu as pltpu

SEG = 32
EPS = 1e-5
MASK_FILL = -1000000000.0
LANES = 128
LAG = 4
K_BLOCK = 256
PLAIN_CHUNK = 256
SUM_ROWS = 32
STAGE_LAG = 5
BF16 = jnp.bfloat16
F32 = jnp.float32
NT_DIMS = (((1,), (1,)), ((), ()))


def _layernorm(x):
    inv_n = 1.0 / x.shape[-1]
    c = x - jnp.sum(x, axis=-1, keepdims=True) * inv_n
    v = jnp.sum(c * c, axis=-1, keepdims=True) * inv_n
    return c * lax.rsqrt(v + EPS)


def _strassen_lhs(a11, a12, a21, a22):
    return [a.astype(BF16) for a in (a11 + a22, a21 + a22, a11, a22, a11 + a12, a21 - a11, a12 - a22)]


def _strassen_rhs_sums(b11, b12, b21, b22):
    return [b.astype(BF16) for b in (b11 + b22, b12 - b22, b21 - b11, b11 + b12, b21 + b22)]


def _strassen_out(m1, m2, m3, m4, m5, m6, m7):
    return m1 + m4 - m5 + m7, m3 + m5, m2 + m4, m1 - m2 + m3 + m6


def _attention_mask(n_x, n_mem):
    rows = n_x + 2 * n_mem
    r = lax.broadcasted_iota(jnp.int32, (rows, rows), 0)
    c = lax.broadcasted_iota(jnp.int32, (rows, rows), 1)
    r_mem, c_mem = r >= n_x, c >= n_x
    r_stream = jnp.where(r_mem, (r - n_x) // n_mem, r // SEG)
    c_stream = jnp.where(c_mem, (c - n_x) // n_mem, c // SEG)
    same = r_stream == c_stream
    visible = same & (r_mem | c_mem | (c <= r))
    fill = jnp.where(same, MASK_FILL, -jnp.inf).astype(F32)
    return visible, fill


def _kernel(xt_hbm, mem0_ref, wq_hbm, wk_hbm, wv_hbm, wot_hbm, w1_hbm, w3_hbm, w2t_hbm,
            out_hbm,
            xt_v, stage, wqkv, wot, w1, w3, w2t, up_sums, down_sums,
            acts, ys, h_a, qkv_scr, p_scr, o_scr, g_scr, g_lhs, acc, out_v, sems, out_sems,
            *, n_heads, d_head, n_mem):
    d_model, seq = xt_v.shape
    n_seg = seq // SEG
    n_chunks = seq // LANES
    segs_per_chunk = LANES // SEG
    f_half = w1.shape[2]
    f_quarter = f_half // 2
    k_lo, k_hi, k_rest = slice(0, K_BLOCK), slice(K_BLOCK, 2 * K_BLOCK), slice(2 * K_BLOCK, d_model)
    scale = d_head ** -0.5

    def seg_rows(base, s):
        return pl.ds(pl.multiple_of(base + s * SEG, SEG), SEG)

    def dot(a, b):
        return jnp.dot(a, b, preferred_element_type=F32)

    def dot_nt(a, b):
        return lax.dot_general(a, b, NT_DIMS, preferred_element_type=F32)

    def trailing_features(w_t, act):
        n, rows = w_t.shape[0], act.shape[0]
        out_t = dot_nt(w_t, act)
        if rows < LANES:
            out_t = jnp.concatenate([out_t, jnp.zeros((n, LANES - rows), F32)], axis=1)
        out_t = jnp.concatenate([out_t, jnp.zeros((LANES - n, LANES), F32)], axis=0)
        return out_t.T[:rows, :n]

    def pair_rows(start):
        return pl.ds(pl.multiple_of(start, 2 * SEG), 2 * SEG)

    def mixer_stages(h, n_x):
        rows = n_x + 2 * n_mem
        visible, fill = _attention_mask(n_x, n_mem)

        def project(i):
            cols = slice(3 * i * d_head, 3 * (i + 1) * d_head)
            qkv_scr[0:rows, cols] = jnp.dot(h, wqkv[:, cols], preferred_element_type=F32).astype(BF16)

        def scores(i):
            q = qkv_scr[0:rows, 3 * i * d_head:(3 * i + 1) * d_head]
            k = qkv_scr[0:rows, (3 * i + 1) * d_head:(3 * i + 2) * d_head]
            s = lax.dot_general(q, k, NT_DIMS, preferred_element_type=F32) * scale
            s = jnp.where(visible, s, fill)
            e = jnp.exp(s - jnp.max(s, axis=-1, keepdims=True))
            p = e * (1.0 / jnp.sum(e, axis=-1, keepdims=True))
            p_scr[i, 0:rows, 0:rows] = p.astype(BF16)

        def mix(i):
            v = qkv_scr[0:rows, (3 * i + 2) * d_head:(3 * i + 3) * d_head]
            o = jnp.dot(p_scr[i, 0:rows, 0:rows], v, preferred_element_type=F32)
            o_scr[0:rows, i * d_head:(i + 1) * d_head] = o.astype(BF16)

        def output():
            rest = trailing_features(wot[k_rest, :], o_scr[0:rows, :])
            main = dot_nt(o_scr[0:rows, :], wot[0:2 * K_BLOCK, :])
            return jnp.concatenate([main, rest], axis=1)

        return project, scores, mix, output

    def swiglu(gate, up):
        half_gate = 0.5 * gate
        return (half_gate + half_gate * jnp.tanh(half_gate)) * up

    def ffn_stages(half, src0, src1, dst0, dst1):
        y = jnp.concatenate([ys[pair_rows(src0), :], ys[pair_rows(src1), :]], axis=0)
        h = _layernorm(y)
        top, bot = slice(0, 2 * SEG), slice(2 * SEG, 4 * SEG)
        lhs = _strassen_lhs(h[top, k_lo], h[top, k_hi], h[bot, k_lo], h[bot, k_hi])
        rest = h[:, k_rest].astype(BF16)

        def hidden_tile(cols):
            gate_rest = dot(rest, w1[half, k_rest, cols])
            up_rest = dot(rest, w3[half, k_rest, cols])
            rhs = (up_sums[half, 0, :, cols], w1[half, k_lo, cols], up_sums[half, 1, :, cols],
                   up_sums[half, 2, :, cols], w3[half, k_hi, cols], up_sums[half, 3, :, cols],
                   up_sums[half, 4, :, cols])
            gate_top, up_top, gate_bot, up_bot = _strassen_out(*(dot(a, b) for a, b in zip(lhs, rhs)))
            g_top = swiglu(gate_top + gate_rest[top], up_top + up_rest[top])
            g_bot = swiglu(gate_bot + gate_rest[bot], up_bot + up_rest[bot])
            g_scr[top, cols] = g_top.astype(BF16)
            g_scr[bot, cols] = g_bot.astype(BF16)
            return g_top, g_bot

        def hidden(f):
            cols = slice(f * LANES, (f + 1) * LANES)
            g11, g21 = hidden_tile(cols)
            g12, g22 = hidden_tile(slice(f_quarter + f * LANES, f_quarter + (f + 1) * LANES))
            sums = _strassen_lhs(g11, g12, g21, g22)
            for k, i in enumerate((0, 1, 4, 5, 6)):
                g_lhs[k, :, cols] = sums[i]

        def output():
            f_lo, f_hi = slice(0, f_quarter), slice(f_quarter, f_half)
            g = (g_lhs[0], g_lhs[1], g_scr[top, f_lo], g_scr[bot, f_hi], g_lhs[2], g_lhs[3], g_lhs[4])
            rhs = (down_sums[half, 0], w2t[half, k_lo, f_lo], down_sums[half, 1], down_sums[half, 2],
                   w2t[half, k_hi, f_hi], down_sums[half, 3], down_sums[half, 4])
            c11, c12, c21, c22 = _strassen_out(*(dot_nt(a, b) for a, b in zip(g, rhs)))
            part = jnp.concatenate(
                [jnp.concatenate([c11, c21], axis=0), jnp.concatenate([c12, c22], axis=0),
                 trailing_features(w2t[half, k_rest, :], g_scr[...])], axis=1)
            z = part + jnp.where(half == 1, acc[...], y)
            acc[...] = z
            acts[pair_rows(dst0), :] = z[top]
            acts[pair_rows(dst1), :] = z[bot]

        return [functools.partial(hidden, f) for f in range(f_quarter // LANES)], output

    def first_ffn():
        y = ys[0:2 * SEG, :]
        h = _layernorm(y).astype(BF16)
        z = y
        for half in range(2):
            for f in range(f_half // PLAIN_CHUNK):
                cols = slice(f * PLAIN_CHUNK, (f + 1) * PLAIN_CHUNK)
                rows = slice(half * 2 * SEG, (half + 1) * 2 * SEG)
                g_scr[rows, cols] = swiglu(dot(h, w1[half, :, cols]), dot(h, w3[half, :, cols])).astype(BF16)
        for half in range(2):
            rows = slice(half * 2 * SEG, (half + 1) * 2 * SEG)
            z = z + lax.dot_general(g_scr[rows, :], w2t[half], NT_DIMS, preferred_element_type=F32)
        acts[seq:seq + 2 * SEG, :] = z

    def form_weight_sums(i, carry):
        per_half = K_BLOCK // SUM_ROWS
        half = i // per_half
        r0 = pl.multiple_of((i % per_half) * SUM_ROWS, SUM_ROWS)
        lo, hi = pl.ds(r0, SUM_ROWS), pl.ds(r0 + K_BLOCK, SUM_ROWS)
        for c in range(f_half // LANES):
            cols = slice(c * LANES, (c + 1) * LANES)
            blocks = (w1[half, lo, cols], w3[half, lo, cols], w1[half, hi, cols], w3[half, hi, cols])
            for k, b in enumerate(_strassen_rhs_sums(*(b.astype(F32) for b in blocks))):
                up_sums[half, k, lo, cols] = b
        for c in range(f_quarter // LANES):
            cols = slice(c * LANES, (c + 1) * LANES)
            cols_hi = slice(f_quarter + c * LANES, f_quarter + (c + 1) * LANES)
            blocks = (w2t[half, lo, cols], w2t[half, hi, cols], w2t[half, lo, cols_hi], w2t[half, hi, cols_hi])
            for k, b in enumerate(_strassen_rhs_sums(*(b.astype(F32) for b in blocks))):
                down_sums[half, k, lo, cols] = b
        return carry

    def emit(matmul_work, scores, mix):
        for i in range(max(len(matmul_work), n_heads + 2 * STAGE_LAG)):
            if i < len(matmul_work):
                matmul_work[i]()
            if 0 <= i - STAGE_LAG < n_heads:
                scores(i - STAGE_LAG)
            if 0 <= i - 2 * STAGE_LAG < n_heads:
                mix(i - 2 * STAGE_LAG)

    def mixer_only(layer, s, mem):
        x = acts[seg_rows(layer * seq, s), :]
        tail = jnp.concatenate([mem, jnp.zeros_like(mem)], axis=0)
        h = jnp.concatenate([_layernorm(x).astype(BF16), tail.astype(BF16)], axis=0)
        project, scores, mix, output = mixer_stages(h, SEG)
        emit([functools.partial(project, i) for i in range(n_heads)], scores, mix)

        @pl.when(s == 0)
        def _():
            for cp in cp_wo:
                cp.wait()

        att = output()
        ys[seg_rows(layer * seq, s), :] = x + att[0:SEG]
        return att[SEG:SEG + n_mem]

    def stage_tokens(t):
        h_a[0:SEG, :] = _layernorm(acts[seg_rows(0, t), :]).astype(BF16)
        h_a[SEG:2 * SEG, :] = _layernorm(acts[seg_rows(seq, t - LAG), :]).astype(BF16)

    def transpose_out(c):
        rows = pl.ds(pl.multiple_of(2 * seq + c * LANES, LANES), LANES)
        out_v[c] = acts[rows, :].T.astype(out_v.dtype)

    def out_copy(c):
        return pltpu.make_async_copy(out_v.at[c], out_hbm.at[:, pl.ds(pl.multiple_of(c * LANES, LANES), LANES)],
                                     out_sems.at[c])

    cp_x0 = pltpu.make_async_copy(xt_hbm.at[:, 0:LANES], xt_v.at[:, 0:LANES], sems.at[8])
    cp_x = pltpu.make_async_copy(xt_hbm.at[:, LANES:], xt_v.at[:, LANES:], sems.at[0])
    cp_qkv = [pltpu.make_async_copy(w, stage.at[i], sems.at[1 + i])
              for i, w in enumerate((wq_hbm, wk_hbm, wv_hbm))]
    cp_wo = [pltpu.make_async_copy(wot_hbm.at[i], wot.at[:, pl.ds(i * d_head, d_head)], sems.at[4])
             for i in range(n_heads)]
    cp_ff = [pltpu.make_async_copy(src.at[:, pl.ds(half * f_half, f_half)], dst.at[half], sems.at[5])
             for src, dst in ((w1_hbm, w1), (w3_hbm, w3), (w2t_hbm, w2t)) for half in range(2)]

    def transpose_in(c):
        acts[c * LANES:(c + 1) * LANES, :] = xt_v[:, c * LANES:(c + 1) * LANES].astype(F32).T

    cp_x0.start()
    cp_qkv[0].start()
    cp_qkv[1].start()
    cp_x0.wait()
    transpose_in(0)
    acts[2 * seq:2 * seq + LANES, :] = jnp.zeros((LANES, d_model), F32)
    acc[...] = jnp.zeros(acc.shape, F32)

    pairs = n_heads // 2
    for i in range(3):
        cp_qkv[i].wait()
        if i == 0:
            cp_qkv[2].start()
        elif i == 1:
            for cp in cp_wo:
                cp.start()
        words = stage.at[i].bitcast(jnp.uint32)
        for j in range(pairs):
            w = words[pl.ds(j, d_model, stride=pairs), :]
            c0 = (2 * j * 3 + i) * d_head
            c1 = ((2 * j + 1) * 3 + i) * d_head
            wqkv[:, c0:c0 + d_head] = pltpu.bitcast(w << 16, F32).astype(BF16)
            wqkv[:, c1:c1 + d_head] = pltpu.bitcast(w & jnp.uint32(0xFFFF0000), F32).astype(BF16)
    for cp in cp_ff:
        cp.start()

    def step(t, carry):
        half = t % 2
        src0 = (t - half - 2) * SEG
        lagged = (t - half - LAG - 2) * SEG
        ready = lagged >= 0
        hidden, ffn_output = ffn_stages(
            half, src0, jnp.where(ready, seq + lagged, 0),
            seq + src0, jnp.where(ready, 2 * seq + lagged, 3 * seq))
        project, scores, mix, mixer_output = mixer_stages(h_a[...], 2 * SEG)
        emit([functools.partial(project, i) for i in range(n_heads)] + hidden, scores, mix)
        transpose_out(jnp.maximum(t - out_delay, 0) // segs_per_chunk)
        ffn_output()
        stage_tokens(jnp.minimum(t + 1, n_seg - 1))
        att = mixer_output()
        h_a[2 * SEG:, :] = att[2 * SEG:].astype(BF16)
        ys[seg_rows(0, t), :] = acts[seg_rows(0, t), :] + att[0:SEG]
        ys[seg_rows(seq, t - LAG), :] = acts[seg_rows(seq, t - LAG), :] + att[SEG:2 * SEG]
        return carry

    out_delay = LAG + 2 + segs_per_chunk
    done = (n_seg - 1 - out_delay) // segs_per_chunk + 1
    mem0 = mem0_ref[...].astype(F32)
    h_a[2 * SEG:, :] = jnp.concatenate([mem0, mem0], axis=0).astype(BF16)

    def schedule_round(layer, carry):
        first = layer * (n_seg - LAG)
        mem = h_a[2 * SEG:, :].astype(F32)[n_mem:]
        mem = lax.fori_loop(first, first + LAG, functools.partial(mixer_only, layer), mem)

        @pl.when(layer == 0)
        def _():
            for cp in cp_ff:
                cp.wait()
            cp_x.start()
            lax.fori_loop(0, 2 * K_BLOCK // SUM_ROWS, form_weight_sums, 0)
            first_ffn()
            cp_x.wait()
            for c in range(1, n_chunks):
                transpose_in(c)
            stage_tokens(LAG)
            h_a[2 * SEG:, :] = jnp.concatenate([mem, mem0], axis=0).astype(BF16)
            lax.fori_loop(LAG, n_seg, step, 0)
            for c in range(done):
                out_copy(c).start()

        src0 = jnp.where(layer == 0, (n_seg - 2) * SEG, seq + (n_seg - 4) * SEG)
        src1 = jnp.where(layer == 0, seq + (n_seg - LAG - 2) * SEG, seq + (n_seg - 2) * SEG)

        def ffn_half(half, inner):
            hidden, output = ffn_stages(half, src0, src1, seq + src0, seq + src1)
            for work in hidden:
                work()
            output()
            return inner

        lax.fori_loop(0, 2, ffn_half, 0)
        transpose_out(done + layer)
        out_copy(done + layer).start()
        return carry

    lax.fori_loop(0, 2, schedule_round, 0)
    for c in range(n_chunks):
        out_copy(c).wait()


@jax.jit
def pallas_interleave_layers__memory_aug_recurrent_mem_tr__glu_gated_swiglu__prompt_kernel(
    A_x, A_mem0, A_Wq, A_Wk, A_Wv, A_Wo, A_seg_len, B_x, B_w1, B_w3, B_w2,
):
    del A_seg_len, B_x
    batch, seq, d_model = A_x.shape
    _, n_heads, d_head = A_Wq.shape
    n_mem = A_mem0.shape[1]
    d_ff = B_w1.shape[1]
    assert batch == 1 and seq % 128 == 0 and d_ff % (4 * LANES) == 0
    rows = 2 * SEG + 2 * n_mem

    def kernel(*refs):
        _kernel(*refs, n_heads=n_heads, d_head=d_head, n_mem=n_mem)

    hbm = pl.BlockSpec(memory_space=pl.ANY)
    vmem = pl.BlockSpec(memory_space=pltpu.VMEM)
    out_t = pl.pallas_call(
        kernel,
        out_shape=jax.ShapeDtypeStruct((d_model, seq), A_x.dtype),
        in_specs=[hbm, vmem, hbm, hbm, hbm, hbm, hbm, hbm, hbm],
        out_specs=hbm,
        scratch_shapes=[
            pltpu.VMEM((d_model, seq), BF16),
            pltpu.VMEM((3, d_model * n_heads, d_head), BF16),
            pltpu.VMEM((d_model, 3 * n_heads * d_head), BF16),
            pltpu.VMEM((d_model, n_heads * d_head), BF16),
            pltpu.VMEM((2, d_model, d_ff // 2), BF16),
            pltpu.VMEM((2, d_model, d_ff // 2), BF16),
            pltpu.VMEM((2, d_model, d_ff // 2), BF16),
            pltpu.VMEM((2, 5, K_BLOCK, d_ff // 2), BF16),
            pltpu.VMEM((2, 5, K_BLOCK, d_ff // 4), BF16),
            pltpu.VMEM((3 * seq + 2 * SEG, d_model), F32),
            pltpu.VMEM((2 * seq, d_model), F32),
            pltpu.VMEM((rows, d_model), BF16),
            pltpu.VMEM((rows, 3 * n_heads * d_head), BF16),
            pltpu.VMEM((n_heads, rows, rows), BF16),
            pltpu.VMEM((rows, n_heads * d_head), BF16),
            pltpu.VMEM((4 * SEG, d_ff // 2), BF16),
            pltpu.VMEM((5, 2 * SEG, d_ff // 4), BF16),
            pltpu.VMEM((4 * SEG, d_model), F32),
            pltpu.VMEM((seq // LANES, d_model, LANES), A_x.dtype),
            pltpu.SemaphoreType.DMA((9,)),
            pltpu.SemaphoreType.DMA((seq // LANES,)),
        ],
        compiler_params=pltpu.CompilerParams(vmem_limit_bytes=126 * 1024 * 1024),
    )(
        A_x[0].T,
        A_mem0[0],
        A_Wq.reshape(d_model * n_heads, d_head),
        A_Wk.reshape(d_model * n_heads, d_head),
        A_Wv.reshape(d_model * n_heads, d_head),
        jnp.transpose(A_Wo, (0, 2, 1)),
        B_w1,
        B_w3,
        B_w2.T,
    )
    return out_t.T[None]
```

```python
import functools

import jax
import jax.numpy as jnp
from jax import lax
import jax.experimental.pallas as pl
import jax.experimental.pallas.tpu as pltpu

SEG = 32
EPS = 1e-5
MASK_FILL = -1000000000.0
LANES = 128
LAG = 4
QKV_PARTS = 4
K_BLOCK = 256
PLAIN_CHUNK = 256
SUM_ROWS = 32
STAGE_LAG = 5
BF16 = jnp.bfloat16
F32 = jnp.float32
NT_DIMS = (((1,), (1,)), ((), ()))


def _layernorm(x):
    inv_n = 1.0 / x.shape[-1]
    c = x - jnp.sum(x, axis=-1, keepdims=True) * inv_n
    v = jnp.sum(c * c, axis=-1, keepdims=True) * inv_n
    return c * lax.rsqrt(v + EPS)


def _strassen_lhs(a11, a12, a21, a22):
    return [a.astype(BF16) for a in (a11 + a22, a21 + a22, a11, a22, a11 + a12, a21 - a11, a12 - a22)]


def _strassen_rhs_sums(b11, b12, b21, b22):
    return [b.astype(BF16) for b in (b11 + b22, b12 - b22, b21 - b11, b11 + b12, b21 + b22)]


def _strassen_out(m1, m2, m3, m4, m5, m6, m7):
    return m1 + m4 - m5 + m7, m3 + m5, m2 + m4, m1 - m2 + m3 + m6


def _attention_mask(n_x, n_mem):
    rows = n_x + 2 * n_mem
    r = lax.broadcasted_iota(jnp.int32, (rows, rows), 0)
    c = lax.broadcasted_iota(jnp.int32, (rows, rows), 1)
    r_mem, c_mem = r >= n_x, c >= n_x
    r_stream = jnp.where(r_mem, (r - n_x) // n_mem, r // SEG)
    c_stream = jnp.where(c_mem, (c - n_x) // n_mem, c // SEG)
    same = r_stream == c_stream
    visible = same & (r_mem | c_mem | (c <= r))
    fill = jnp.where(same, MASK_FILL, -jnp.inf).astype(F32)
    return visible, fill


def _kernel(xt_hbm, mem0_ref, wq_hbm, wk_hbm, wv_hbm, wot_hbm, w1_hbm, w3_hbm, w2t_hbm,
            out_hbm,
            xt_v, stage, wqkv, wot, w1, w3, w2t, up_sums, down_sums,
            acts, ys, h_a, qkv_scr, p_scr, o_scr, g_scr, g_lhs, acc, out_v, sems, qkv_sems, out_sems,
            *, n_heads, d_head, n_mem):
    d_model, seq = xt_v.shape
    n_seg = seq // SEG
    n_chunks = seq // LANES
    segs_per_chunk = LANES // SEG
    f_half = w1.shape[2]
    f_quarter = f_half // 2
    k_lo, k_hi, k_rest = slice(0, K_BLOCK), slice(K_BLOCK, 2 * K_BLOCK), slice(2 * K_BLOCK, d_model)
    scale = d_head ** -0.5

    def seg_rows(base, s):
        return pl.ds(pl.multiple_of(base + s * SEG, SEG), SEG)

    def dot(a, b):
        return jnp.dot(a, b, preferred_element_type=F32)

    def dot_nt(a, b):
        return lax.dot_general(a, b, NT_DIMS, preferred_element_type=F32)

    def trailing_features(w_t, act):
        n, rows = w_t.shape[0], act.shape[0]
        out_t = dot_nt(w_t, act)
        if rows < LANES:
            out_t = jnp.concatenate([out_t, jnp.zeros((n, LANES - rows), F32)], axis=1)
        out_t = jnp.concatenate([out_t, jnp.zeros((LANES - n, LANES), F32)], axis=0)
        return out_t.T[:rows, :n]

    def pair_rows(start):
        return pl.ds(pl.multiple_of(start, 2 * SEG), 2 * SEG)

    def mixer_stages(h, n_x):
        rows = n_x + 2 * n_mem
        visible, fill = _attention_mask(n_x, n_mem)

        def project(i):
            cols = slice(3 * i * d_head, 3 * (i + 1) * d_head)
            qkv_scr[0:rows, cols] = jnp.dot(h, wqkv[:, cols], preferred_element_type=F32).astype(BF16)

        def scores(i):
            q = qkv_scr[0:rows, 3 * i * d_head:(3 * i + 1) * d_head]
            k = qkv_scr[0:rows, (3 * i + 1) * d_head:(3 * i + 2) * d_head]
            s = lax.dot_general(q, k, NT_DIMS, preferred_element_type=F32) * scale
            s = jnp.where(visible, s, fill)
            e = jnp.exp(s - jnp.max(s, axis=-1, keepdims=True))
            p = e * (1.0 / jnp.sum(e, axis=-1, keepdims=True))
            p_scr[i, 0:rows, 0:rows] = p.astype(BF16)

        def mix(i):
            v = qkv_scr[0:rows, (3 * i + 2) * d_head:(3 * i + 3) * d_head]
            o = jnp.dot(p_scr[i, 0:rows, 0:rows], v, preferred_element_type=F32)
            o_scr[0:rows, i * d_head:(i + 1) * d_head] = o.astype(BF16)

        def output():
            rest = trailing_features(wot[k_rest, :], o_scr[0:rows, :])
            main = dot_nt(o_scr[0:rows, :], wot[0:2 * K_BLOCK, :])
            return jnp.concatenate([main, rest], axis=1)

        return project, scores, mix, output

    def swiglu(gate, up):
        half_gate = 0.5 * gate
        return (half_gate + half_gate * jnp.tanh(half_gate)) * up

    def ffn_stages(half, src0, src1, dst0, dst1):
        y = jnp.concatenate([ys[pair_rows(src0), :], ys[pair_rows(src1), :]], axis=0)
        h = _layernorm(y)
        top, bot = slice(0, 2 * SEG), slice(2 * SEG, 4 * SEG)
        lhs = _strassen_lhs(h[top, k_lo], h[top, k_hi], h[bot, k_lo], h[bot, k_hi])
        rest = h[:, k_rest].astype(BF16)

        def hidden_tile(cols):
            gate_rest = dot(rest, w1[half, k_rest, cols])
            up_rest = dot(rest, w3[half, k_rest, cols])
            rhs = (up_sums[half, 0, :, cols], w1[half, k_lo, cols], up_sums[half, 1, :, cols],
                   up_sums[half, 2, :, cols], w3[half, k_hi, cols], up_sums[half, 3, :, cols],
                   up_sums[half, 4, :, cols])
            gate_top, up_top, gate_bot, up_bot = _strassen_out(*(dot(a, b) for a, b in zip(lhs, rhs)))
            g_top = swiglu(gate_top + gate_rest[top], up_top + up_rest[top])
            g_bot = swiglu(gate_bot + gate_rest[bot], up_bot + up_rest[bot])
            g_scr[top, cols] = g_top.astype(BF16)
            g_scr[bot, cols] = g_bot.astype(BF16)
            return g_top, g_bot

        def hidden(f):
            cols = slice(f * LANES, (f + 1) * LANES)
            g11, g21 = hidden_tile(cols)
            g12, g22 = hidden_tile(slice(f_quarter + f * LANES, f_quarter + (f + 1) * LANES))
            sums = _strassen_lhs(g11, g12, g21, g22)
            for k, i in enumerate((0, 1, 4, 5, 6)):
                g_lhs[k, :, cols] = sums[i]

        def output():
            f_lo, f_hi = slice(0, f_quarter), slice(f_quarter, f_half)
            g = (g_lhs[0], g_lhs[1], g_scr[top, f_lo], g_scr[bot, f_hi], g_lhs[2], g_lhs[3], g_lhs[4])
            rhs = (down_sums[half, 0], w2t[half, k_lo, f_lo], down_sums[half, 1], down_sums[half, 2],
                   w2t[half, k_hi, f_hi], down_sums[half, 3], down_sums[half, 4])
            c11, c12, c21, c22 = _strassen_out(*(dot_nt(a, b) for a, b in zip(g, rhs)))
            part = jnp.concatenate(
                [jnp.concatenate([c11, c21], axis=0), jnp.concatenate([c12, c22], axis=0),
                 trailing_features(w2t[half, k_rest, :], g_scr[...])], axis=1)
            z = part + jnp.where(half == 1, acc[...], y)
            acc[...] = z
            acts[pair_rows(dst0), :] = z[top]
            acts[pair_rows(dst1), :] = z[bot]

        return [functools.partial(hidden, f) for f in range(f_quarter // LANES)], output

    def first_ffn():
        y = ys[0:2 * SEG, :]
        h = _layernorm(y).astype(BF16)
        z = y
        for half in range(2):
            for f in range(f_half // PLAIN_CHUNK):
                cols = slice(f * PLAIN_CHUNK, (f + 1) * PLAIN_CHUNK)
                rows = slice(half * 2 * SEG, (half + 1) * 2 * SEG)
                g_scr[rows, cols] = swiglu(dot(h, w1[half, :, cols]), dot(h, w3[half, :, cols])).astype(BF16)
        for half in range(2):
            rows = slice(half * 2 * SEG, (half + 1) * 2 * SEG)
            z = z + lax.dot_general(g_scr[rows, :], w2t[half], NT_DIMS, preferred_element_type=F32)
        acts[seq:seq + 2 * SEG, :] = z

    def form_weight_sums(i, carry):
        per_half = K_BLOCK // SUM_ROWS
        half = i // per_half
        r0 = pl.multiple_of((i % per_half) * SUM_ROWS, SUM_ROWS)
        lo, hi = pl.ds(r0, SUM_ROWS), pl.ds(r0 + K_BLOCK, SUM_ROWS)
        for c in range(f_half // LANES):
            cols = slice(c * LANES, (c + 1) * LANES)
            blocks = (w1[half, lo, cols], w3[half, lo, cols], w1[half, hi, cols], w3[half, hi, cols])
            for k, b in enumerate(_strassen_rhs_sums(*(b.astype(F32) for b in blocks))):
                up_sums[half, k, lo, cols] = b
        for c in range(f_quarter // LANES):
            cols = slice(c * LANES, (c + 1) * LANES)
            cols_hi = slice(f_quarter + c * LANES, f_quarter + (c + 1) * LANES)
            blocks = (w2t[half, lo, cols], w2t[half, hi, cols], w2t[half, lo, cols_hi], w2t[half, hi, cols_hi])
            for k, b in enumerate(_strassen_rhs_sums(*(b.astype(F32) for b in blocks))):
                down_sums[half, k, lo, cols] = b
        return carry

    def emit(matmul_work, scores, mix):
        for i in range(max(len(matmul_work), n_heads + 2 * STAGE_LAG)):
            if i < len(matmul_work):
                matmul_work[i]()
            if 0 <= i - STAGE_LAG < n_heads:
                scores(i - STAGE_LAG)
            if 0 <= i - 2 * STAGE_LAG < n_heads:
                mix(i - 2 * STAGE_LAG)

    def mixer_only(layer, s, mem):
        x = acts[seg_rows(layer * seq, s), :]
        tail = jnp.concatenate([mem, jnp.zeros_like(mem)], axis=0)
        h = jnp.concatenate([_layernorm(x).astype(BF16), tail.astype(BF16)], axis=0)
        project, scores, mix, output = mixer_stages(h, SEG)
        emit([functools.partial(project, i) for i in range(n_heads)], scores, mix)

        @pl.when(s == 0)
        def _():
            for cp in cp_wo:
                cp.wait()

        att = output()
        ys[seg_rows(layer * seq, s), :] = x + att[0:SEG]
        return att[SEG:SEG + n_mem]

    def stage_tokens(t):
        h_a[0:SEG, :] = _layernorm(acts[seg_rows(0, t), :]).astype(BF16)
        h_a[SEG:2 * SEG, :] = _layernorm(acts[seg_rows(seq, t - LAG), :]).astype(BF16)

    def transpose_out(c):
        rows = pl.ds(pl.multiple_of(2 * seq + c * LANES, LANES), LANES)
        out_v[c] = acts[rows, :].T.astype(out_v.dtype)

    def out_copy(c):
        return pltpu.make_async_copy(out_v.at[c], out_hbm.at[:, pl.ds(pl.multiple_of(c * LANES, LANES), LANES)],
                                     out_sems.at[c])

    cp_x0 = pltpu.make_async_copy(xt_hbm.at[:, 0:LANES], xt_v.at[:, 0:LANES], sems.at[8])
    cp_x = pltpu.make_async_copy(xt_hbm.at[:, LANES:], xt_v.at[:, LANES:], sems.at[0])
    part_rows = d_model // QKV_PARTS
    cp_qkv = [pltpu.make_async_copy(w.at[pl.ds(p * part_rows * n_heads, part_rows * n_heads)],
                                    stage.at[i * QKV_PARTS + p], qkv_sems.at[i * QKV_PARTS + p])
              for i, w in enumerate((wq_hbm, wk_hbm, wv_hbm)) for p in range(QKV_PARTS)]
    cp_wo = [pltpu.make_async_copy(wot_hbm.at[i], wot.at[:, pl.ds(i * d_head, d_head)], sems.at[4])
             for i in range(n_heads)]
    cp_ff = [pltpu.make_async_copy(src.at[:, pl.ds(half * f_half, f_half)], dst.at[half], sems.at[5])
             for src, dst in ((w1_hbm, w1), (w3_hbm, w3), (w2t_hbm, w2t)) for half in range(2)]

    def transpose_in(c):
        acts[c * LANES:(c + 1) * LANES, :] = xt_v[:, c * LANES:(c + 1) * LANES].astype(F32).T

    cp_x0.start()
    cp_qkv[0].start()
    cp_qkv[1].start()
    cp_x0.wait()
    transpose_in(0)
    acts[2 * seq:2 * seq + LANES, :] = jnp.zeros((LANES, d_model), F32)
    acc[...] = jnp.zeros(acc.shape, F32)

    pairs = n_heads // 2
    for n, cp in enumerate(cp_qkv):
        cp.wait()
        if n + 2 < len(cp_qkv):
            cp_qkv[n + 2].start()
        elif n + 2 == len(cp_qkv):
            for cp_head in cp_wo:
                cp_head.start()
        i, p = divmod(n, QKV_PARTS)
        words = stage.at[n].bitcast(jnp.uint32)
        features = slice(p * part_rows, (p + 1) * part_rows)
        for j in range(pairs):
            w = words[pl.ds(j, part_rows, stride=pairs), :]
            c0 = (2 * j * 3 + i) * d_head
            c1 = ((2 * j + 1) * 3 + i) * d_head
            wqkv[features, c0:c0 + d_head] = pltpu.bitcast(w << 16, F32).astype(BF16)
            wqkv[features, c1:c1 + d_head] = pltpu.bitcast(w & jnp.uint32(0xFFFF0000), F32).astype(BF16)
    for cp in cp_ff:
        cp.start()

    def step(t, carry):
        half = t % 2
        src0 = (t - half - 2) * SEG
        lagged = (t - half - LAG - 2) * SEG
        ready = lagged >= 0
        hidden, ffn_output = ffn_stages(
            half, src0, jnp.where(ready, seq + lagged, 0),
            seq + src0, jnp.where(ready, 2 * seq + lagged, 3 * seq))
        project, scores, mix, mixer_output = mixer_stages(h_a[...], 2 * SEG)
        emit([functools.partial(project, i) for i in range(n_heads)] + hidden, scores, mix)
        transpose_out(jnp.maximum(t - out_delay, 0) // segs_per_chunk)
        ffn_output()
        stage_tokens(jnp.minimum(t + 1, n_seg - 1))
        att = mixer_output()
        h_a[2 * SEG:, :] = att[2 * SEG:].astype(BF16)
        ys[seg_rows(0, t), :] = acts[seg_rows(0, t), :] + att[0:SEG]
        ys[seg_rows(seq, t - LAG), :] = acts[seg_rows(seq, t - LAG), :] + att[SEG:2 * SEG]
        return carry

    out_delay = LAG + 2 + segs_per_chunk
    done = (n_seg - 1 - out_delay) // segs_per_chunk + 1
    mem0 = mem0_ref[...].astype(F32)
    h_a[2 * SEG:, :] = jnp.concatenate([mem0, mem0], axis=0).astype(BF16)

    def schedule_round(layer, carry):
        first = layer * (n_seg - LAG)
        mem = h_a[2 * SEG:, :].astype(F32)[n_mem:]
        mem = lax.fori_loop(first, first + LAG, functools.partial(mixer_only, layer), mem)

        @pl.when(layer == 0)
        def _():
            for cp in cp_ff:
                cp.wait()
            cp_x.start()
            lax.fori_loop(0, 2 * K_BLOCK // SUM_ROWS, form_weight_sums, 0)
            first_ffn()
            cp_x.wait()
            for c in range(1, n_chunks):
                transpose_in(c)
            stage_tokens(LAG)
            h_a[2 * SEG:, :] = jnp.concatenate([mem, mem0], axis=0).astype(BF16)
            lax.fori_loop(LAG, n_seg, step, 0)
            for c in range(done):
                out_copy(c).start()

        src0 = jnp.where(layer == 0, (n_seg - 2) * SEG, seq + (n_seg - 4) * SEG)
        src1 = jnp.where(layer == 0, seq + (n_seg - LAG - 2) * SEG, seq + (n_seg - 2) * SEG)

        def ffn_half(half, inner):
            hidden, output = ffn_stages(half, src0, src1, seq + src0, seq + src1)
            for work in hidden:
                work()
            output()
            return inner

        lax.fori_loop(0, 2, ffn_half, 0)
        transpose_out(done + layer)
        out_copy(done + layer).start()
        return carry

    lax.fori_loop(0, 2, schedule_round, 0)
    for c in range(n_chunks):
        out_copy(c).wait()


@jax.jit
def pallas_interleave_layers__memory_aug_recurrent_mem_tr__glu_gated_swiglu__prompt_kernel(
    A_x, A_mem0, A_Wq, A_Wk, A_Wv, A_Wo, A_seg_len, B_x, B_w1, B_w3, B_w2,
):
    del A_seg_len, B_x
    batch, seq, d_model = A_x.shape
    _, n_heads, d_head = A_Wq.shape
    n_mem = A_mem0.shape[1]
    d_ff = B_w1.shape[1]
    assert batch == 1 and seq % 128 == 0 and d_ff % (4 * LANES) == 0
    rows = 2 * SEG + 2 * n_mem

    def kernel(*refs):
        _kernel(*refs, n_heads=n_heads, d_head=d_head, n_mem=n_mem)

    hbm = pl.BlockSpec(memory_space=pl.ANY)
    vmem = pl.BlockSpec(memory_space=pltpu.VMEM)
    out_t = pl.pallas_call(
        kernel,
        out_shape=jax.ShapeDtypeStruct((d_model, seq), A_x.dtype),
        in_specs=[hbm, vmem, hbm, hbm, hbm, hbm, hbm, hbm, hbm],
        out_specs=hbm,
        scratch_shapes=[
            pltpu.VMEM((d_model, seq), BF16),
            pltpu.VMEM((3 * QKV_PARTS, d_model * n_heads // QKV_PARTS, d_head), BF16),
            pltpu.VMEM((d_model, 3 * n_heads * d_head), BF16),
            pltpu.VMEM((d_model, n_heads * d_head), BF16),
            pltpu.VMEM((2, d_model, d_ff // 2), BF16),
            pltpu.VMEM((2, d_model, d_ff // 2), BF16),
            pltpu.VMEM((2, d_model, d_ff // 2), BF16),
            pltpu.VMEM((2, 5, K_BLOCK, d_ff // 2), BF16),
            pltpu.VMEM((2, 5, K_BLOCK, d_ff // 4), BF16),
            pltpu.VMEM((3 * seq + 2 * SEG, d_model), F32),
            pltpu.VMEM((2 * seq, d_model), F32),
            pltpu.VMEM((rows, d_model), BF16),
            pltpu.VMEM((rows, 3 * n_heads * d_head), BF16),
            pltpu.VMEM((n_heads, rows, rows), BF16),
            pltpu.VMEM((rows, n_heads * d_head), BF16),
            pltpu.VMEM((4 * SEG, d_ff // 2), BF16),
            pltpu.VMEM((5, 2 * SEG, d_ff // 4), BF16),
            pltpu.VMEM((4 * SEG, d_model), F32),
            pltpu.VMEM((seq // LANES, d_model, LANES), A_x.dtype),
            pltpu.SemaphoreType.DMA((9,)),
            pltpu.SemaphoreType.DMA((3 * QKV_PARTS,)),
            pltpu.SemaphoreType.DMA((seq // LANES,)),
        ],
        compiler_params=pltpu.CompilerParams(vmem_limit_bytes=126 * 1024 * 1024),
    )(
        A_x[0].T,
        A_mem0[0],
        A_Wq.reshape(d_model * n_heads, d_head),
        A_Wk.reshape(d_model * n_heads, d_head),
        A_Wv.reshape(d_model * n_heads, d_head),
        jnp.transpose(A_Wo, (0, 2, 1)),
        B_w1,
        B_w3,
        B_w2.T,
    )
    return out_t.T[None]
```

```python
import functools

import jax
import jax.numpy as jnp
from jax import lax
import jax.experimental.pallas as pl
import jax.experimental.pallas.tpu as pltpu

SEG = 32
EPS = 1e-5
MASK_FILL = -1000000000.0
LANES = 128
LAG = 4
SPLIT_ROWS = 48
QKV_PARTS = 4
K_BLOCK = 256
PLAIN_CHUNK = 256
SUM_ROWS = 32
STAGE_LAG = 5
BF16 = jnp.bfloat16
F32 = jnp.float32
NT_DIMS = (((1,), (1,)), ((), ()))


def _layernorm(x):
    inv_n = 1.0 / x.shape[-1]
    c = x - jnp.sum(x, axis=-1, keepdims=True) * inv_n
    v = jnp.sum(c * c, axis=-1, keepdims=True) * inv_n
    return c * lax.rsqrt(v + EPS)


def _strassen_lhs(a11, a12, a21, a22):
    return [a.astype(BF16) for a in (a11 + a22, a21 + a22, a11, a22, a11 + a12, a21 - a11, a12 - a22)]


def _strassen_rhs_sums(b11, b12, b21, b22):
    return [b.astype(BF16) for b in (b11 + b22, b12 - b22, b21 - b11, b11 + b12, b21 + b22)]


def _strassen_out(m1, m2, m3, m4, m5, m6, m7):
    return m1 + m4 - m5 + m7, m3 + m5, m2 + m4, m1 - m2 + m3 + m6


def _attention_mask(n_x, n_mem):
    rows = n_x + 2 * n_mem
    r = lax.broadcasted_iota(jnp.int32, (rows, rows), 0)
    c = lax.broadcasted_iota(jnp.int32, (rows, rows), 1)
    r_mem, c_mem = r >= n_x, c >= n_x
    r_stream = jnp.where(r_mem, (r - n_x) // n_mem, r // SEG)
    c_stream = jnp.where(c_mem, (c - n_x) // n_mem, c // SEG)
    same = r_stream == c_stream
    visible = same & (r_mem | c_mem | (c <= r))
    fill = jnp.where(same, MASK_FILL, -jnp.inf).astype(F32)
    return visible, fill


def _kernel(xt_hbm, mem0_ref, wq_hbm, wk_hbm, wv_hbm, wot_hbm, w1_hbm, w3_hbm, w2t_hbm,
            out_hbm,
            xt_v, stage, wqkv, wot, w1, w3, w2t, up_sums, down_sums,
            acts, ys, h_a, qkv_scr, p_scr, o_scr, g_scr, g_lhs, acc, out_v, sems, qkv_sems, out_sems,
            *, n_heads, d_head, n_mem):
    d_model, seq = xt_hbm.shape
    n_seg = seq // SEG
    n_chunks = seq // LANES
    segs_per_chunk = LANES // SEG
    f_half = w1.shape[2]
    f_quarter = f_half // 2
    k_lo, k_hi, k_rest = slice(0, K_BLOCK), slice(K_BLOCK, 2 * K_BLOCK), slice(2 * K_BLOCK, d_model)
    scale = d_head ** -0.5

    def seg_rows(base, s):
        return pl.ds(pl.multiple_of(base + s * SEG, SEG), SEG)

    def dot(a, b):
        return jnp.dot(a, b, preferred_element_type=F32)

    def dot_nt(a, b):
        return lax.dot_general(a, b, NT_DIMS, preferred_element_type=F32)

    def trailing_features(w_t, act):
        n, rows = w_t.shape[0], act.shape[0]
        out_t = dot_nt(w_t, act)
        if rows < LANES:
            out_t = jnp.concatenate([out_t, jnp.zeros((n, LANES - rows), F32)], axis=1)
        out_t = jnp.concatenate([out_t, jnp.zeros((LANES - n, LANES), F32)], axis=0)
        return out_t.T[:rows, :n]

    def pair_rows(start):
        return pl.ds(pl.multiple_of(start, 2 * SEG), 2 * SEG)

    def mixer_stages(h, n_x):
        rows = n_x + 2 * n_mem
        visible, fill = _attention_mask(n_x, n_mem)

        def project(i):
            cols = slice(3 * i * d_head, 3 * (i + 1) * d_head)
            qkv_scr[0:rows, cols] = jnp.dot(h, wqkv[:, cols], preferred_element_type=F32).astype(BF16)

        def scores(i):
            q = qkv_scr[0:rows, 3 * i * d_head:(3 * i + 1) * d_head]
            k = qkv_scr[0:rows, (3 * i + 1) * d_head:(3 * i + 2) * d_head]
            s = lax.dot_general(q, k, NT_DIMS, preferred_element_type=F32) * scale
            s = jnp.where(visible, s, fill)
            e = jnp.exp(s - jnp.max(s, axis=-1, keepdims=True))
            p = e * (1.0 / jnp.sum(e, axis=-1, keepdims=True))
            p_scr[i, 0:rows, 0:rows] = p.astype(BF16)

        def mix(i):
            v = qkv_scr[0:rows, (3 * i + 2) * d_head:(3 * i + 3) * d_head]
            o = jnp.dot(p_scr[i, 0:rows, 0:rows], v, preferred_element_type=F32)
            o_scr[0:rows, i * d_head:(i + 1) * d_head] = o.astype(BF16)

        def output():
            rest = trailing_features(wot[k_rest, :], o_scr[0:rows, :])
            main = dot_nt(o_scr[0:rows, :], wot[0:2 * K_BLOCK, :])
            return jnp.concatenate([main, rest], axis=1)

        return project, scores, mix, output

    def swiglu(gate, up):
        half_gate = 0.5 * gate
        return (half_gate + half_gate * jnp.tanh(half_gate)) * up

    def ffn_stages(src0, src1, dst0, dst1):
        y = jnp.concatenate([ys[pair_rows(src0), :], ys[pair_rows(src1), :]], axis=0)
        h = _layernorm(y)
        top, bot = slice(0, 2 * SEG), slice(2 * SEG, 4 * SEG)
        lhs = _strassen_lhs(h[top, k_lo], h[top, k_hi], h[bot, k_lo], h[bot, k_hi])
        rest = h[:, k_rest].astype(BF16)

        def hidden_tile(half, cols):
            rhs = (up_sums[half, 0, :, cols], w1[half, k_lo, cols], up_sums[half, 1, :, cols],
                   up_sums[half, 2, :, cols], w3[half, k_hi, cols], up_sums[half, 3, :, cols],
                   up_sums[half, 4, :, cols])
            gate_top, up_top, gate_bot, up_bot = _strassen_out(*(dot(a, b) for a, b in zip(lhs, rhs)))
            gate_rest = dot(rest, w1[half, k_rest, cols])
            gate_top, gate_bot = gate_top + gate_rest[top], gate_bot + gate_rest[bot]
            up_rest = dot(rest, w3[half, k_rest, cols])
            g_top = swiglu(gate_top, up_top + up_rest[top])
            g_bot = swiglu(gate_bot, up_bot + up_rest[bot])
            g_scr[top, cols] = g_top.astype(BF16)
            g_scr[bot, cols] = g_bot.astype(BF16)
            return g_top, g_bot

        def hidden(half, f):
            cols = slice(f * LANES, (f + 1) * LANES)
            g11, g21 = hidden_tile(half, cols)
            g12, g22 = hidden_tile(half, slice(f_quarter + f * LANES, f_quarter + (f + 1) * LANES))
            sums = _strassen_lhs(g11, g12, g21, g22)
            for k, i in enumerate((0, 1, 4, 5, 6)):
                g_lhs[k, :, cols] = sums[i]

        def output(half):
            f_lo, f_hi = slice(0, f_quarter), slice(f_quarter, f_half)
            g = (g_lhs[0], g_lhs[1], g_scr[top, f_lo], g_scr[bot, f_hi], g_lhs[2], g_lhs[3], g_lhs[4])
            rhs = (down_sums[half, 0], w2t[half, k_lo, f_lo], down_sums[half, 1], down_sums[half, 2],
                   w2t[half, k_hi, f_hi], down_sums[half, 3], down_sums[half, 4])
            c11, c12, c21, c22 = _strassen_out(*(dot_nt(a, b) for a, b in zip(g, rhs)))
            part = jnp.concatenate(
                [jnp.concatenate([c11, c21], axis=0), jnp.concatenate([c12, c22], axis=0),
                 trailing_features(w2t[half, k_rest, :], g_scr[...])], axis=1)
            return part

        def finish(update):
            z = y + update
            acts[pair_rows(dst0), :] = z[top]
            acts[pair_rows(dst1), :] = z[bot]

        def half_stages(half):
            return ([functools.partial(hidden, half, f) for f in range(f_quarter // LANES)],
                    functools.partial(output, half))

        return half_stages, finish

    def first_ffn():
        y = ys[0:2 * SEG, :]
        h = _layernorm(y).astype(BF16)

        def half_pass(half, z):
            for f in range(f_half // PLAIN_CHUNK):
                cols = slice(f * PLAIN_CHUNK, (f + 1) * PLAIN_CHUNK)
                g_scr[0:2 * SEG, cols] = swiglu(dot(h, w1[half, :, cols]), dot(h, w3[half, :, cols])).astype(BF16)
            g = g_scr[0:2 * SEG, :]
            trailing = trailing_features(w2t[half, k_rest, :], g)
            return z + jnp.concatenate([dot_nt(g, w2t[half, 0:2 * K_BLOCK, :]), trailing], axis=1)

        acts[seq:seq + 2 * SEG, :] = lax.fori_loop(0, 2, half_pass, y)

    def form_weight_sums(i, carry):
        per_half = K_BLOCK // SUM_ROWS
        half = i // per_half
        r0 = pl.multiple_of((i % per_half) * SUM_ROWS, SUM_ROWS)
        lo, hi = pl.ds(r0, SUM_ROWS), pl.ds(r0 + K_BLOCK, SUM_ROWS)
        for c in range(f_half // LANES):
            cols = slice(c * LANES, (c + 1) * LANES)
            blocks = (w1[half, lo, cols], w3[half, lo, cols], w1[half, hi, cols], w3[half, hi, cols])
            for k, b in enumerate(_strassen_rhs_sums(*(b.astype(F32) for b in blocks))):
                up_sums[half, k, lo, cols] = b
        for c in range(f_quarter // LANES):
            cols = slice(c * LANES, (c + 1) * LANES)
            cols_hi = slice(f_quarter + c * LANES, f_quarter + (c + 1) * LANES)
            blocks = (w2t[half, lo, cols], w2t[half, hi, cols], w2t[half, lo, cols_hi], w2t[half, hi, cols_hi])
            for k, b in enumerate(_strassen_rhs_sums(*(b.astype(F32) for b in blocks))):
                down_sums[half, k, lo, cols] = b
        return carry

    def emit(matmul_work, scores, mix):
        for i in range(max(len(matmul_work), n_heads + 2 * STAGE_LAG)):
            if i < len(matmul_work):
                matmul_work[i]()
            if 0 <= i - STAGE_LAG < n_heads:
                scores(i - STAGE_LAG)
            if 0 <= i - 2 * STAGE_LAG < n_heads:
                mix(i - 2 * STAGE_LAG)

    def mixer_only(layer, s, mem):
        x = acts[seg_rows(layer * seq, s), :]
        tail = jnp.concatenate([mem, jnp.zeros_like(mem)], axis=0)
        h = jnp.concatenate([_layernorm(x).astype(BF16), tail.astype(BF16)], axis=0)
        project, scores, mix, output = mixer_stages(h, SEG)
        emit([functools.partial(project, i) for i in range(n_heads)], scores, mix)

        @pl.when(s == 0)
        def _():
            for cp in cp_wo:
                cp.wait()

        att = output()
        ys[seg_rows(layer * seq, s), :] = x + att[0:SEG]
        return att[SEG:SEG + n_mem]

    def stage_tokens(t):
        h_a[0:SEG, :] = _layernorm(acts[seg_rows(0, t), :]).astype(BF16)
        h_a[SEG:2 * SEG, :] = _layernorm(acts[seg_rows(seq, t - LAG), :]).astype(BF16)

    def transpose_out(c):
        rows = pl.ds(pl.multiple_of(2 * seq + c * LANES, LANES), LANES)
        out_v[c] = acts[rows, :].T.astype(out_v.dtype)

    def out_copy(c):
        return pltpu.make_async_copy(out_v.at[c], out_hbm.at[:, pl.ds(pl.multiple_of(c * LANES, LANES), LANES)],
                                     out_sems.at[c])

    cp_x0 = pltpu.make_async_copy(xt_hbm.at[:, 0:LANES], xt_v.at[:, 0:LANES], sems.at[8])
    cp_x = pltpu.make_async_copy(xt_hbm.at[:, LANES:], xt_v.at[:, LANES:], sems.at[0])
    part_rows = d_model // QKV_PARTS
    cp_qkv = [pltpu.make_async_copy(w.at[pl.ds(p * part_rows * n_heads, part_rows * n_heads)],
                                    stage.at[i * QKV_PARTS + p], qkv_sems.at[i * QKV_PARTS + p])
              for i, w in enumerate((wq_hbm, wk_hbm, wv_hbm)) for p in range(QKV_PARTS)]
    cp_wo = [pltpu.make_async_copy(wot_hbm.at[i], wot.at[:, pl.ds(i * d_head, d_head)], sems.at[4])
             for i in range(n_heads)]
    cp_ff = [pltpu.make_async_copy(src.at[:, pl.ds(half * f_half, f_half)], dst.at[half], sems.at[5])
             for src, dst in ((w1_hbm, w1), (w3_hbm, w3), (w2t_hbm, w2t)) for half in range(2)]

    def transpose_in(c, carry):
        chunk = pl.ds(pl.multiple_of(c * LANES, LANES), LANES)
        acts[chunk, :] = xt_v[:, chunk].astype(F32).T
        return carry

    cp_x0.start()
    cp_qkv[0].start()
    cp_qkv[1].start()
    cp_x0.wait()
    acts[0:LANES, :] = xt_v[:, 0:LANES].astype(F32).T
    acts[2 * seq:2 * seq + LANES, :] = jnp.zeros((LANES, d_model), F32)

    pairs = n_heads // 2

    def split_heads(n, b, carry):
        i, p = n // QKV_PARTS, n % QKV_PARTS
        first = pl.multiple_of(b * SPLIT_ROWS * pairs, SPLIT_ROWS * pairs)
        block = stage.at[n].bitcast(jnp.uint32).at[pl.ds(first, SPLIT_ROWS * pairs)]
        features = pl.ds(pl.multiple_of(p * part_rows + b * SPLIT_ROWS, SPLIT_ROWS), SPLIT_ROWS)
        for j in range(pairs):
            w = block[pl.ds(j, SPLIT_ROWS, stride=pairs), :]
            even = pl.ds(pl.multiple_of((2 * j * 3 + i) * d_head, d_head), d_head)
            odd = pl.ds(pl.multiple_of(((2 * j + 1) * 3 + i) * d_head, d_head), d_head)
            wqkv[features, even] = pltpu.bitcast(w << 16, F32).astype(BF16)
            wqkv[features, odd] = pltpu.bitcast(w & jnp.uint32(0xFFFF0000), F32).astype(BF16)
        return carry

    def split_part(n, carry):
        pltpu.make_async_copy(stage.at[n], stage.at[n], qkv_sems.at[n]).wait()
        for m in range(2, len(cp_qkv)):
            pl.when(n + 2 == m)(cp_qkv[m].start)

        @pl.when(n + 2 == len(cp_qkv))
        def _():
            for cp in cp_wo:
                cp.start()

        return lax.fori_loop(0, part_rows // SPLIT_ROWS, functools.partial(split_heads, n), carry)

    lax.fori_loop(0, len(cp_qkv), split_part, 0)
    for cp in cp_ff:
        cp.start()

    def step_pair(i, carry):
        t0 = 2 * i
        src0 = (t0 - 2) * SEG
        lagged = (t0 - LAG - 2) * SEG
        ready = lagged >= 0
        half_stages, finish = ffn_stages(
            src0, jnp.where(ready, seq + lagged, 0), seq + src0, jnp.where(ready, 2 * seq + lagged, 3 * seq))
        for half in range(2):
            t = t0 + half
            hidden, ffn_output = half_stages(half)
            project, scores, mix, mixer_output = mixer_stages(h_a[...], 2 * SEG)
            emit([functools.partial(project, i) for i in range(n_heads)] + hidden, scores, mix)
            if half == 0:
                transpose_out(jnp.maximum(t - out_delay, 0) // segs_per_chunk)
                acc[...] = ffn_output()
            else:
                finish(acc[...] + ffn_output())
            stage_tokens(jnp.minimum(t + 1, n_seg - 1))
            att = mixer_output()
            h_a[2 * SEG:, :] = att[2 * SEG:].astype(BF16)
            ys[seg_rows(0, t), :] = acts[seg_rows(0, t), :] + att[0:SEG]
            ys[seg_rows(seq, t - LAG), :] = acts[seg_rows(seq, t - LAG), :] + att[SEG:2 * SEG]
        return carry

    out_delay = LAG + 2 + segs_per_chunk
    done = (n_seg - 2 - out_delay) // segs_per_chunk + 1
    mem0 = mem0_ref[...].astype(F32)
    h_a[2 * SEG:, :] = jnp.concatenate([mem0, mem0], axis=0).astype(BF16)

    def schedule_round(layer, carry):
        first = layer * (n_seg - LAG)
        mem = h_a[2 * SEG:, :].astype(F32)[n_mem:]
        mem = lax.fori_loop(first, first + LAG, functools.partial(mixer_only, layer), mem)

        @pl.when(layer == 0)
        def _():
            for cp in cp_ff:
                cp.wait()
            cp_x.start()
            lax.fori_loop(0, 2 * K_BLOCK // SUM_ROWS, form_weight_sums, 0)
            first_ffn()
            cp_x.wait()
            lax.fori_loop(1, n_chunks, transpose_in, 0, unroll=3)
            stage_tokens(LAG)
            h_a[2 * SEG:, :] = jnp.concatenate([mem, mem0], axis=0).astype(BF16)
            lax.fori_loop(LAG // 2, n_seg // 2, step_pair, 0)
            for c in range(done):
                out_copy(c).start()

        src0 = jnp.where(layer == 0, (n_seg - 2) * SEG, seq + (n_seg - 4) * SEG)
        src1 = jnp.where(layer == 0, seq + (n_seg - LAG - 2) * SEG, seq + (n_seg - 2) * SEG)

        def ffn_half(half, inner):
            half_stages, finish = ffn_stages(src0, src1, seq + src0, seq + src1)
            hidden, output = half_stages(half)
            for work in hidden:
                work()
            total = output() + jnp.where(half == 1, acc[...], 0.0)
            acc[...] = total
            finish(total)
            return inner

        lax.fori_loop(0, 2, ffn_half, 0)
        transpose_out(done + layer)
        out_copy(done + layer).start()
        return carry

    lax.fori_loop(0, 2, schedule_round, 0)
    for c in range(n_chunks):
        out_copy(c).wait()


@jax.jit
def pallas_interleave_layers__memory_aug_recurrent_mem_tr__glu_gated_swiglu__prompt_kernel(
    A_x, A_mem0, A_Wq, A_Wk, A_Wv, A_Wo, A_seg_len, B_x, B_w1, B_w3, B_w2,
):
    del A_seg_len, B_x
    batch, seq, d_model = A_x.shape
    _, n_heads, d_head = A_Wq.shape
    n_mem = A_mem0.shape[1]
    d_ff = B_w1.shape[1]
    assert batch == 1 and seq % 128 == 0 and d_ff % (4 * LANES) == 0
    rows = 2 * SEG + 2 * n_mem

    def kernel(*refs):
        _kernel(*refs, n_heads=n_heads, d_head=d_head, n_mem=n_mem)

    hbm = pl.BlockSpec(memory_space=pl.ANY)
    vmem = pl.BlockSpec(memory_space=pltpu.VMEM)
    out_t = pl.pallas_call(
        kernel,
        out_shape=jax.ShapeDtypeStruct((d_model, seq), A_x.dtype),
        in_specs=[hbm, vmem, hbm, hbm, hbm, hbm, hbm, hbm, hbm],
        out_specs=hbm,
        scratch_shapes=[
            pltpu.VMEM((d_model, seq), BF16),
            pltpu.VMEM((3 * QKV_PARTS, d_model * n_heads // QKV_PARTS, d_head), BF16),
            pltpu.VMEM((d_model, 3 * n_heads * d_head), BF16),
            pltpu.VMEM((d_model, n_heads * d_head), BF16),
            pltpu.VMEM((2, d_model, d_ff // 2), BF16),
            pltpu.VMEM((2, d_model, d_ff // 2), BF16),
            pltpu.VMEM((2, d_model, d_ff // 2), BF16),
            pltpu.VMEM((2, 5, K_BLOCK, d_ff // 2), BF16),
            pltpu.VMEM((2, 5, K_BLOCK, d_ff // 4), BF16),
            pltpu.VMEM((3 * seq + 2 * SEG, d_model), F32),
            pltpu.VMEM((2 * seq, d_model), F32),
            pltpu.VMEM((rows, d_model), BF16),
            pltpu.VMEM((rows, 3 * n_heads * d_head), BF16),
            pltpu.VMEM((n_heads, rows, rows), BF16),
            pltpu.VMEM((rows, n_heads * d_head), BF16),
            pltpu.VMEM((4 * SEG, d_ff // 2), BF16),
            pltpu.VMEM((5, 2 * SEG, d_ff // 4), BF16),
            pltpu.VMEM((4 * SEG, d_model), F32),
            pltpu.VMEM((seq // LANES, d_model, LANES), A_x.dtype),
            pltpu.SemaphoreType.DMA((9,)),
            pltpu.SemaphoreType.DMA((3 * QKV_PARTS,)),
            pltpu.SemaphoreType.DMA((seq // LANES,)),
        ],
        compiler_params=pltpu.CompilerParams(vmem_limit_bytes=126 * 1024 * 1024),
    )(
        A_x[0].T,
        A_mem0[0],
        A_Wq.reshape(d_model * n_heads, d_head),
        A_Wk.reshape(d_model * n_heads, d_head),
        A_Wv.reshape(d_model * n_heads, d_head),
        jnp.transpose(A_Wo, (0, 2, 1)),
        B_w1,
        B_w3,
        B_w2.T,
    )
    return out_t.T[None]
```

```python
import functools

import jax
import jax.numpy as jnp
from jax import lax
import jax.experimental.pallas as pl
import jax.experimental.pallas.tpu as pltpu

SEG = 32
EPS = 1e-5
MASK_FILL = -1000000000.0
LANES = 128
LAG = 4
SPLIT_ROWS = 48
QKV_PARTS = 4
K_BLOCK = 256
PLAIN_CHUNK = 256
SUM_ROWS = 32
STAGE_LAG = 5
BF16 = jnp.bfloat16
F32 = jnp.float32
NT_DIMS = (((1,), (1,)), ((), ()))


def _layernorm(x):
    inv_n = 1.0 / x.shape[-1]
    c = x - jnp.sum(x, axis=-1, keepdims=True) * inv_n
    v = jnp.sum(c * c, axis=-1, keepdims=True) * inv_n
    return c * lax.rsqrt(v + EPS)


def _strassen_lhs(a11, a12, a21, a22):
    return [a.astype(BF16) for a in (a11 + a22, a21 + a22, a11, a22, a11 + a12, a21 - a11, a12 - a22)]


def _strassen_rhs_sums(*blocks):
    words = [pltpu.bitcast(b, jnp.uint32) for b in blocks]
    halves = []
    for index in range(2):
        b11, b12, b21, b22 = (
            pltpu.unpack_elementwise(w, index=index, packed_dtype=BF16, unpacked_dtype=F32) for w in words)
        halves.append((b11 + b22, b12 - b22, b21 - b11, b11 + b12, b21 + b22))
    return [pltpu.pack_elementwise(list(pair), packed_dtype=BF16) for pair in zip(*halves)]


def _strassen_out(m1, m2, m3, m4, m5, m6, m7):
    return m1 + m4 - m5 + m7, m3 + m5, m2 + m4, m1 - m2 + m3 + m6


def _attention_mask(n_x, n_mem):
    rows = n_x + 2 * n_mem
    r = lax.broadcasted_iota(jnp.int32, (rows, rows), 0)
    c = lax.broadcasted_iota(jnp.int32, (rows, rows), 1)
    r_mem, c_mem = r >= n_x, c >= n_x
    r_stream = jnp.where(r_mem, (r - n_x) // n_mem, r // SEG)
    c_stream = jnp.where(c_mem, (c - n_x) // n_mem, c // SEG)
    same = r_stream == c_stream
    visible = same & (r_mem | c_mem | (c <= r))
    fill = jnp.where(same, MASK_FILL, -jnp.inf).astype(F32)
    return visible, fill


def _kernel(xt_hbm, mem0_ref, wq_hbm, wk_hbm, wv_hbm, wot_hbm, w1_hbm, w3_hbm, w2t_hbm,
            out_hbm,
            xt_v, stage, wqkv, wot, w1, w3, w2t, up_sums, down_sums,
            acts, ys, h_a, qkv_scr, p_scr, o_scr, g_scr, g_lhs, acc, out_v, sems, qkv_sems, out_sems,
            *, n_heads, d_head, n_mem):
    d_model, seq = xt_hbm.shape
    n_seg = seq // SEG
    n_chunks = seq // LANES
    segs_per_chunk = LANES // SEG
    f_half = w1.shape[2]
    f_quarter = f_half // 2
    k_lo, k_hi, k_rest = slice(0, K_BLOCK), slice(K_BLOCK, 2 * K_BLOCK), slice(2 * K_BLOCK, d_model)
    scale = d_head ** -0.5

    def seg_rows(base, s):
        return pl.ds(pl.multiple_of(base + s * SEG, SEG), SEG)

    def dot(a, b):
        return jnp.dot(a, b, preferred_element_type=F32)

    def dot_nt(a, b):
        return lax.dot_general(a, b, NT_DIMS, preferred_element_type=F32)

    def trailing_features(w_t, act):
        n, rows = w_t.shape[0], act.shape[0]
        out_t = dot_nt(w_t, act)
        if rows < LANES:
            out_t = jnp.concatenate([out_t, jnp.zeros((n, LANES - rows), F32)], axis=1)
        out_t = jnp.concatenate([out_t, jnp.zeros((LANES - n, LANES), F32)], axis=0)
        return out_t.T[:rows, :n]

    def pair_rows(start):
        return pl.ds(pl.multiple_of(start, 2 * SEG), 2 * SEG)

    def mixer_stages(h, n_x):
        rows = n_x + 2 * n_mem
        visible, fill = _attention_mask(n_x, n_mem)

        def project(i):
            cols = slice(3 * i * d_head, 3 * (i + 1) * d_head)
            qkv_scr[0:rows, cols] = jnp.dot(h, wqkv[:, cols], preferred_element_type=F32).astype(BF16)

        def scores(i):
            q = qkv_scr[0:rows, 3 * i * d_head:(3 * i + 1) * d_head]
            k = qkv_scr[0:rows, (3 * i + 1) * d_head:(3 * i + 2) * d_head]
            s = lax.dot_general(q, k, NT_DIMS, preferred_element_type=F32) * scale
            s = jnp.where(visible, s, fill)
            e = jnp.exp(s - jnp.max(s, axis=-1, keepdims=True))
            p = e * (1.0 / jnp.sum(e, axis=-1, keepdims=True))
            p_scr[i, 0:rows, 0:rows] = p.astype(BF16)

        def mix(i):
            v = qkv_scr[0:rows, (3 * i + 2) * d_head:(3 * i + 3) * d_head]
            o = jnp.dot(p_scr[i, 0:rows, 0:rows], v, preferred_element_type=F32)
            o_scr[0:rows, i * d_head:(i + 1) * d_head] = o.astype(BF16)

        def output():
            rest = trailing_features(wot[k_rest, :], o_scr[0:rows, :])
            main = dot_nt(o_scr[0:rows, :], wot[0:2 * K_BLOCK, :])
            return jnp.concatenate([main, rest], axis=1)

        return project, scores, mix, output

    def swiglu(gate, up):
        half_gate = 0.5 * gate
        return (half_gate + half_gate * jnp.tanh(half_gate)) * up

    def ffn_stages(src0, src1, dst0, dst1):
        y = jnp.concatenate([ys[pair_rows(src0), :], ys[pair_rows(src1), :]], axis=0)
        h = _layernorm(y)
        top, bot = slice(0, 2 * SEG), slice(2 * SEG, 4 * SEG)
        lhs = _strassen_lhs(h[top, k_lo], h[top, k_hi], h[bot, k_lo], h[bot, k_hi])
        rest = h[:, k_rest].astype(BF16)

        def hidden_tile(half, cols):
            rhs = (pltpu.bitcast(up_sums[half, 0, :, cols], BF16), w1[half, k_lo, cols], pltpu.bitcast(up_sums[half, 1, :, cols], BF16),
                   pltpu.bitcast(up_sums[half, 2, :, cols], BF16), w3[half, k_hi, cols], pltpu.bitcast(up_sums[half, 3, :, cols], BF16),
                   pltpu.bitcast(up_sums[half, 4, :, cols], BF16))
            gate_top, up_top, gate_bot, up_bot = _strassen_out(*(dot(a, b) for a, b in zip(lhs, rhs)))
            gate_rest = dot(rest, w1[half, k_rest, cols])
            gate_top, gate_bot = gate_top + gate_rest[top], gate_bot + gate_rest[bot]
            up_rest = dot(rest, w3[half, k_rest, cols])
            g_top = swiglu(gate_top, up_top + up_rest[top])
            g_bot = swiglu(gate_bot, up_bot + up_rest[bot])
            g_scr[top, cols] = g_top.astype(BF16)
            g_scr[bot, cols] = g_bot.astype(BF16)
            return g_top, g_bot

        def hidden(half, f):
            cols = slice(f * LANES, (f + 1) * LANES)
            g11, g21 = hidden_tile(half, cols)
            g12, g22 = hidden_tile(half, slice(f_quarter + f * LANES, f_quarter + (f + 1) * LANES))
            sums = _strassen_lhs(g11, g12, g21, g22)
            for k, i in enumerate((0, 1, 4, 5, 6)):
                g_lhs[k, :, cols] = sums[i]

        def output(half):
            f_lo, f_hi = slice(0, f_quarter), slice(f_quarter, f_half)
            g = (g_lhs[0], g_lhs[1], g_scr[top, f_lo], g_scr[bot, f_hi], g_lhs[2], g_lhs[3], g_lhs[4])
            rhs = (pltpu.bitcast(down_sums[half, 0], BF16), w2t[half, k_lo, f_lo], pltpu.bitcast(down_sums[half, 1], BF16), pltpu.bitcast(down_sums[half, 2], BF16),
                   w2t[half, k_hi, f_hi], pltpu.bitcast(down_sums[half, 3], BF16), pltpu.bitcast(down_sums[half, 4], BF16))
            c11, c12, c21, c22 = _strassen_out(*(dot_nt(a, b) for a, b in zip(g, rhs)))
            part = jnp.concatenate(
                [jnp.concatenate([c11, c21], axis=0), jnp.concatenate([c12, c22], axis=0),
                 trailing_features(w2t[half, k_rest, :], g_scr[...])], axis=1)
            return part

        def finish(update):
            z = y + update
            acts[pair_rows(dst0), :] = z[top]
            acts[pair_rows(dst1), :] = z[bot]

        def half_stages(half):
            return ([functools.partial(hidden, half, f) for f in range(f_quarter // LANES)],
                    functools.partial(output, half))

        return half_stages, finish

    def first_ffn():
        y = ys[0:2 * SEG, :]
        h = _layernorm(y).astype(BF16)

        def half_pass(half, z):
            for f in range(f_half // PLAIN_CHUNK):
                cols = slice(f * PLAIN_CHUNK, (f + 1) * PLAIN_CHUNK)
                g_scr[0:2 * SEG, cols] = swiglu(dot(h, w1[half, :, cols]), dot(h, w3[half, :, cols])).astype(BF16)
            g = g_scr[0:2 * SEG, :]
            trailing = trailing_features(w2t[half, k_rest, :], g)
            return z + jnp.concatenate([dot_nt(g, w2t[half, 0:2 * K_BLOCK, :]), trailing], axis=1)

        acts[seq:seq + 2 * SEG, :] = lax.fori_loop(0, 2, half_pass, y)

    def form_weight_sums(i, carry):
        per_half = K_BLOCK // SUM_ROWS
        half = i // per_half
        r0 = pl.multiple_of((i % per_half) * SUM_ROWS, SUM_ROWS)
        lo, hi = pl.ds(r0, SUM_ROWS), pl.ds(r0 + K_BLOCK, SUM_ROWS)
        packed = pl.ds(pl.multiple_of(r0 // 2, SUM_ROWS // 2), SUM_ROWS // 2)
        for c in range(f_half // LANES):
            cols = slice(c * LANES, (c + 1) * LANES)
            blocks = (w1[half, lo, cols], w3[half, lo, cols], w1[half, hi, cols], w3[half, hi, cols])
            for k, b in enumerate(_strassen_rhs_sums(*blocks)):
                up_sums[half, k, packed, cols] = b
        for c in range(f_quarter // LANES):
            cols = slice(c * LANES, (c + 1) * LANES)
            cols_hi = slice(f_quarter + c * LANES, f_quarter + (c + 1) * LANES)
            blocks = (w2t[half, lo, cols], w2t[half, hi, cols], w2t[half, lo, cols_hi], w2t[half, hi, cols_hi])
            for k, b in enumerate(_strassen_rhs_sums(*blocks)):
                down_sums[half, k, packed, cols] = b
        return carry

    def emit(matmul_work, scores, mix):
        for i in range(max(len(matmul_work), n_heads + 2 * STAGE_LAG)):
            if i < len(matmul_work):
                matmul_work[i]()
            if 0 <= i - STAGE_LAG < n_heads:
                scores(i - STAGE_LAG)
            if 0 <= i - 2 * STAGE_LAG < n_heads:
                mix(i - 2 * STAGE_LAG)

    def mixer_only(layer, s, mem):
        x = acts[seg_rows(layer * seq, s), :]
        tail = jnp.concatenate([mem, jnp.zeros_like(mem)], axis=0)
        h = jnp.concatenate([_layernorm(x).astype(BF16), tail.astype(BF16)], axis=0)
        project, scores, mix, output = mixer_stages(h, SEG)
        emit([functools.partial(project, i) for i in range(n_heads)], scores, mix)

        @pl.when(s == 0)
        def _():
            for cp in cp_wo:
                cp.wait()

        att = output()
        ys[seg_rows(layer * seq, s), :] = x + att[0:SEG]
        return att[SEG:SEG + n_mem]

    def stage_tokens(t):
        h_a[0:SEG, :] = _layernorm(acts[seg_rows(0, t), :]).astype(BF16)
        h_a[SEG:2 * SEG, :] = _layernorm(acts[seg_rows(seq, t - LAG), :]).astype(BF16)

    def transpose_out(c):
        rows = pl.ds(pl.multiple_of(2 * seq + c * LANES, LANES), LANES)
        out_v[c] = acts[rows, :].T.astype(out_v.dtype)

    def out_copy(c):
        return pltpu.make_async_copy(out_v.at[c], out_hbm.at[:, pl.ds(pl.multiple_of(c * LANES, LANES), LANES)],
                                     out_sems.at[c])

    cp_x0 = pltpu.make_async_copy(xt_hbm.at[:, 0:LANES], xt_v.at[:, 0:LANES], sems.at[8])
    cp_x = pltpu.make_async_copy(xt_hbm.at[:, LANES:], xt_v.at[:, LANES:], sems.at[0])
    part_rows = d_model // QKV_PARTS
    cp_qkv = [pltpu.make_async_copy(w.at[pl.ds(p * part_rows * n_heads, part_rows * n_heads)],
                                    stage.at[i * QKV_PARTS + p], qkv_sems.at[i * QKV_PARTS + p])
              for i, w in enumerate((wq_hbm, wk_hbm, wv_hbm)) for p in range(QKV_PARTS)]
    cp_wo = [pltpu.make_async_copy(wot_hbm.at[i], wot.at[:, pl.ds(i * d_head, d_head)], sems.at[4])
             for i in range(n_heads)]
    cp_ff = [pltpu.make_async_copy(src.at[:, pl.ds(half * f_half, f_half)], dst.at[half], sems.at[5])
             for src, dst in ((w1_hbm, w1), (w3_hbm, w3), (w2t_hbm, w2t)) for half in range(2)]

    def transpose_in(c, carry):
        chunk = pl.ds(pl.multiple_of(c * LANES, LANES), LANES)
        acts[chunk, :] = xt_v[:, chunk].astype(F32).T
        return carry

    cp_x0.start()
    cp_qkv[0].start()
    cp_qkv[1].start()
    cp_x0.wait()
    acts[0:LANES, :] = xt_v[:, 0:LANES].astype(F32).T
    acts[2 * seq:2 * seq + LANES, :] = jnp.zeros((LANES, d_model), F32)

    pairs = n_heads // 2

    def split_heads(n, b, carry):
        i, p = n // QKV_PARTS, n % QKV_PARTS
        first = pl.multiple_of(b * SPLIT_ROWS * pairs, SPLIT_ROWS * pairs)
        block = stage.at[n].bitcast(jnp.uint32).at[pl.ds(first, SPLIT_ROWS * pairs)]
        features = pl.ds(pl.multiple_of(p * part_rows + b * SPLIT_ROWS, SPLIT_ROWS), SPLIT_ROWS)
        for j in range(pairs):
            w = block[pl.ds(j, SPLIT_ROWS, stride=pairs), :]
            even = pl.ds(pl.multiple_of((2 * j * 3 + i) * d_head, d_head), d_head)
            odd = pl.ds(pl.multiple_of(((2 * j + 1) * 3 + i) * d_head, d_head), d_head)
            wqkv[features, even] = pltpu.bitcast(w << 16, F32).astype(BF16)
            wqkv[features, odd] = pltpu.bitcast(w & jnp.uint32(0xFFFF0000), F32).astype(BF16)
        return carry

    def split_part(n, carry):
        pltpu.make_async_copy(stage.at[n], stage.at[n], qkv_sems.at[n]).wait()
        for m in range(2, len(cp_qkv)):
            pl.when(n + 2 == m)(cp_qkv[m].start)

        @pl.when(n + 2 == len(cp_qkv))
        def _():
            for cp in cp_wo:
                cp.start()

        return lax.fori_loop(0, part_rows // SPLIT_ROWS, functools.partial(split_heads, n), carry)

    lax.fori_loop(0, len(cp_qkv), split_part, 0)
    for cp in cp_ff:
        cp.start()

    def step_pair(i, carry):
        t0 = 2 * i
        src0 = (t0 - 2) * SEG
        lagged = (t0 - LAG - 2) * SEG
        ready = lagged >= 0
        half_stages, finish = ffn_stages(
            src0, jnp.where(ready, seq + lagged, 0), seq + src0, jnp.where(ready, 2 * seq + lagged, 3 * seq))
        for half in range(2):
            t = t0 + half
            hidden, ffn_output = half_stages(half)
            project, scores, mix, mixer_output = mixer_stages(h_a[...], 2 * SEG)
            emit([functools.partial(project, i) for i in range(n_heads)] + hidden, scores, mix)
            if half == 0:
                transpose_out(jnp.maximum(t - out_delay, 0) // segs_per_chunk)
                acc[...] = ffn_output()
            else:
                finish(acc[...] + ffn_output())
            stage_tokens(jnp.minimum(t + 1, n_seg - 1))
            att = mixer_output()
            h_a[2 * SEG:, :] = att[2 * SEG:].astype(BF16)
            ys[seg_rows(0, t), :] = acts[seg_rows(0, t), :] + att[0:SEG]
            ys[seg_rows(seq, t - LAG), :] = acts[seg_rows(seq, t - LAG), :] + att[SEG:2 * SEG]
        return carry

    out_delay = LAG + 2 + segs_per_chunk
    done = (n_seg - 2 - out_delay) // segs_per_chunk + 1
    mem0 = mem0_ref[...].astype(F32)
    h_a[2 * SEG:, :] = jnp.concatenate([mem0, mem0], axis=0).astype(BF16)

    def schedule_round(layer, carry):
        first = layer * (n_seg - LAG)
        mem = h_a[2 * SEG:, :].astype(F32)[n_mem:]
        mem = lax.fori_loop(first, first + LAG, functools.partial(mixer_only, layer), mem)

        @pl.when(layer == 0)
        def _():
            for cp in cp_ff:
                cp.wait()
            cp_x.start()
            lax.fori_loop(0, 2 * K_BLOCK // SUM_ROWS, form_weight_sums, 0)
            first_ffn()
            cp_x.wait()
            lax.fori_loop(1, n_chunks, transpose_in, 0, unroll=3)
            stage_tokens(LAG)
            h_a[2 * SEG:, :] = jnp.concatenate([mem, mem0], axis=0).astype(BF16)
            lax.fori_loop(LAG // 2, n_seg // 2, step_pair, 0)
            for c in range(done):
                out_copy(c).start()

        src0 = jnp.where(layer == 0, (n_seg - 2) * SEG, seq + (n_seg - 4) * SEG)
        src1 = jnp.where(layer == 0, seq + (n_seg - LAG - 2) * SEG, seq + (n_seg - 2) * SEG)

        def ffn_half(half, inner):
            half_stages, finish = ffn_stages(src0, src1, seq + src0, seq + src1)
            hidden, output = half_stages(half)
            for work in hidden:
                work()
            total = output() + jnp.where(half == 1, acc[...], 0.0)
            acc[...] = total
            finish(total)
            return inner

        lax.fori_loop(0, 2, ffn_half, 0)
        transpose_out(done + layer)
        out_copy(done + layer).start()
        return carry

    lax.fori_loop(0, 2, schedule_round, 0)
    for c in range(n_chunks):
        out_copy(c).wait()


@jax.jit
def pallas_interleave_layers__memory_aug_recurrent_mem_tr__glu_gated_swiglu__prompt_kernel(
    A_x, A_mem0, A_Wq, A_Wk, A_Wv, A_Wo, A_seg_len, B_x, B_w1, B_w3, B_w2,
):
    del A_seg_len, B_x
    batch, seq, d_model = A_x.shape
    _, n_heads, d_head = A_Wq.shape
    n_mem = A_mem0.shape[1]
    d_ff = B_w1.shape[1]
    assert batch == 1 and seq % 128 == 0 and d_ff % (4 * LANES) == 0
    rows = 2 * SEG + 2 * n_mem

    def kernel(*refs):
        _kernel(*refs, n_heads=n_heads, d_head=d_head, n_mem=n_mem)

    hbm = pl.BlockSpec(memory_space=pl.ANY)
    vmem = pl.BlockSpec(memory_space=pltpu.VMEM)
    out_t = pl.pallas_call(
        kernel,
        out_shape=jax.ShapeDtypeStruct((d_model, seq), A_x.dtype),
        in_specs=[hbm, vmem, hbm, hbm, hbm, hbm, hbm, hbm, hbm],
        out_specs=hbm,
        scratch_shapes=[
            pltpu.VMEM((d_model, seq), BF16),
            pltpu.VMEM((3 * QKV_PARTS, d_model * n_heads // QKV_PARTS, d_head), BF16),
            pltpu.VMEM((d_model, 3 * n_heads * d_head), BF16),
            pltpu.VMEM((d_model, n_heads * d_head), BF16),
            pltpu.VMEM((2, d_model, d_ff // 2), BF16),
            pltpu.VMEM((2, d_model, d_ff // 2), BF16),
            pltpu.VMEM((2, d_model, d_ff // 2), BF16),
            pltpu.VMEM((2, 5, K_BLOCK // 2, d_ff // 2), jnp.uint32),
            pltpu.VMEM((2, 5, K_BLOCK // 2, d_ff // 4), jnp.uint32),
            pltpu.VMEM((3 * seq + 2 * SEG, d_model), F32),
            pltpu.VMEM((2 * seq, d_model), F32),
            pltpu.VMEM((rows, d_model), BF16),
            pltpu.VMEM((rows, 3 * n_heads * d_head), BF16),
            pltpu.VMEM((n_heads, rows, rows), BF16),
            pltpu.VMEM((rows, n_heads * d_head), BF16),
            pltpu.VMEM((4 * SEG, d_ff // 2), BF16),
            pltpu.VMEM((5, 2 * SEG, d_ff // 4), BF16),
            pltpu.VMEM((4 * SEG, d_model), F32),
            pltpu.VMEM((seq // LANES, d_model, LANES), A_x.dtype),
            pltpu.SemaphoreType.DMA((9,)),
            pltpu.SemaphoreType.DMA((3 * QKV_PARTS,)),
            pltpu.SemaphoreType.DMA((seq // LANES,)),
        ],
        compiler_params=pltpu.CompilerParams(vmem_limit_bytes=126 * 1024 * 1024),
    )(
        A_x[0].T,
        A_mem0[0],
        A_Wq.reshape(d_model * n_heads, d_head),
        A_Wk.reshape(d_model * n_heads, d_head),
        A_Wv.reshape(d_model * n_heads, d_head),
        jnp.transpose(A_Wo, (0, 2, 1)),
        B_w1,
        B_w3,
        B_w2.T,
    )
    return out_t.T[None]
```

```python
import functools

import jax
import jax.numpy as jnp
from jax import lax
import jax.experimental.pallas as pl
import jax.experimental.pallas.tpu as pltpu

SEG = 32
EPS = 1e-5
MASK_FILL = -1000000000.0
LANES = 128
LAG = 4
SPLIT_ROWS = 48
QKV_PARTS = 4
K_BLOCK = 256
PLAIN_CHUNK = 256
SUM_ROWS = 32
STAGE_LAG = 5
BF16 = jnp.bfloat16
F32 = jnp.float32
NT_DIMS = (((1,), (1,)), ((), ()))


def _layernorm(x):
    inv_n = 1.0 / x.shape[-1]
    c = x - jnp.sum(x, axis=-1, keepdims=True) * inv_n
    v = jnp.sum(c * c, axis=-1, keepdims=True) * inv_n
    return c * lax.rsqrt(v + EPS)


def _strassen_lhs(a11, a12, a21, a22):
    return [a.astype(BF16) for a in (a11 + a22, a21 + a22, a11, a22, a11 + a12, a21 - a11, a12 - a22)]


def _strassen_rhs_sums(*blocks):
    words = [pltpu.bitcast(b, jnp.uint32) for b in blocks]
    halves = []
    for index in range(2):
        b11, b12, b21, b22 = (
            pltpu.unpack_elementwise(w, index=index, packed_dtype=BF16, unpacked_dtype=F32) for w in words)
        halves.append((b11 + b22, b12 - b22, b21 - b11, b11 + b12, b21 + b22))
    return [pltpu.pack_elementwise(list(pair), packed_dtype=BF16) for pair in zip(*halves)]


def _strassen_out(m1, m2, m3, m4, m5, m6, m7):
    return m1 + m4 - m5 + m7, m3 + m5, m2 + m4, m1 - m2 + m3 + m6


def _attention_mask(n_x, n_mem):
    rows = n_x + 2 * n_mem
    r = lax.broadcasted_iota(jnp.int32, (rows, rows), 0)
    c = lax.broadcasted_iota(jnp.int32, (rows, rows), 1)
    r_mem, c_mem = r >= n_x, c >= n_x
    r_stream = jnp.where(r_mem, (r - n_x) // n_mem, r // SEG)
    c_stream = jnp.where(c_mem, (c - n_x) // n_mem, c // SEG)
    same = r_stream == c_stream
    visible = same & (r_mem | c_mem | (c <= r))
    fill = jnp.where(same, MASK_FILL, -jnp.inf).astype(F32)
    return visible, fill


def _kernel(xt_hbm, mem0_ref, wq_hbm, wk_hbm, wv_hbm, wot_hbm, w1_hbm, w3_hbm, w2t_hbm,
            out_hbm,
            xt_v, stage, wqkv, wot, w1, w3, w2t, up_sums, down_sums,
            acts, ys, h_a, g_scr, acc, out_v, sems, qkv_sems, out_sems,
            *, n_heads, d_head, n_mem):
    d_model, seq = xt_hbm.shape
    n_seg = seq // SEG
    n_chunks = seq // LANES
    segs_per_chunk = LANES // SEG
    f_half = w1.shape[2]
    f_quarter = f_half // 2
    k_lo, k_hi, k_rest = slice(0, K_BLOCK), slice(K_BLOCK, 2 * K_BLOCK), slice(2 * K_BLOCK, d_model)
    scale = d_head ** -0.5

    def seg_rows(base, s):
        return pl.ds(pl.multiple_of(base + s * SEG, SEG), SEG)

    def dot(a, b):
        return jnp.dot(a, b, preferred_element_type=F32)

    def dot_nt(a, b):
        return lax.dot_general(a, b, NT_DIMS, preferred_element_type=F32)

    def trailing_features(w_t, act):
        n, rows = w_t.shape[0], act.shape[0]
        out_t = dot_nt(w_t, act)
        if rows < LANES:
            out_t = jnp.concatenate([out_t, jnp.zeros((n, LANES - rows), F32)], axis=1)
        out_t = jnp.concatenate([out_t, jnp.zeros((LANES - n, LANES), F32)], axis=0)
        return out_t.T[:rows, :n]

    def pair_rows(start):
        return pl.ds(pl.multiple_of(start, 2 * SEG), 2 * SEG)

    def mixer_stages(h, n_x):
        rows = n_x + 2 * n_mem
        visible, fill = _attention_mask(n_x, n_mem)

        qkv, probs, mixed = {}, {}, {}

        def project(i):
            qkv[i] = dot(h, wqkv[:, 3 * i * d_head:3 * (i + 1) * d_head]).astype(BF16)

        def scores(i):
            s = dot_nt(qkv[i][:, 0:d_head], qkv[i][:, d_head:2 * d_head]) * scale
            s = jnp.where(visible, s, fill)
            e = jnp.exp(s - jnp.max(s, axis=-1, keepdims=True))
            probs[i] = (e * (1.0 / jnp.sum(e, axis=-1, keepdims=True))).astype(BF16)

        def mix(i):
            mixed[i] = dot(probs[i], qkv[i][:, 2 * d_head:]).astype(BF16)

        def output():
            o = jnp.concatenate([mixed[i] for i in range(n_heads)], axis=1)
            rest = trailing_features(wot[k_rest, :], o)
            return jnp.concatenate([dot_nt(o, wot[0:2 * K_BLOCK, :]), rest], axis=1)

        return project, scores, mix, output

    def swiglu(gate, up):
        half_gate = 0.5 * gate
        return (half_gate + half_gate * jnp.tanh(half_gate)) * up

    def ffn_stages(src0, src1, dst0, dst1):
        y = jnp.concatenate([ys[pair_rows(src0), :], ys[pair_rows(src1), :]], axis=0)
        h = _layernorm(y)
        top, bot = slice(0, 2 * SEG), slice(2 * SEG, 4 * SEG)
        lhs = _strassen_lhs(h[top, k_lo], h[top, k_hi], h[bot, k_lo], h[bot, k_hi])
        rest = h[:, k_rest].astype(BF16)

        tiles = {}

        def hidden_tile(half, cols):
            rhs = (pltpu.bitcast(up_sums[half, 0, :, cols], BF16), w1[half, k_lo, cols], pltpu.bitcast(up_sums[half, 1, :, cols], BF16),
                   pltpu.bitcast(up_sums[half, 2, :, cols], BF16), w3[half, k_hi, cols], pltpu.bitcast(up_sums[half, 3, :, cols], BF16),
                   pltpu.bitcast(up_sums[half, 4, :, cols], BF16))
            gate_top, up_top, gate_bot, up_bot = _strassen_out(*(dot(a, b) for a, b in zip(lhs, rhs)))
            gate_rest = dot(rest, w1[half, k_rest, cols])
            gate_top, gate_bot = gate_top + gate_rest[top], gate_bot + gate_rest[bot]
            up_rest = dot(rest, w3[half, k_rest, cols])
            g_top = swiglu(gate_top, up_top + up_rest[top])
            g_bot = swiglu(gate_bot, up_bot + up_rest[bot])
            return g_top, g_bot

        def hidden(half, f):
            cols = slice(f * LANES, (f + 1) * LANES)
            g11, g21 = hidden_tile(half, cols)
            g12, g22 = hidden_tile(half, slice(f_quarter + f * LANES, f_quarter + (f + 1) * LANES))
            tiles[f] = _strassen_lhs(g11, g12, g21, g22) + [g12.astype(BF16), g21.astype(BF16)]

        def output(half):
            f_lo, f_hi = slice(0, f_quarter), slice(f_quarter, f_half)
            g = [jnp.concatenate([tiles[f][k] for f in range(f_quarter // LANES)], axis=1) for k in range(9)]
            plain = jnp.concatenate([jnp.concatenate([g[2], g[7]], axis=1),
                                     jnp.concatenate([g[8], g[3]], axis=1)], axis=0)
            rhs = (pltpu.bitcast(down_sums[half, 0], BF16), w2t[half, k_lo, f_lo], pltpu.bitcast(down_sums[half, 1], BF16), pltpu.bitcast(down_sums[half, 2], BF16),
                   w2t[half, k_hi, f_hi], pltpu.bitcast(down_sums[half, 3], BF16), pltpu.bitcast(down_sums[half, 4], BF16))
            c11, c12, c21, c22 = _strassen_out(*(dot_nt(a, b) for a, b in zip(g, rhs)))
            part = jnp.concatenate(
                [jnp.concatenate([c11, c21], axis=0), jnp.concatenate([c12, c22], axis=0),
                 trailing_features(w2t[half, k_rest, :], plain)], axis=1)
            return part

        def finish(update):
            z = y + update
            acts[pair_rows(dst0), :] = z[top]
            acts[pair_rows(dst1), :] = z[bot]

        def half_stages(half):
            return ([functools.partial(hidden, half, f) for f in range(f_quarter // LANES)],
                    functools.partial(output, half))

        return half_stages, finish

    def first_ffn():
        y = ys[0:2 * SEG, :]
        h = _layernorm(y).astype(BF16)

        def half_pass(half, z):
            for f in range(f_half // PLAIN_CHUNK):
                cols = slice(f * PLAIN_CHUNK, (f + 1) * PLAIN_CHUNK)
                g_scr[0:2 * SEG, cols] = swiglu(dot(h, w1[half, :, cols]), dot(h, w3[half, :, cols])).astype(BF16)
            g = g_scr[0:2 * SEG, :]
            trailing = trailing_features(w2t[half, k_rest, :], g)
            return z + jnp.concatenate([dot_nt(g, w2t[half, 0:2 * K_BLOCK, :]), trailing], axis=1)

        acts[seq:seq + 2 * SEG, :] = lax.fori_loop(0, 2, half_pass, y)

    def form_weight_sums(i, carry):
        per_half = K_BLOCK // SUM_ROWS
        half = i // per_half
        r0 = pl.multiple_of((i % per_half) * SUM_ROWS, SUM_ROWS)
        lo, hi = pl.ds(r0, SUM_ROWS), pl.ds(r0 + K_BLOCK, SUM_ROWS)
        packed = pl.ds(pl.multiple_of(r0 // 2, SUM_ROWS // 2), SUM_ROWS // 2)
        for c in range(f_half // LANES):
            cols = slice(c * LANES, (c + 1) * LANES)
            blocks = (w1[half, lo, cols], w3[half, lo, cols], w1[half, hi, cols], w3[half, hi, cols])
            for k, b in enumerate(_strassen_rhs_sums(*blocks)):
                up_sums[half, k, packed, cols] = b
        for c in range(f_quarter // LANES):
            cols = slice(c * LANES, (c + 1) * LANES)
            cols_hi = slice(f_quarter + c * LANES, f_quarter + (c + 1) * LANES)
            blocks = (w2t[half, lo, cols], w2t[half, hi, cols], w2t[half, lo, cols_hi], w2t[half, hi, cols_hi])
            for k, b in enumerate(_strassen_rhs_sums(*blocks)):
                down_sums[half, k, packed, cols] = b
        return carry

    def emit(matmul_work, scores, mix):
        for i in range(max(len(matmul_work), n_heads + 2 * STAGE_LAG)):
            if i < len(matmul_work):
                matmul_work[i]()
            if 0 <= i - STAGE_LAG < n_heads:
                scores(i - STAGE_LAG)
            if 0 <= i - 2 * STAGE_LAG < n_heads:
                mix(i - 2 * STAGE_LAG)

    def mixer_only(layer, s, mem):
        x = acts[seg_rows(layer * seq, s), :]
        tail = jnp.concatenate([mem, jnp.zeros_like(mem)], axis=0)
        h = jnp.concatenate([_layernorm(x).astype(BF16), tail.astype(BF16)], axis=0)
        project, scores, mix, output = mixer_stages(h, SEG)
        emit([functools.partial(project, i) for i in range(n_heads)], scores, mix)

        @pl.when(s == 0)
        def _():
            for cp in cp_wo:
                cp.wait()

        att = output()
        ys[seg_rows(layer * seq, s), :] = x + att[0:SEG]
        return att[SEG:SEG + n_mem]

    def stage_tokens(t):
        h_a[0:SEG, :] = _layernorm(acts[seg_rows(0, t), :]).astype(BF16)
        h_a[SEG:2 * SEG, :] = _layernorm(acts[seg_rows(seq, t - LAG), :]).astype(BF16)

    def transpose_out(c):
        rows = pl.ds(pl.multiple_of(2 * seq + c * LANES, LANES), LANES)
        out_v[c] = acts[rows, :].T.astype(out_v.dtype)

    def out_copy(c):
        return pltpu.make_async_copy(out_v.at[c], out_hbm.at[:, pl.ds(pl.multiple_of(c * LANES, LANES), LANES)],
                                     out_sems.at[c])

    cp_x0 = pltpu.make_async_copy(xt_hbm.at[:, 0:LANES], xt_v.at[:, 0:LANES], sems.at[8])
    cp_x = pltpu.make_async_copy(xt_hbm.at[:, LANES:], xt_v.at[:, LANES:], sems.at[0])
    part_rows = d_model // QKV_PARTS
    cp_qkv = [pltpu.make_async_copy(w.at[pl.ds(p * part_rows * n_heads, part_rows * n_heads)],
                                    stage.at[i * QKV_PARTS + p], qkv_sems.at[i * QKV_PARTS + p])
              for i, w in enumerate((wq_hbm, wk_hbm, wv_hbm)) for p in range(QKV_PARTS)]
    cp_wo = [pltpu.make_async_copy(wot_hbm.at[i], wot.at[:, pl.ds(i * d_head, d_head)], sems.at[4])
             for i in range(n_heads)]
    cp_ff = [pltpu.make_async_copy(src.at[:, pl.ds(half * f_half, f_half)], dst.at[half], sems.at[5])
             for src, dst in ((w1_hbm, w1), (w3_hbm, w3), (w2t_hbm, w2t)) for half in range(2)]

    def transpose_in(c, carry):
        chunk = pl.ds(pl.multiple_of(c * LANES, LANES), LANES)
        acts[chunk, :] = xt_v[:, chunk].astype(F32).T
        return carry

    cp_x0.start()
    cp_qkv[0].start()
    cp_qkv[1].start()
    cp_x0.wait()
    acts[0:LANES, :] = xt_v[:, 0:LANES].astype(F32).T
    acts[2 * seq:2 * seq + LANES, :] = jnp.zeros((LANES, d_model), F32)

    pairs = n_heads // 2

    def split_heads(n, b, carry):
        i, p = n // QKV_PARTS, n % QKV_PARTS
        first = pl.multiple_of(b * SPLIT_ROWS * pairs, SPLIT_ROWS * pairs)
        block = stage.at[n].bitcast(jnp.uint32).at[pl.ds(first, SPLIT_ROWS * pairs)]
        features = pl.ds(pl.multiple_of(p * part_rows + b * SPLIT_ROWS, SPLIT_ROWS), SPLIT_ROWS)
        for j in range(pairs):
            w = block[pl.ds(j, SPLIT_ROWS, stride=pairs), :]
            even = pl.ds(pl.multiple_of((2 * j * 3 + i) * d_head, d_head), d_head)
            odd = pl.ds(pl.multiple_of(((2 * j + 1) * 3 + i) * d_head, d_head), d_head)
            wqkv[features, even] = pltpu.bitcast(w << 16, F32).astype(BF16)
            wqkv[features, odd] = pltpu.bitcast(w & jnp.uint32(0xFFFF0000), F32).astype(BF16)
        return carry

    def split_part(n, carry):
        pltpu.make_async_copy(stage.at[n], stage.at[n], qkv_sems.at[n]).wait()
        for m in range(2, len(cp_qkv)):
            pl.when(n + 2 == m)(cp_qkv[m].start)

        @pl.when(n + 2 == len(cp_qkv))
        def _():
            for cp in cp_wo:
                cp.start()

        return lax.fori_loop(0, part_rows // SPLIT_ROWS, functools.partial(split_heads, n), carry)

    lax.fori_loop(0, len(cp_qkv), split_part, 0)
    for cp in cp_ff:
        cp.start()

    def step_pair(i, carry):
        t0 = 2 * i
        src0 = (t0 - 2) * SEG
        lagged = (t0 - LAG - 2) * SEG
        ready = lagged >= 0
        half_stages, finish = ffn_stages(
            src0, jnp.where(ready, seq + lagged, 0), seq + src0, jnp.where(ready, 2 * seq + lagged, 3 * seq))
        for half in range(2):
            t = t0 + half
            hidden, ffn_output = half_stages(half)
            project, scores, mix, mixer_output = mixer_stages(h_a[...], 2 * SEG)
            emit([functools.partial(project, i) for i in range(n_heads)] + hidden, scores, mix)
            if half == 0:
                transpose_out(jnp.maximum(t - out_delay, 0) // segs_per_chunk)
                acc[...] = ffn_output()
            else:
                finish(acc[...] + ffn_output())
            stage_tokens(jnp.minimum(t + 1, n_seg - 1))
            att = mixer_output()
            h_a[2 * SEG:, :] = att[2 * SEG:].astype(BF16)
            ys[seg_rows(0, t), :] = acts[seg_rows(0, t), :] + att[0:SEG]
            ys[seg_rows(seq, t - LAG), :] = acts[seg_rows(seq, t - LAG), :] + att[SEG:2 * SEG]
        return carry

    out_delay = LAG + 2 + segs_per_chunk
    done = (n_seg - 2 - out_delay) // segs_per_chunk + 1
    mem0 = mem0_ref[...].astype(F32)
    h_a[2 * SEG:, :] = jnp.concatenate([mem0, mem0], axis=0).astype(BF16)

    def schedule_round(layer, carry):
        first = layer * (n_seg - LAG)
        mem = h_a[2 * SEG:, :].astype(F32)[n_mem:]
        mem = lax.fori_loop(first, first + LAG, functools.partial(mixer_only, layer), mem)

        @pl.when(layer == 0)
        def _():
            for cp in cp_ff:
                cp.wait()
            cp_x.start()
            lax.fori_loop(0, 2 * K_BLOCK // SUM_ROWS, form_weight_sums, 0)
            first_ffn()
            cp_x.wait()
            lax.fori_loop(1, n_chunks, transpose_in, 0, unroll=3)
            stage_tokens(LAG)
            h_a[2 * SEG:, :] = jnp.concatenate([mem, mem0], axis=0).astype(BF16)
            lax.fori_loop(LAG // 2, n_seg // 2, step_pair, 0)
            for c in range(done):
                out_copy(c).start()

        src0 = jnp.where(layer == 0, (n_seg - 2) * SEG, seq + (n_seg - 4) * SEG)
        src1 = jnp.where(layer == 0, seq + (n_seg - LAG - 2) * SEG, seq + (n_seg - 2) * SEG)

        def ffn_half(half, inner):
            half_stages, finish = ffn_stages(src0, src1, seq + src0, seq + src1)
            hidden, output = half_stages(half)
            for work in hidden:
                work()
            total = output() + jnp.where(half == 1, acc[...], 0.0)
            acc[...] = total
            finish(total)
            return inner

        lax.fori_loop(0, 2, ffn_half, 0)
        transpose_out(done + layer)
        out_copy(done + layer).start()
        return carry

    lax.fori_loop(0, 2, schedule_round, 0)
    for c in range(n_chunks):
        out_copy(c).wait()


@jax.jit
def pallas_interleave_layers__memory_aug_recurrent_mem_tr__glu_gated_swiglu__prompt_kernel(
    A_x, A_mem0, A_Wq, A_Wk, A_Wv, A_Wo, A_seg_len, B_x, B_w1, B_w3, B_w2,
):
    del A_seg_len, B_x
    batch, seq, d_model = A_x.shape
    _, n_heads, d_head = A_Wq.shape
    n_mem = A_mem0.shape[1]
    d_ff = B_w1.shape[1]
    assert batch == 1 and seq % 128 == 0 and d_ff % (4 * LANES) == 0
    rows = 2 * SEG + 2 * n_mem

    def kernel(*refs):
        _kernel(*refs, n_heads=n_heads, d_head=d_head, n_mem=n_mem)

    hbm = pl.BlockSpec(memory_space=pl.ANY)
    vmem = pl.BlockSpec(memory_space=pltpu.VMEM)
    out_t = pl.pallas_call(
        kernel,
        out_shape=jax.ShapeDtypeStruct((d_model, seq), A_x.dtype),
        in_specs=[hbm, vmem, hbm, hbm, hbm, hbm, hbm, hbm, hbm],
        out_specs=hbm,
        scratch_shapes=[
            pltpu.VMEM((d_model, seq), BF16),
            pltpu.VMEM((3 * QKV_PARTS, d_model * n_heads // QKV_PARTS, d_head), BF16),
            pltpu.VMEM((d_model, 3 * n_heads * d_head), BF16),
            pltpu.VMEM((d_model, n_heads * d_head), BF16),
            pltpu.VMEM((2, d_model, d_ff // 2), BF16),
            pltpu.VMEM((2, d_model, d_ff // 2), BF16),
            pltpu.VMEM((2, d_model, d_ff // 2), BF16),
            pltpu.VMEM((2, 5, K_BLOCK // 2, d_ff // 2), jnp.uint32),
            pltpu.VMEM((2, 5, K_BLOCK // 2, d_ff // 4), jnp.uint32),
            pltpu.VMEM((3 * seq + 2 * SEG, d_model), F32),
            pltpu.VMEM((2 * seq, d_model), F32),
            pltpu.VMEM((rows, d_model), BF16),
            pltpu.VMEM((4 * SEG, d_ff // 2), BF16),
            pltpu.VMEM((4 * SEG, d_model), F32),
            pltpu.VMEM((seq // LANES, d_model, LANES), A_x.dtype),
            pltpu.SemaphoreType.DMA((9,)),
            pltpu.SemaphoreType.DMA((3 * QKV_PARTS,)),
            pltpu.SemaphoreType.DMA((seq // LANES,)),
        ],
        compiler_params=pltpu.CompilerParams(vmem_limit_bytes=126 * 1024 * 1024),
    )(
        A_x[0].T,
        A_mem0[0],
        A_Wq.reshape(d_model * n_heads, d_head),
        A_Wk.reshape(d_model * n_heads, d_head),
        A_Wv.reshape(d_model * n_heads, d_head),
        jnp.transpose(A_Wo, (0, 2, 1)),
        B_w1,
        B_w3,
        B_w2.T,
    )
    return out_t.T[None]
```

```python
import functools

import jax
import jax.numpy as jnp
from jax import lax
import jax.experimental.pallas as pl
import jax.experimental.pallas.tpu as pltpu

SEG = 32
EPS = 1e-5
MASK_FILL = -1000000000.0
LANES = 128
LAG = 4
SPLIT_ROWS = 48
QKV_PARTS = 4
K_BLOCK = 256
PLAIN_CHUNK = 384
SUM_ROWS = 32
STAGE_LAG = 5
BF16 = jnp.bfloat16
F32 = jnp.float32
NT_DIMS = (((1,), (1,)), ((), ()))


def _layernorm(x):
    inv_n = 1.0 / x.shape[-1]
    c = x - jnp.sum(x, axis=-1, keepdims=True) * inv_n
    v = jnp.sum(c * c, axis=-1, keepdims=True) * inv_n
    return c * lax.rsqrt(v + EPS)


def _strassen_lhs(a11, a12, a21, a22):
    return [a.astype(BF16) for a in (a11 + a22, a21 + a22, a11, a22, a11 + a12, a21 - a11, a12 - a22)]


def _strassen_rhs_sums(*blocks):
    words = [pltpu.bitcast(b, jnp.uint32) for b in blocks]
    halves = []
    for index in range(2):
        b11, b12, b21, b22 = (
            pltpu.unpack_elementwise(w, index=index, packed_dtype=BF16, unpacked_dtype=F32) for w in words)
        halves.append((b11 + b22, b12 - b22, b21 - b11, b11 + b12, b21 + b22))
    return [pltpu.pack_elementwise(list(pair), packed_dtype=BF16) for pair in zip(*halves)]


def _strassen_out(m1, m2, m3, m4, m5, m6, m7):
    return m1 + m4 - m5 + m7, m3 + m5, m2 + m4, m1 - m2 + m3 + m6


def _attention_mask(n_x, n_mem):
    rows = n_x + 2 * n_mem
    r = lax.broadcasted_iota(jnp.int32, (rows, rows), 0)
    c = lax.broadcasted_iota(jnp.int32, (rows, rows), 1)
    r_mem, c_mem = r >= n_x, c >= n_x
    r_stream = jnp.where(r_mem, (r - n_x) // n_mem, r // SEG)
    c_stream = jnp.where(c_mem, (c - n_x) // n_mem, c // SEG)
    same = r_stream == c_stream
    visible = same & (r_mem | c_mem | (c <= r))
    fill = jnp.where(same, MASK_FILL, -jnp.inf).astype(F32)
    return visible, fill


def _kernel(xt_hbm, mem0_ref, wq_hbm, wk_hbm, wv_hbm, wot_hbm, w1_hbm, w3_hbm, w2t_hbm,
            out_hbm,
            xt_v, stage, wqkv, wot, w1, w3, w2t, up_sums, down_sums,
            acts, ys, h_a, acc, out_v, sems, qkv_sems, out_sems,
            *, n_heads, d_head, n_mem):
    d_model, seq = xt_hbm.shape
    n_seg = seq // SEG
    n_chunks = seq // LANES
    segs_per_chunk = LANES // SEG
    f_half = w1.shape[2]
    f_quarter = f_half // 2
    k_lo, k_hi, k_rest = slice(0, K_BLOCK), slice(K_BLOCK, 2 * K_BLOCK), slice(2 * K_BLOCK, d_model)
    scale = d_head ** -0.5

    def seg_rows(base, s):
        return pl.ds(pl.multiple_of(base + s * SEG, SEG), SEG)

    def dot(a, b):
        return jnp.dot(a, b, preferred_element_type=F32)

    def dot_nt(a, b):
        return lax.dot_general(a, b, NT_DIMS, preferred_element_type=F32)

    def trailing_features(w_t, act):
        n, rows = w_t.shape[0], act.shape[0]
        out_t = dot_nt(w_t, act)
        if rows < LANES:
            out_t = jnp.concatenate([out_t, jnp.zeros((n, LANES - rows), F32)], axis=1)
        out_t = jnp.concatenate([out_t, jnp.zeros((LANES - n, LANES), F32)], axis=0)
        return out_t.T[:rows, :n]

    def pair_rows(start):
        return pl.ds(pl.multiple_of(start, 2 * SEG), 2 * SEG)

    def mixer_stages(h, n_x):
        rows = n_x + 2 * n_mem
        visible, fill = _attention_mask(n_x, n_mem)

        qkv, probs, mixed = {}, {}, {}

        def project(i):
            qkv[i] = dot(h, wqkv[:, 3 * i * d_head:3 * (i + 1) * d_head]).astype(BF16)

        def scores(i):
            s = dot_nt(qkv[i][:, 0:d_head], qkv[i][:, d_head:2 * d_head]) * scale
            s = jnp.where(visible, s, fill)
            e = jnp.exp(s - jnp.max(s, axis=-1, keepdims=True))
            probs[i] = (e * (1.0 / jnp.sum(e, axis=-1, keepdims=True))).astype(BF16)

        def mix(i):
            mixed[i] = dot(probs[i], qkv[i][:, 2 * d_head:]).astype(BF16)

        def output():
            o = jnp.concatenate([mixed[i] for i in range(n_heads)], axis=1)
            rest = trailing_features(wot[k_rest, :], o)
            return jnp.concatenate([dot_nt(o, wot[0:2 * K_BLOCK, :]), rest], axis=1)

        return project, scores, mix, output

    def swiglu(gate, up):
        half_gate = 0.5 * gate
        return (half_gate + half_gate * jnp.tanh(half_gate)) * up

    def ffn_stages(src0, src1, dst0, dst1):
        y = jnp.concatenate([ys[pair_rows(src0), :], ys[pair_rows(src1), :]], axis=0)
        h = _layernorm(y)
        top, bot = slice(0, 2 * SEG), slice(2 * SEG, 4 * SEG)
        lhs = _strassen_lhs(h[top, k_lo], h[top, k_hi], h[bot, k_lo], h[bot, k_hi])
        rest = h[:, k_rest].astype(BF16)

        tiles = {}

        def hidden_tile(half, cols):
            rhs = (pltpu.bitcast(up_sums[half, 0, :, cols], BF16), w1[half, k_lo, cols], pltpu.bitcast(up_sums[half, 1, :, cols], BF16),
                   pltpu.bitcast(up_sums[half, 2, :, cols], BF16), w3[half, k_hi, cols], pltpu.bitcast(up_sums[half, 3, :, cols], BF16),
                   pltpu.bitcast(up_sums[half, 4, :, cols], BF16))
            gate_top, up_top, gate_bot, up_bot = _strassen_out(*(dot(a, b) for a, b in zip(lhs, rhs)))
            gate_rest = dot(rest, w1[half, k_rest, cols])
            gate_top, gate_bot = gate_top + gate_rest[top], gate_bot + gate_rest[bot]
            up_rest = dot(rest, w3[half, k_rest, cols])
            g_top = swiglu(gate_top, up_top + up_rest[top])
            g_bot = swiglu(gate_bot, up_bot + up_rest[bot])
            return g_top, g_bot

        def hidden(half, f):
            cols = slice(f * LANES, (f + 1) * LANES)
            g11, g21 = hidden_tile(half, cols)
            g12, g22 = hidden_tile(half, slice(f_quarter + f * LANES, f_quarter + (f + 1) * LANES))
            tiles[f] = _strassen_lhs(g11, g12, g21, g22) + [g12.astype(BF16), g21.astype(BF16)]

        def output(half):
            f_lo, f_hi = slice(0, f_quarter), slice(f_quarter, f_half)
            g = [jnp.concatenate([tiles[f][k] for f in range(f_quarter // LANES)], axis=1) for k in range(9)]
            plain = jnp.concatenate([jnp.concatenate([g[2], g[7]], axis=1),
                                     jnp.concatenate([g[8], g[3]], axis=1)], axis=0)
            rhs = (pltpu.bitcast(down_sums[half, 0], BF16), w2t[half, k_lo, f_lo], pltpu.bitcast(down_sums[half, 1], BF16), pltpu.bitcast(down_sums[half, 2], BF16),
                   w2t[half, k_hi, f_hi], pltpu.bitcast(down_sums[half, 3], BF16), pltpu.bitcast(down_sums[half, 4], BF16))
            c11, c12, c21, c22 = _strassen_out(*(dot_nt(a, b) for a, b in zip(g, rhs)))
            part = jnp.concatenate(
                [jnp.concatenate([c11, c21], axis=0), jnp.concatenate([c12, c22], axis=0),
                 trailing_features(w2t[half, k_rest, :], plain)], axis=1)
            return part

        def finish(update):
            z = y + update
            acts[pair_rows(dst0), :] = z[top]
            acts[pair_rows(dst1), :] = z[bot]

        def half_stages(half):
            return ([functools.partial(hidden, half, f) for f in range(f_quarter // LANES)],
                    functools.partial(output, half))

        return half_stages, finish

    def first_ffn():
        y = ys[0:2 * SEG, :]
        h = _layernorm(y).astype(BF16)

        def quarter_pass(n, z):
            half, first = n // 2, (n % 2) * f_quarter
            g = []
            for f in range(f_quarter // PLAIN_CHUNK):
                cols = pl.ds(pl.multiple_of(first + f * PLAIN_CHUNK, LANES), PLAIN_CHUNK)
                g.append(swiglu(dot(h, w1[half, :, cols]), dot(h, w3[half, :, cols])).astype(BF16))
            g = jnp.concatenate(g, axis=1)
            cols = pl.ds(pl.multiple_of(first, LANES), f_quarter)
            trailing = trailing_features(w2t[half, k_rest, cols], g)
            return z + jnp.concatenate([dot_nt(g, w2t[half, 0:2 * K_BLOCK, cols]), trailing], axis=1)

        acts[seq:seq + 2 * SEG, :] = lax.fori_loop(0, 4, quarter_pass, y)

    def form_weight_sums(i, carry):
        per_half = K_BLOCK // SUM_ROWS
        half = i // per_half
        r0 = pl.multiple_of((i % per_half) * SUM_ROWS, SUM_ROWS)
        lo, hi = pl.ds(r0, SUM_ROWS), pl.ds(r0 + K_BLOCK, SUM_ROWS)
        packed = pl.ds(pl.multiple_of(r0 // 2, SUM_ROWS // 2), SUM_ROWS // 2)
        for c in range(f_half // LANES):
            cols = slice(c * LANES, (c + 1) * LANES)
            blocks = (w1[half, lo, cols], w3[half, lo, cols], w1[half, hi, cols], w3[half, hi, cols])
            for k, b in enumerate(_strassen_rhs_sums(*blocks)):
                up_sums[half, k, packed, cols] = b
        for c in range(f_quarter // LANES):
            cols = slice(c * LANES, (c + 1) * LANES)
            cols_hi = slice(f_quarter + c * LANES, f_quarter + (c + 1) * LANES)
            blocks = (w2t[half, lo, cols], w2t[half, hi, cols], w2t[half, lo, cols_hi], w2t[half, hi, cols_hi])
            for k, b in enumerate(_strassen_rhs_sums(*blocks)):
                down_sums[half, k, packed, cols] = b
        return carry

    def emit(matmul_work, scores, mix):
        for i in range(max(len(matmul_work), n_heads + 2 * STAGE_LAG)):
            if i < len(matmul_work):
                matmul_work[i]()
            if 0 <= i - STAGE_LAG < n_heads:
                scores(i - STAGE_LAG)
            if 0 <= i - 2 * STAGE_LAG < n_heads:
                mix(i - 2 * STAGE_LAG)

    def mixer_only(layer, s, mem):
        x = acts[seg_rows(layer * seq, s), :]
        tail = jnp.concatenate([mem, jnp.zeros_like(mem)], axis=0)
        h = jnp.concatenate([_layernorm(x).astype(BF16), tail.astype(BF16)], axis=0)
        project, scores, mix, output = mixer_stages(h, SEG)
        emit([functools.partial(project, i) for i in range(n_heads)], scores, mix)

        @pl.when(s == 0)
        def _():
            for cp in cp_wo:
                cp.wait()

        att = output()
        ys[seg_rows(layer * seq, s), :] = x + att[0:SEG]
        return att[SEG:SEG + n_mem]

    def stage_tokens(t):
        h_a[0:SEG, :] = _layernorm(acts[seg_rows(0, t), :]).astype(BF16)
        h_a[SEG:2 * SEG, :] = _layernorm(acts[seg_rows(seq, t - LAG), :]).astype(BF16)

    def transpose_out(c):
        rows = pl.ds(pl.multiple_of(2 * seq + c * LANES, LANES), LANES)
        out_v[c] = acts[rows, :].T.astype(out_v.dtype)

    def out_copy(c):
        return pltpu.make_async_copy(out_v.at[c], out_hbm.at[:, pl.ds(pl.multiple_of(c * LANES, LANES), LANES)],
                                     out_sems.at[c])

    cp_x0 = pltpu.make_async_copy(xt_hbm.at[:, 0:LANES], xt_v.at[:, 0:LANES], sems.at[8])
    cp_x = pltpu.make_async_copy(xt_hbm.at[:, LANES:], xt_v.at[:, LANES:], sems.at[0])
    part_rows = d_model // QKV_PARTS
    cp_qkv = [pltpu.make_async_copy(w.at[pl.ds(p * part_rows * n_heads, part_rows * n_heads)],
                                    stage.at[i * QKV_PARTS + p], qkv_sems.at[i * QKV_PARTS + p])
              for i, w in enumerate((wq_hbm, wk_hbm, wv_hbm)) for p in range(QKV_PARTS)]
    cp_wo = [pltpu.make_async_copy(wot_hbm.at[i], wot.at[:, pl.ds(i * d_head, d_head)], sems.at[4])
             for i in range(n_heads)]
    cp_ff = [pltpu.make_async_copy(src.at[:, pl.ds(half * f_half, f_half)], dst.at[half], sems.at[5])
             for src, dst in ((w1_hbm, w1), (w3_hbm, w3), (w2t_hbm, w2t)) for half in range(2)]

    def transpose_in(c, carry):
        chunk = pl.ds(pl.multiple_of(c * LANES, LANES), LANES)
        acts[chunk, :] = xt_v[:, chunk].astype(F32).T
        return carry

    cp_x0.start()
    cp_qkv[0].start()
    cp_qkv[1].start()
    cp_x0.wait()
    acts[0:LANES, :] = xt_v[:, 0:LANES].astype(F32).T
    acts[2 * seq:2 * seq + LANES, :] = jnp.zeros((LANES, d_model), F32)

    pairs = n_heads // 2

    def split_heads(n, b, carry):
        i, p = n // QKV_PARTS, n % QKV_PARTS
        first = pl.multiple_of(b * SPLIT_ROWS * pairs, SPLIT_ROWS * pairs)
        block = stage.at[n].bitcast(jnp.uint32).at[pl.ds(first, SPLIT_ROWS * pairs)]
        features = pl.ds(pl.multiple_of(p * part_rows + b * SPLIT_ROWS, SPLIT_ROWS), SPLIT_ROWS)
        for j in range(pairs):
            w = block[pl.ds(j, SPLIT_ROWS, stride=pairs), :]
            even = pl.ds(pl.multiple_of((2 * j * 3 + i) * d_head, d_head), d_head)
            odd = pl.ds(pl.multiple_of(((2 * j + 1) * 3 + i) * d_head, d_head), d_head)
            wqkv[features, even] = pltpu.bitcast(w << 16, F32).astype(BF16)
            wqkv[features, odd] = pltpu.bitcast(w & jnp.uint32(0xFFFF0000), F32).astype(BF16)
        return carry

    def split_part(n, carry):
        pltpu.make_async_copy(stage.at[n], stage.at[n], qkv_sems.at[n]).wait()
        for m in range(2, len(cp_qkv)):
            pl.when(n + 2 == m)(cp_qkv[m].start)

        @pl.when(n + 2 == len(cp_qkv))
        def _():
            for cp in cp_wo:
                cp.start()

        return lax.fori_loop(0, part_rows // SPLIT_ROWS, functools.partial(split_heads, n), carry)

    lax.fori_loop(0, len(cp_qkv), split_part, 0)
    for cp in cp_ff:
        cp.start()

    def step_pair(i, carry):
        t0 = 2 * i
        src0 = (t0 - 2) * SEG
        lagged = (t0 - LAG - 2) * SEG
        ready = lagged >= 0
        half_stages, finish = ffn_stages(
            src0, jnp.where(ready, seq + lagged, 0), seq + src0, jnp.where(ready, 2 * seq + lagged, 3 * seq))
        for half in range(2):
            t = t0 + half
            hidden, ffn_output = half_stages(half)
            project, scores, mix, mixer_output = mixer_stages(h_a[...], 2 * SEG)
            emit([functools.partial(project, i) for i in range(n_heads)] + hidden, scores, mix)
            if half == 0:
                transpose_out(jnp.maximum(t - out_delay, 0) // segs_per_chunk)
                first_half = ffn_output()
            else:
                finish(first_half + ffn_output())
            stage_tokens(jnp.minimum(t + 1, n_seg - 1))
            att = mixer_output()
            h_a[2 * SEG:, :] = att[2 * SEG:].astype(BF16)
            ys[seg_rows(0, t), :] = acts[seg_rows(0, t), :] + att[0:SEG]
            ys[seg_rows(seq, t - LAG), :] = acts[seg_rows(seq, t - LAG), :] + att[SEG:2 * SEG]
        return carry

    out_delay = LAG + 2 + segs_per_chunk
    done = (n_seg - 2 - out_delay) // segs_per_chunk + 1
    mem0 = mem0_ref[...].astype(F32)
    h_a[2 * SEG:, :] = jnp.concatenate([mem0, mem0], axis=0).astype(BF16)

    def schedule_round(layer, carry):
        first = layer * (n_seg - LAG)
        mem = h_a[2 * SEG:, :].astype(F32)[n_mem:]
        mem = lax.fori_loop(first, first + LAG, functools.partial(mixer_only, layer), mem)

        @pl.when(layer == 0)
        def _():
            for cp in cp_ff:
                cp.wait()
            cp_x.start()
            lax.fori_loop(0, 2 * K_BLOCK // SUM_ROWS, form_weight_sums, 0)
            first_ffn()
            cp_x.wait()
            lax.fori_loop(1, n_chunks, transpose_in, 0, unroll=5)
            stage_tokens(LAG)
            h_a[2 * SEG:, :] = jnp.concatenate([mem, mem0], axis=0).astype(BF16)
            lax.fori_loop(LAG // 2, n_seg // 2, step_pair, 0)
            for c in range(done):
                out_copy(c).start()

        src0 = jnp.where(layer == 0, (n_seg - 2) * SEG, seq + (n_seg - 4) * SEG)
        src1 = jnp.where(layer == 0, seq + (n_seg - LAG - 2) * SEG, seq + (n_seg - 2) * SEG)

        def ffn_half(half, inner):
            half_stages, finish = ffn_stages(src0, src1, seq + src0, seq + src1)
            hidden, output = half_stages(half)
            for work in hidden:
                work()
            total = output() + jnp.where(half == 1, acc[...], 0.0)
            acc[...] = total
            finish(total)
            return inner

        lax.fori_loop(0, 2, ffn_half, 0)
        transpose_out(done + layer)
        out_copy(done + layer).start()
        return carry

    lax.fori_loop(0, 2, schedule_round, 0)
    for c in range(n_chunks):
        out_copy(c).wait()


@jax.jit
def pallas_interleave_layers__memory_aug_recurrent_mem_tr__glu_gated_swiglu__prompt_kernel(
    A_x, A_mem0, A_Wq, A_Wk, A_Wv, A_Wo, A_seg_len, B_x, B_w1, B_w3, B_w2,
):
    del A_seg_len, B_x
    batch, seq, d_model = A_x.shape
    _, n_heads, d_head = A_Wq.shape
    n_mem = A_mem0.shape[1]
    d_ff = B_w1.shape[1]
    assert batch == 1 and seq % 128 == 0 and d_ff % (4 * LANES) == 0
    rows = 2 * SEG + 2 * n_mem

    def kernel(*refs):
        _kernel(*refs, n_heads=n_heads, d_head=d_head, n_mem=n_mem)

    hbm = pl.BlockSpec(memory_space=pl.ANY)
    vmem = pl.BlockSpec(memory_space=pltpu.VMEM)
    out_t = pl.pallas_call(
        kernel,
        out_shape=jax.ShapeDtypeStruct((d_model, seq), A_x.dtype),
        in_specs=[hbm, vmem, hbm, hbm, hbm, hbm, hbm, hbm, hbm],
        out_specs=hbm,
        scratch_shapes=[
            pltpu.VMEM((d_model, seq), BF16),
            pltpu.VMEM((3 * QKV_PARTS, d_model * n_heads // QKV_PARTS, d_head), BF16),
            pltpu.VMEM((d_model, 3 * n_heads * d_head), BF16),
            pltpu.VMEM((d_model, n_heads * d_head), BF16),
            pltpu.VMEM((2, d_model, d_ff // 2), BF16),
            pltpu.VMEM((2, d_model, d_ff // 2), BF16),
            pltpu.VMEM((2, d_model, d_ff // 2), BF16),
            pltpu.VMEM((2, 5, K_BLOCK // 2, d_ff // 2), jnp.uint32),
            pltpu.VMEM((2, 5, K_BLOCK // 2, d_ff // 4), jnp.uint32),
            pltpu.VMEM((3 * seq + 2 * SEG, d_model), F32),
            pltpu.VMEM((2 * seq, d_model), F32),
            pltpu.VMEM((rows, d_model), BF16),
            pltpu.VMEM((4 * SEG, d_model), F32),
            pltpu.VMEM((seq // LANES, d_model, LANES), A_x.dtype),
            pltpu.SemaphoreType.DMA((9,)),
            pltpu.SemaphoreType.DMA((3 * QKV_PARTS,)),
            pltpu.SemaphoreType.DMA((seq // LANES,)),
        ],
        compiler_params=pltpu.CompilerParams(vmem_limit_bytes=126 * 1024 * 1024),
    )(
        A_x[0].T,
        A_mem0[0],
        A_Wq.reshape(d_model * n_heads, d_head),
        A_Wk.reshape(d_model * n_heads, d_head),
        A_Wv.reshape(d_model * n_heads, d_head),
        jnp.transpose(A_Wo, (0, 2, 1)),
        B_w1,
        B_w3,
        B_w2.T,
    )
    return out_t.T[None]
```

```python
import functools

import jax
import jax.numpy as jnp
from jax import lax
import jax.experimental.pallas as pl
import jax.experimental.pallas.tpu as pltpu

SEG = 32
EPS = 1e-5
MASK_FILL = -1000000000.0
LANES = 128
LAG = 4
SPLIT_ROWS = 48
QKV_PARTS = 4
K_BLOCK = 256
PLAIN_CHUNK = 384
SUM_ROWS = 32
STAGE_LAG = 5
BF16 = jnp.bfloat16
F32 = jnp.float32
NT_DIMS = (((1,), (1,)), ((), ()))


def _layernorm(x):
    inv_n = 1.0 / x.shape[-1]
    c = x - jnp.sum(x, axis=-1, keepdims=True) * inv_n
    v = jnp.sum(c * c, axis=-1, keepdims=True) * inv_n
    return c * lax.rsqrt(v + EPS)


def _strassen_lhs(a11, a12, a21, a22):
    return [a.astype(BF16) for a in (a11 + a22, a21 + a22, a11, a22, a11 + a12, a21 - a11, a12 - a22)]


def _strassen_rhs_sums(*blocks):
    words = [pltpu.bitcast(b, jnp.uint32) for b in blocks]
    halves = []
    for index in range(2):
        b11, b12, b21, b22 = (
            pltpu.unpack_elementwise(w, index=index, packed_dtype=BF16, unpacked_dtype=F32) for w in words)
        halves.append((b11 + b22, b12 - b22, b21 - b11, b11 + b12, b21 + b22))
    return [pltpu.pack_elementwise(list(pair), packed_dtype=BF16) for pair in zip(*halves)]


def _strassen_out(m1, m2, m3, m4, m5, m6, m7):
    return m1 + m4 - m5 + m7, m3 + m5, m2 + m4, m1 - m2 + m3 + m6


def _attention_mask(n_x, n_mem):
    rows = n_x + 2 * n_mem
    r = lax.broadcasted_iota(jnp.int32, (rows, rows), 0)
    c = lax.broadcasted_iota(jnp.int32, (rows, rows), 1)
    r_mem, c_mem = r >= n_x, c >= n_x
    r_stream = jnp.where(r_mem, (r - n_x) // n_mem, r // SEG)
    c_stream = jnp.where(c_mem, (c - n_x) // n_mem, c // SEG)
    same = r_stream == c_stream
    visible = same & (r_mem | c_mem | (c <= r))
    fill = jnp.where(same, MASK_FILL, -jnp.inf).astype(F32)
    return visible, fill


def _kernel(xt_hbm, mem0_ref, wq_hbm, wk_hbm, wv_hbm, wot_hbm, w1_hbm, w3_hbm, w2t_hbm,
            out_hbm,
            xt_v, stage, wqkv, wot, w1, w3, w2t, up_sums, down_sums,
            acts, ys, h_a, acc, out_v, sems, qkv_sems, out_sems,
            *, n_heads, d_head, n_mem):
    d_model, seq = xt_hbm.shape
    n_seg = seq // SEG
    n_chunks = seq // LANES
    segs_per_chunk = LANES // SEG
    f_half = w1.shape[2]
    f_quarter = f_half // 2
    k_lo, k_hi, k_rest = slice(0, K_BLOCK), slice(K_BLOCK, 2 * K_BLOCK), slice(2 * K_BLOCK, d_model)
    scale = d_head ** -0.5

    def seg_rows(base, s):
        return pl.ds(pl.multiple_of(base + s * SEG, SEG), SEG)

    def dot(a, b):
        return jnp.dot(a, b, preferred_element_type=F32)

    def dot_nt(a, b):
        return lax.dot_general(a, b, NT_DIMS, preferred_element_type=F32)

    def trailing_features(w_t, act):
        n, rows = w_t.shape[0], act.shape[0]
        out_t = dot_nt(w_t, act)
        if rows < LANES:
            out_t = jnp.concatenate([out_t, jnp.zeros((n, LANES - rows), F32)], axis=1)
        out_t = jnp.concatenate([out_t, jnp.zeros((LANES - n, LANES), F32)], axis=0)
        return out_t.T[:rows, :n]

    def pair_rows(start):
        return pl.ds(pl.multiple_of(start, 2 * SEG), 2 * SEG)

    def mixer_stages(h, n_x):
        rows = n_x + 2 * n_mem
        visible, fill = _attention_mask(n_x, n_mem)

        qkv, probs, mixed = {}, {}, {}

        def project(i):
            qkv[i] = dot(h, wqkv[:, 3 * i * d_head:3 * (i + 1) * d_head]).astype(BF16)

        def scores(i):
            s = dot_nt(qkv[i][:, 0:d_head], qkv[i][:, d_head:2 * d_head]) * scale
            s = jnp.where(visible, s, fill)
            e = jnp.exp(s - jnp.max(s, axis=-1, keepdims=True))
            probs[i] = (e * (1.0 / jnp.sum(e, axis=-1, keepdims=True))).astype(BF16)

        def mix(i):
            mixed[i] = dot(probs[i], qkv[i][:, 2 * d_head:]).astype(BF16)

        def output(lo=0, hi=n_heads):
            cols = slice(lo * d_head, hi * d_head)
            o = jnp.concatenate([mixed[i] for i in range(lo, hi)], axis=1)
            rest = trailing_features(wot[k_rest, cols], o)
            lead = dot_nt(o, wot[0:2 * K_BLOCK, cols])
            return jnp.concatenate([lead, rest], axis=1)

        return project, scores, mix, output

    def swiglu(gate, up):
        half_gate = 0.5 * gate
        return (half_gate + half_gate * jnp.tanh(half_gate)) * up

    def ffn_stages(src0, src1, dst0, dst1):
        y = jnp.concatenate([ys[pair_rows(src0), :], ys[pair_rows(src1), :]], axis=0)
        h = _layernorm(y)
        top, bot = slice(0, 2 * SEG), slice(2 * SEG, 4 * SEG)
        lhs = _strassen_lhs(h[top, k_lo], h[top, k_hi], h[bot, k_lo], h[bot, k_hi])
        rest = h[:, k_rest].astype(BF16)

        tiles = {}

        def hidden_tile(half, cols):
            rhs = (pltpu.bitcast(up_sums[half, 0, :, cols], BF16), w1[half, k_lo, cols], pltpu.bitcast(up_sums[half, 1, :, cols], BF16),
                   pltpu.bitcast(up_sums[half, 2, :, cols], BF16), w3[half, k_hi, cols], pltpu.bitcast(up_sums[half, 3, :, cols], BF16),
                   pltpu.bitcast(up_sums[half, 4, :, cols], BF16))
            gate_top, up_top, gate_bot, up_bot = _strassen_out(*(dot(a, b) for a, b in zip(lhs, rhs)))
            gate_rest = dot(rest, w1[half, k_rest, cols])
            gate_top, gate_bot = gate_top + gate_rest[top], gate_bot + gate_rest[bot]
            up_rest = dot(rest, w3[half, k_rest, cols])
            g_top = swiglu(gate_top, up_top + up_rest[top])
            g_bot = swiglu(gate_bot, up_bot + up_rest[bot])
            return g_top, g_bot

        def hidden(half, f):
            cols = slice(f * LANES, (f + 1) * LANES)
            g11, g21 = hidden_tile(half, cols)
            g12, g22 = hidden_tile(half, slice(f_quarter + f * LANES, f_quarter + (f + 1) * LANES))
            tiles[f] = _strassen_lhs(g11, g12, g21, g22) + [g12.astype(BF16), g21.astype(BF16)]

        def output(half):
            f_lo, f_hi = slice(0, f_quarter), slice(f_quarter, f_half)
            g = [jnp.concatenate([tiles[f][k] for f in range(f_quarter // LANES)], axis=1) for k in range(9)]
            plain = jnp.concatenate([jnp.concatenate([g[2], g[7]], axis=1),
                                     jnp.concatenate([g[8], g[3]], axis=1)], axis=0)
            rhs = (pltpu.bitcast(down_sums[half, 0], BF16), w2t[half, k_lo, f_lo], pltpu.bitcast(down_sums[half, 1], BF16), pltpu.bitcast(down_sums[half, 2], BF16),
                   w2t[half, k_hi, f_hi], pltpu.bitcast(down_sums[half, 3], BF16), pltpu.bitcast(down_sums[half, 4], BF16))
            c11, c12, c21, c22 = _strassen_out(*(dot_nt(a, b) for a, b in zip(g, rhs)))
            part = jnp.concatenate(
                [jnp.concatenate([c11, c21], axis=0), jnp.concatenate([c12, c22], axis=0),
                 trailing_features(w2t[half, k_rest, :], plain)], axis=1)
            return part

        def finish(update):
            z = y + update
            acts[pair_rows(dst0), :] = z[top]
            acts[pair_rows(dst1), :] = z[bot]

        def half_stages(half):
            return ([functools.partial(hidden, half, f) for f in range(f_quarter // LANES)],
                    functools.partial(output, half))

        return half_stages, finish

    def first_ffn():
        y = ys[0:2 * SEG, :]
        h = _layernorm(y).astype(BF16)

        def quarter_pass(n, z):
            half, first = n // 2, (n % 2) * f_quarter
            g = []
            for f in range(f_quarter // PLAIN_CHUNK):
                cols = pl.ds(pl.multiple_of(first + f * PLAIN_CHUNK, LANES), PLAIN_CHUNK)
                g.append(swiglu(dot(h, w1[half, :, cols]), dot(h, w3[half, :, cols])).astype(BF16))
            g = jnp.concatenate(g, axis=1)
            cols = pl.ds(pl.multiple_of(first, LANES), f_quarter)
            trailing = trailing_features(w2t[half, k_rest, cols], g)
            return z + jnp.concatenate([dot_nt(g, w2t[half, 0:2 * K_BLOCK, cols]), trailing], axis=1)

        acts[seq:seq + 2 * SEG, :] = lax.fori_loop(0, 4, quarter_pass, y)

    def form_weight_sums(i, carry):
        per_half = K_BLOCK // SUM_ROWS
        half = i // per_half
        r0 = pl.multiple_of((i % per_half) * SUM_ROWS, SUM_ROWS)
        lo, hi = pl.ds(r0, SUM_ROWS), pl.ds(r0 + K_BLOCK, SUM_ROWS)
        packed = pl.ds(pl.multiple_of(r0 // 2, SUM_ROWS // 2), SUM_ROWS // 2)
        for c in range(f_half // LANES):
            cols = slice(c * LANES, (c + 1) * LANES)
            blocks = (w1[half, lo, cols], w3[half, lo, cols], w1[half, hi, cols], w3[half, hi, cols])
            for k, b in enumerate(_strassen_rhs_sums(*blocks)):
                up_sums[half, k, packed, cols] = b
        for c in range(f_quarter // LANES):
            cols = slice(c * LANES, (c + 1) * LANES)
            cols_hi = slice(f_quarter + c * LANES, f_quarter + (c + 1) * LANES)
            blocks = (w2t[half, lo, cols], w2t[half, hi, cols], w2t[half, lo, cols_hi], w2t[half, hi, cols_hi])
            for k, b in enumerate(_strassen_rhs_sums(*blocks)):
                down_sums[half, k, packed, cols] = b
        return carry

    def emit(matmul_work, scores, mix, lag=STAGE_LAG):
        for i in range(max(len(matmul_work), n_heads + 2 * lag)):
            if i < len(matmul_work):
                matmul_work[i]()
            if 0 <= i - lag < n_heads:
                scores(i - lag)
            if 0 <= i - 2 * lag < n_heads:
                mix(i - 2 * lag)

    def stage_segment(layer, s):
        h_a[0:SEG, :] = _layernorm(acts[seg_rows(layer * seq, s), :]).astype(BF16)

    def mixer_only(layer, s, mem):
        x = acts[seg_rows(layer * seq, s), :]
        tail = jnp.concatenate([mem, jnp.zeros_like(mem)], axis=0)
        h = jnp.concatenate([h_a[0:SEG, :], tail.astype(BF16)], axis=0)
        project, scores, mix, output = mixer_stages(h, SEG)

        def await_weights():
            @pl.when(s == 0)
            def _():
                for cp in cp_wo:
                    cp.wait()

        work = [functools.partial(project, i) for i in range(n_heads)]
        emit(work, scores, mix, 5)
        await_weights()
        stage_segment(layer, jnp.minimum(s + 1, layer * (n_seg - LAG) + LAG - 1))
        att = output()
        ys[seg_rows(layer * seq, s), :] = x + att[0:SEG]
        return att[SEG:SEG + n_mem]

    def stage_tokens(t):
        h_a[0:SEG, :] = _layernorm(acts[seg_rows(0, t), :]).astype(BF16)
        h_a[SEG:2 * SEG, :] = _layernorm(acts[seg_rows(seq, t - LAG), :]).astype(BF16)

    def transpose_out(c):
        rows = pl.ds(pl.multiple_of(2 * seq + c * LANES, LANES), LANES)
        out_v[c] = acts[rows, :].T.astype(out_v.dtype)

    def out_copy(c):
        return pltpu.make_async_copy(out_v.at[c], out_hbm.at[:, pl.ds(pl.multiple_of(c * LANES, LANES), LANES)],
                                     out_sems.at[c])

    cp_x0 = pltpu.make_async_copy(xt_hbm.at[:, 0:LANES], xt_v.at[:, 0:LANES], sems.at[8])
    cp_x = pltpu.make_async_copy(xt_hbm.at[:, LANES:], xt_v.at[:, LANES:], sems.at[0])
    part_rows = d_model // QKV_PARTS
    cp_qkv = [pltpu.make_async_copy(w.at[pl.ds(p * part_rows * n_heads, part_rows * n_heads)],
                                    stage.at[i * QKV_PARTS + p], qkv_sems.at[i * QKV_PARTS + p])
              for i, w in enumerate((wq_hbm, wk_hbm, wv_hbm)) for p in range(QKV_PARTS)]
    cp_wo = [pltpu.make_async_copy(wot_hbm.at[i], wot.at[:, pl.ds(i * d_head, d_head)], sems.at[4])
             for i in range(n_heads)]
    cp_ff = [pltpu.make_async_copy(src.at[:, pl.ds(half * f_half, f_half)], dst.at[half], sems.at[5])
             for src, dst in ((w1_hbm, w1), (w3_hbm, w3), (w2t_hbm, w2t)) for half in range(2)]

    def transpose_in(c, carry):
        chunk = pl.ds(pl.multiple_of(c * LANES, LANES), LANES)
        acts[chunk, :] = xt_v[:, chunk].astype(F32).T
        return carry

    cp_x0.start()
    cp_qkv[0].start()
    cp_qkv[1].start()
    cp_x0.wait()
    acts[0:LANES, :] = xt_v[:, 0:LANES].astype(F32).T
    acts[2 * seq:2 * seq + LANES, :] = jnp.zeros((LANES, d_model), F32)

    pairs = n_heads // 2

    def split_heads(n, b, carry):
        i, p = n // QKV_PARTS, n % QKV_PARTS
        first = pl.multiple_of(b * SPLIT_ROWS * pairs, SPLIT_ROWS * pairs)
        block = stage.at[n].bitcast(jnp.uint32).at[pl.ds(first, SPLIT_ROWS * pairs)]
        features = pl.ds(pl.multiple_of(p * part_rows + b * SPLIT_ROWS, SPLIT_ROWS), SPLIT_ROWS)
        for j in range(pairs):
            w = block[pl.ds(j, SPLIT_ROWS, stride=pairs), :]
            even = pl.ds(pl.multiple_of((2 * j * 3 + i) * d_head, d_head), d_head)
            odd = pl.ds(pl.multiple_of(((2 * j + 1) * 3 + i) * d_head, d_head), d_head)
            wqkv[features, even] = pltpu.bitcast(w << 16, F32).astype(BF16)
            wqkv[features, odd] = pltpu.bitcast(w & jnp.uint32(0xFFFF0000), F32).astype(BF16)
        return carry

    def split_part(n, carry):
        pltpu.make_async_copy(stage.at[n], stage.at[n], qkv_sems.at[n]).wait()
        for m in range(2, len(cp_qkv)):
            pl.when(n + 2 == m)(cp_qkv[m].start)

        @pl.when(n + 2 == len(cp_qkv))
        def _():
            for cp in cp_wo:
                cp.start()

        return lax.fori_loop(0, part_rows // SPLIT_ROWS, functools.partial(split_heads, n), carry)

    lax.fori_loop(0, len(cp_qkv), split_part, 0)
    for cp in cp_ff:
        cp.start()

    def step_pair(i, carry):
        t0 = 2 * i
        src0 = (t0 - 2) * SEG
        lagged = (t0 - LAG - 2) * SEG
        ready = lagged >= 0
        half_stages, finish = ffn_stages(
            src0, jnp.where(ready, seq + lagged, 0), seq + src0, jnp.where(ready, 2 * seq + lagged, 3 * seq))
        for half in range(2):
            t = t0 + half
            hidden, ffn_output = half_stages(half)
            project, scores, mix, mixer_output = mixer_stages(h_a[...], 2 * SEG)
            emit([functools.partial(project, i) for i in range(n_heads)] + hidden, scores, mix)
            if half == 0:
                transpose_out(jnp.maximum(t - out_delay, 0) // segs_per_chunk)
                first_half = ffn_output()
            else:
                finish(first_half + ffn_output())
            stage_tokens(jnp.minimum(t + 1, n_seg - 1))
            att = mixer_output()
            h_a[2 * SEG:, :] = att[2 * SEG:].astype(BF16)
            ys[seg_rows(0, t), :] = acts[seg_rows(0, t), :] + att[0:SEG]
            ys[seg_rows(seq, t - LAG), :] = acts[seg_rows(seq, t - LAG), :] + att[SEG:2 * SEG]
        return carry

    out_delay = LAG + 2 + segs_per_chunk
    done = (n_seg - 2 - out_delay) // segs_per_chunk + 1
    mem0 = mem0_ref[...].astype(F32)
    h_a[2 * SEG:, :] = jnp.concatenate([mem0, mem0], axis=0).astype(BF16)

    def schedule_round(layer, carry):
        first = layer * (n_seg - LAG)
        mem = h_a[2 * SEG:, :].astype(F32)[n_mem:]
        stage_segment(layer, first)
        mem = lax.fori_loop(first, first + LAG, functools.partial(mixer_only, layer), mem)

        @pl.when(layer == 0)
        def _():
            for cp in cp_ff:
                cp.wait()
            cp_x.start()
            lax.fori_loop(0, 2 * K_BLOCK // SUM_ROWS, form_weight_sums, 0)
            first_ffn()
            cp_x.wait()
            lax.fori_loop(1, n_chunks, transpose_in, 0, unroll=5)
            stage_tokens(LAG)
            h_a[2 * SEG:, :] = jnp.concatenate([mem, mem0], axis=0).astype(BF16)
            lax.fori_loop(LAG // 2, n_seg // 2, step_pair, 0)
            for c in range(done):
                out_copy(c).start()

        src0 = jnp.where(layer == 0, (n_seg - 2) * SEG, seq + (n_seg - 4) * SEG)
        src1 = jnp.where(layer == 0, seq + (n_seg - LAG - 2) * SEG, seq + (n_seg - 2) * SEG)

        def ffn_half(half, inner):
            half_stages, finish = ffn_stages(src0, src1, seq + src0, seq + src1)
            hidden, output = half_stages(half)
            for work in hidden:
                work()
            total = output() + jnp.where(half == 1, acc[...], 0.0)
            acc[...] = total
            finish(total)
            return inner

        lax.fori_loop(0, 2, ffn_half, 0)
        transpose_out(done + layer)
        out_copy(done + layer).start()
        return carry

    lax.fori_loop(0, 2, schedule_round, 0)
    for c in range(n_chunks):
        out_copy(c).wait()


@jax.jit
def pallas_interleave_layers__memory_aug_recurrent_mem_tr__glu_gated_swiglu__prompt_kernel(
    A_x, A_mem0, A_Wq, A_Wk, A_Wv, A_Wo, A_seg_len, B_x, B_w1, B_w3, B_w2,
):
    del A_seg_len, B_x
    batch, seq, d_model = A_x.shape
    _, n_heads, d_head = A_Wq.shape
    n_mem = A_mem0.shape[1]
    d_ff = B_w1.shape[1]
    assert batch == 1 and seq % 128 == 0 and d_ff % (4 * LANES) == 0
    rows = 2 * SEG + 2 * n_mem

    def kernel(*refs):
        _kernel(*refs, n_heads=n_heads, d_head=d_head, n_mem=n_mem)

    hbm = pl.BlockSpec(memory_space=pl.ANY)
    vmem = pl.BlockSpec(memory_space=pltpu.VMEM)
    out_t = pl.pallas_call(
        kernel,
        out_shape=jax.ShapeDtypeStruct((d_model, seq), A_x.dtype),
        in_specs=[hbm, vmem, hbm, hbm, hbm, hbm, hbm, hbm, hbm],
        out_specs=hbm,
        scratch_shapes=[
            pltpu.VMEM((d_model, seq), BF16),
            pltpu.VMEM((3 * QKV_PARTS, d_model * n_heads // QKV_PARTS, d_head), BF16),
            pltpu.VMEM((d_model, 3 * n_heads * d_head), BF16),
            pltpu.VMEM((d_model, n_heads * d_head), BF16),
            pltpu.VMEM((2, d_model, d_ff // 2), BF16),
            pltpu.VMEM((2, d_model, d_ff // 2), BF16),
            pltpu.VMEM((2, d_model, d_ff // 2), BF16),
            pltpu.VMEM((2, 5, K_BLOCK // 2, d_ff // 2), jnp.uint32),
            pltpu.VMEM((2, 5, K_BLOCK // 2, d_ff // 4), jnp.uint32),
            pltpu.VMEM((3 * seq + 2 * SEG, d_model), F32),
            pltpu.VMEM((2 * seq, d_model), F32),
            pltpu.VMEM((rows, d_model), BF16),
            pltpu.VMEM((4 * SEG, d_model), F32),
            pltpu.VMEM((seq // LANES, d_model, LANES), A_x.dtype),
            pltpu.SemaphoreType.DMA((9,)),
            pltpu.SemaphoreType.DMA((3 * QKV_PARTS,)),
            pltpu.SemaphoreType.DMA((seq // LANES,)),
        ],
        compiler_params=pltpu.CompilerParams(vmem_limit_bytes=126 * 1024 * 1024),
    )(
        A_x[0].T,
        A_mem0[0],
        A_Wq.reshape(d_model * n_heads, d_head),
        A_Wk.reshape(d_model * n_heads, d_head),
        A_Wv.reshape(d_model * n_heads, d_head),
        jnp.transpose(A_Wo, (0, 2, 1)),
        B_w1,
        B_w3,
        B_w2.T,
    )
    return out_t.T[None]
```

```python
import functools

import jax
import jax.numpy as jnp
from jax import lax
import jax.experimental.pallas as pl
import jax.experimental.pallas.tpu as pltpu

SEG = 32
EPS = 1e-5
MASK_FILL = -1000000000.0
LANES = 128
LAG = 4
SPLIT_ROWS = 48
QKV_PARTS = 4
K_BLOCK = 256
PLAIN_CHUNK = 384
SUM_ROWS = 32
STAGE_LAG = 5
BF16 = jnp.bfloat16
F32 = jnp.float32
NT_DIMS = (((1,), (1,)), ((), ()))


def _layernorm(x):
    inv_n = 1.0 / x.shape[-1]
    c = x - jnp.sum(x, axis=-1, keepdims=True) * inv_n
    v = jnp.sum(c * c, axis=-1, keepdims=True) * inv_n
    return c * lax.rsqrt(v + EPS)


def _strassen_lhs(a11, a12, a21, a22):
    return [a.astype(BF16) for a in (a11 + a22, a21 + a22, a11, a22, a11 + a12, a21 - a11, a12 - a22)]


def _strassen_rhs_sums(*blocks):
    words = [pltpu.bitcast(b, jnp.uint32) for b in blocks]
    halves = []
    for index in range(2):
        b11, b12, b21, b22 = (
            pltpu.unpack_elementwise(w, index=index, packed_dtype=BF16, unpacked_dtype=F32) for w in words)
        halves.append((b11 + b22, b12 - b22, b21 - b11, b11 + b12, b21 + b22))
    return [pltpu.pack_elementwise(list(pair), packed_dtype=BF16) for pair in zip(*halves)]


def _strassen_out(m1, m2, m3, m4, m5, m6, m7):
    return m1 + m4 - m5 + m7, m3 + m5, m2 + m4, m1 - m2 + m3 + m6


def _attention_mask(n_x, n_mem):
    rows = n_x + 2 * n_mem
    r = lax.broadcasted_iota(jnp.int32, (rows, rows), 0)
    c = lax.broadcasted_iota(jnp.int32, (rows, rows), 1)
    r_mem, c_mem = r >= n_x, c >= n_x
    r_stream = jnp.where(r_mem, (r - n_x) // n_mem, r // SEG)
    c_stream = jnp.where(c_mem, (c - n_x) // n_mem, c // SEG)
    same = r_stream == c_stream
    visible = same & (r_mem | c_mem | (c <= r))
    fill = jnp.where(same, MASK_FILL, -jnp.inf).astype(F32)
    return visible, fill


def _kernel(xt_hbm, mem0_ref, wq_hbm, wk_hbm, wv_hbm, wot_hbm, w1_hbm, w3_hbm, w2t_hbm,
            out_hbm,
            xt_v, stage, wqkv, wot, w1, w3, w2t, up_sums, down_sums,
            acts, ys, h_a, acc, out_v, sems, qkv_sems, out_sems,
            *, n_heads, d_head, n_mem):
    d_model, seq = xt_hbm.shape
    n_seg = seq // SEG
    n_chunks = seq // LANES
    segs_per_chunk = LANES // SEG
    f_half = w1.shape[2]
    f_quarter = f_half // 2
    k_lo, k_hi, k_rest = slice(0, K_BLOCK), slice(K_BLOCK, 2 * K_BLOCK), slice(2 * K_BLOCK, d_model)
    scale = d_head ** -0.5

    def seg_rows(base, s):
        return pl.ds(pl.multiple_of(base + s * SEG, SEG), SEG)

    def dot(a, b):
        return jnp.dot(a, b, preferred_element_type=F32)

    def dot_nt(a, b):
        return lax.dot_general(a, b, NT_DIMS, preferred_element_type=F32)

    def trailing_features(w_t, act):
        n, rows = w_t.shape[0], act.shape[0]
        out_t = dot_nt(w_t, act)
        if rows < LANES:
            out_t = jnp.concatenate([out_t, jnp.zeros((n, LANES - rows), F32)], axis=1)
        out_t = jnp.concatenate([out_t, jnp.zeros((LANES - n, LANES), F32)], axis=0)
        return out_t.T[:rows, :n]

    def pair_rows(start):
        return pl.ds(pl.multiple_of(start, 2 * SEG), 2 * SEG)

    def mixer_stages(h, n_x):
        rows = n_x + 2 * n_mem
        visible, fill = _attention_mask(n_x, n_mem)

        qkv, probs, mixed = {}, {}, {}

        def project(i):
            qkv[i] = dot(h, wqkv[:, 3 * i * d_head:3 * (i + 1) * d_head]).astype(BF16)

        def scores(i):
            s = dot_nt(qkv[i][:, 0:d_head], qkv[i][:, d_head:2 * d_head]) * scale
            s = jnp.where(visible, s, fill)
            e = jnp.exp(s - jnp.max(s, axis=-1, keepdims=True))
            probs[i] = (e * (1.0 / jnp.sum(e, axis=-1, keepdims=True))).astype(BF16)

        def mix(i):
            mixed[i] = dot(probs[i], qkv[i][:, 2 * d_head:]).astype(BF16)

        def output():
            o = jnp.concatenate([mixed[i] for i in range(n_heads)], axis=1)
            rest = trailing_features(wot[k_rest, :], o)
            return jnp.concatenate([dot_nt(o, wot[0:2 * K_BLOCK, :]), rest], axis=1)

        return project, scores, mix, output

    def swiglu(gate, up):
        half_gate = 0.5 * gate
        return (half_gate + half_gate * jnp.tanh(half_gate)) * up

    def ffn_stages(src0, src1, dst0, dst1):
        y = jnp.concatenate([ys[pair_rows(src0), :], ys[pair_rows(src1), :]], axis=0)
        h = _layernorm(y)
        top, bot = slice(0, 2 * SEG), slice(2 * SEG, 4 * SEG)
        lhs = _strassen_lhs(h[top, k_lo], h[top, k_hi], h[bot, k_lo], h[bot, k_hi])
        rest = h[:, k_rest].astype(BF16)

        tiles = {}

        def hidden_tile(half, cols):
            rhs = (pltpu.bitcast(up_sums[half, 0, :, cols], BF16), w1[half, k_lo, cols], pltpu.bitcast(up_sums[half, 1, :, cols], BF16),
                   pltpu.bitcast(up_sums[half, 2, :, cols], BF16), w3[half, k_hi, cols], pltpu.bitcast(up_sums[half, 3, :, cols], BF16),
                   pltpu.bitcast(up_sums[half, 4, :, cols], BF16))
            gate_top, up_top, gate_bot, up_bot = _strassen_out(*(dot(a, b) for a, b in zip(lhs, rhs)))
            gate_rest = dot(rest, w1[half, k_rest, cols])
            gate_top, gate_bot = gate_top + gate_rest[top], gate_bot + gate_rest[bot]
            up_rest = dot(rest, w3[half, k_rest, cols])
            g_top = swiglu(gate_top, up_top + up_rest[top])
            g_bot = swiglu(gate_bot, up_bot + up_rest[bot])
            return g_top, g_bot

        def hidden(half, f):
            cols = slice(f * LANES, (f + 1) * LANES)
            g11, g21 = hidden_tile(half, cols)
            g12, g22 = hidden_tile(half, slice(f_quarter + f * LANES, f_quarter + (f + 1) * LANES))
            tiles[f] = _strassen_lhs(g11, g12, g21, g22) + [g12.astype(BF16), g21.astype(BF16)]

        def output(half):
            f_lo, f_hi = slice(0, f_quarter), slice(f_quarter, f_half)
            g = [jnp.concatenate([tiles[f][k] for f in range(f_quarter // LANES)], axis=1) for k in range(9)]
            plain = jnp.concatenate([jnp.concatenate([g[2], g[7]], axis=1),
                                     jnp.concatenate([g[8], g[3]], axis=1)], axis=0)
            rhs = (pltpu.bitcast(down_sums[half, 0], BF16), w2t[half, k_lo, f_lo], pltpu.bitcast(down_sums[half, 1], BF16), pltpu.bitcast(down_sums[half, 2], BF16),
                   w2t[half, k_hi, f_hi], pltpu.bitcast(down_sums[half, 3], BF16), pltpu.bitcast(down_sums[half, 4], BF16))
            c11, c12, c21, c22 = _strassen_out(*(dot_nt(a, b) for a, b in zip(g, rhs)))
            part = jnp.concatenate(
                [jnp.concatenate([c11, c21], axis=0), jnp.concatenate([c12, c22], axis=0),
                 trailing_features(w2t[half, k_rest, :], plain)], axis=1)
            return part

        def finish(update):
            z = y + update
            acts[pair_rows(dst0), :] = z[top]
            acts[pair_rows(dst1), :] = z[bot]

        def half_stages(half):
            return ([functools.partial(hidden, half, f) for f in range(f_quarter // LANES)],
                    functools.partial(output, half))

        return half_stages, finish

    def first_ffn():
        y = ys[0:2 * SEG, :]
        h = _layernorm(y).astype(BF16)

        def quarter_pass(n, z):
            half, first = n // 2, (n % 2) * f_quarter
            g = []
            for f in range(f_quarter // PLAIN_CHUNK):
                cols = pl.ds(pl.multiple_of(first + f * PLAIN_CHUNK, LANES), PLAIN_CHUNK)
                g.append(swiglu(dot(h, w1[half, :, cols]), dot(h, w3[half, :, cols])).astype(BF16))
            g = jnp.concatenate(g, axis=1)
            cols = pl.ds(pl.multiple_of(first, LANES), f_quarter)
            trailing = trailing_features(w2t[half, k_rest, cols], g)
            return z + jnp.concatenate([dot_nt(g, w2t[half, 0:2 * K_BLOCK, cols]), trailing], axis=1)

        acts[seq:seq + 2 * SEG, :] = lax.fori_loop(0, 4, quarter_pass, y)

    def form_weight_sums(i, carry):
        per_half = K_BLOCK // SUM_ROWS
        half = i // per_half
        r0 = pl.multiple_of((i % per_half) * SUM_ROWS, SUM_ROWS)
        lo, hi = pl.ds(r0, SUM_ROWS), pl.ds(r0 + K_BLOCK, SUM_ROWS)
        packed = pl.ds(pl.multiple_of(r0 // 2, SUM_ROWS // 2), SUM_ROWS // 2)
        for c in range(f_half // LANES):
            cols = slice(c * LANES, (c + 1) * LANES)
            blocks = (w1[half, lo, cols], w3[half, lo, cols], w1[half, hi, cols], w3[half, hi, cols])
            for k, b in enumerate(_strassen_rhs_sums(*blocks)):
                up_sums[half, k, packed, cols] = b
        for c in range(f_quarter // LANES):
            cols = slice(c * LANES, (c + 1) * LANES)
            cols_hi = slice(f_quarter + c * LANES, f_quarter + (c + 1) * LANES)
            blocks = (w2t[half, lo, cols], w2t[half, hi, cols], w2t[half, lo, cols_hi], w2t[half, hi, cols_hi])
            for k, b in enumerate(_strassen_rhs_sums(*blocks)):
                down_sums[half, k, packed, cols] = b
        return carry

    def emit(matmul_work, scores, mix):
        for i in range(max(len(matmul_work), n_heads + 2 * STAGE_LAG)):
            if i < len(matmul_work):
                matmul_work[i]()
            if 0 <= i - STAGE_LAG < n_heads:
                scores(i - STAGE_LAG)
            if 0 <= i - 2 * STAGE_LAG < n_heads:
                mix(i - 2 * STAGE_LAG)

    def stage_segment(layer, s):
        h_a[0:SEG, :] = _layernorm(acts[seg_rows(layer * seq, s), :]).astype(BF16)

    def mixer_only(layer, s, mem):
        x = acts[seg_rows(layer * seq, s), :]
        tail = jnp.concatenate([mem, jnp.zeros_like(mem)], axis=0)
        h = jnp.concatenate([h_a[0:SEG, :], tail.astype(BF16)], axis=0)
        project, scores, mix, output = mixer_stages(h, SEG)
        emit([functools.partial(project, i) for i in range(n_heads)], scores, mix)

        @pl.when(s == 0)
        def _():
            for cp in cp_wo:
                cp.wait()

        stage_segment(layer, jnp.minimum(s + 1, layer * (n_seg - LAG) + LAG - 1))
        att = output()
        ys[seg_rows(layer * seq, s), :] = x + att[0:SEG]
        return att[SEG:SEG + n_mem]

    def stage_tokens(t):
        h_a[0:SEG, :] = _layernorm(acts[seg_rows(0, t), :]).astype(BF16)
        h_a[SEG:2 * SEG, :] = _layernorm(acts[seg_rows(seq, t - LAG), :]).astype(BF16)

    def transpose_out(c):
        rows = pl.ds(pl.multiple_of(2 * seq + c * LANES, LANES), LANES)
        out_v[c] = acts[rows, :].T.astype(out_v.dtype)

    def out_copy(c):
        return pltpu.make_async_copy(out_v.at[c], out_hbm.at[:, pl.ds(pl.multiple_of(c * LANES, LANES), LANES)],
                                     out_sems.at[c])

    cp_x0 = pltpu.make_async_copy(xt_hbm.at[:, 0:LANES], xt_v.at[:, 0:LANES], sems.at[8])
    cp_x = pltpu.make_async_copy(xt_hbm.at[:, LANES:], xt_v.at[:, LANES:], sems.at[0])
    part_rows = d_model // QKV_PARTS
    cp_qkv = [pltpu.make_async_copy(w.at[pl.ds(p * part_rows * n_heads, part_rows * n_heads)],
                                    stage.at[i * QKV_PARTS + p, pl.ds(0, part_rows * n_heads)],
                                    qkv_sems.at[i * QKV_PARTS + p])
              for i, w in enumerate((wq_hbm, wk_hbm, wv_hbm)) for p in range(QKV_PARTS)]
    cp_wo = [pltpu.make_async_copy(wot_hbm.at[i], wot.at[:, pl.ds(i * d_head, d_head)], sems.at[4])
             for i in range(n_heads)]
    cp_ff = [pltpu.make_async_copy(src.at[:, pl.ds(half * f_half, f_half)], dst.at[half], sems.at[5])
             for src, dst in ((w1_hbm, w1), (w3_hbm, w3), (w2t_hbm, w2t)) for half in range(2)]

    def transpose_in(c, carry):
        chunk = pl.ds(pl.multiple_of(c * LANES, LANES), LANES)
        acts[chunk, :] = xt_v[:, chunk].astype(F32).T
        return carry

    cp_x0.start()
    cp_qkv[0].start()
    cp_qkv[1].start()
    cp_x0.wait()
    acts[0:LANES, :] = xt_v[:, 0:LANES].astype(F32).T
    acts[2 * seq:2 * seq + LANES, :] = jnp.zeros((LANES, d_model), F32)
    acc[...] = jnp.zeros(acc.shape, F32)

    pairs = n_heads // 2

    def split_heads(n, b, carry):
        i, p = n // QKV_PARTS, n % QKV_PARTS
        first = pl.multiple_of(b * SPLIT_ROWS * pairs, SPLIT_ROWS * pairs)
        block = stage.at[n].bitcast(jnp.uint32).at[pl.ds(first, (SPLIT_ROWS + 1) * pairs)]
        features = pl.ds(pl.multiple_of(p * part_rows + b * SPLIT_ROWS, SPLIT_ROWS), SPLIT_ROWS)
        for j in range(pairs):
            w = block[pl.ds(j, SPLIT_ROWS, stride=pairs), :]
            even = pl.ds(pl.multiple_of((2 * j * 3 + i) * d_head, d_head), d_head)
            odd = pl.ds(pl.multiple_of(((2 * j + 1) * 3 + i) * d_head, d_head), d_head)
            wqkv[features, even] = pltpu.bitcast(w << 16, F32).astype(BF16)
            wqkv[features, odd] = pltpu.bitcast(w & jnp.uint32(0xFFFF0000), F32).astype(BF16)
        return carry

    def split_part(n, carry):
        landed = stage.at[n, pl.ds(0, part_rows * n_heads)]
        pltpu.make_async_copy(landed, landed, qkv_sems.at[n]).wait()
        for m in range(2, len(cp_qkv)):
            pl.when(n + 2 == m)(cp_qkv[m].start)

        @pl.when(n + 2 == len(cp_qkv))
        def _():
            for cp in cp_wo:
                cp.start()

        return lax.fori_loop(0, part_rows // SPLIT_ROWS, functools.partial(split_heads, n), carry)

    lax.fori_loop(0, len(cp_qkv), split_part, 0)
    for cp in cp_ff:
        cp.start()

    def step_pair(i, carry):
        t0 = 2 * i
        src0 = (t0 - 2) * SEG
        lagged = (t0 - LAG - 2) * SEG
        ready = lagged >= 0
        half_stages, finish = ffn_stages(
            src0, jnp.where(ready, seq + lagged, 0), seq + src0, jnp.where(ready, 2 * seq + lagged, 3 * seq))
        for half in range(2):
            t = t0 + half
            hidden, ffn_output = half_stages(half)
            project, scores, mix, mixer_output = mixer_stages(h_a[...], 2 * SEG)
            emit([functools.partial(project, i) for i in range(n_heads)] + hidden, scores, mix)
            if half == 0:
                transpose_out(jnp.maximum(t - out_delay, 0) // segs_per_chunk)
                first_half = ffn_output()
            else:
                finish(first_half + ffn_output())
            stage_tokens(jnp.minimum(t + 1, n_seg - 1))
            att = mixer_output()
            h_a[2 * SEG:, :] = att[2 * SEG:].astype(BF16)
            ys[seg_rows(0, t), :] = acts[seg_rows(0, t), :] + att[0:SEG]
            ys[seg_rows(seq, t - LAG), :] = acts[seg_rows(seq, t - LAG), :] + att[SEG:2 * SEG]
        return carry

    out_delay = LAG + 2 + segs_per_chunk
    done = (n_seg - 2 - out_delay) // segs_per_chunk + 1
    mem0 = mem0_ref[...].astype(F32)
    h_a[2 * SEG:, :] = jnp.concatenate([mem0, mem0], axis=0).astype(BF16)

    def schedule_round(layer, carry):
        first = layer * (n_seg - LAG)
        mem = h_a[2 * SEG:, :].astype(F32)[n_mem:]
        stage_segment(layer, first)
        mem = lax.fori_loop(first, first + LAG, functools.partial(mixer_only, layer), mem)

        @pl.when(layer == 0)
        def _():
            for cp in cp_ff:
                cp.wait()
            cp_x.start()
            lax.fori_loop(0, 2 * K_BLOCK // SUM_ROWS, form_weight_sums, 0)
            first_ffn()
            cp_x.wait()
            lax.fori_loop(1, n_chunks, transpose_in, 0, unroll=5)
            stage_tokens(LAG)
            h_a[2 * SEG:, :] = jnp.concatenate([mem, mem0], axis=0).astype(BF16)
            lax.fori_loop(LAG // 2, n_seg // 2, step_pair, 0)
            for c in range(done):
                out_copy(c).start()

        src0 = jnp.where(layer == 0, (n_seg - 2) * SEG, seq + (n_seg - 4) * SEG)
        src1 = jnp.where(layer == 0, seq + (n_seg - LAG - 2) * SEG, seq + (n_seg - 2) * SEG)

        def ffn_half(half, inner):
            half_stages, finish = ffn_stages(src0, src1, seq + src0, seq + src1)
            hidden, output = half_stages(half)
            for work in hidden:
                work()
            total = output() + jnp.where(half == 1, acc[...], 0.0)
            acc[...] = total
            finish(total)
            return inner

        lax.fori_loop(0, 2, ffn_half, 0)
        transpose_out(done + layer)
        out_copy(done + layer).start()
        return carry

    lax.fori_loop(0, 2, schedule_round, 0)
    for c in range(n_chunks):
        out_copy(c).wait()


@jax.jit
def pallas_interleave_layers__memory_aug_recurrent_mem_tr__glu_gated_swiglu__prompt_kernel(
    A_x, A_mem0, A_Wq, A_Wk, A_Wv, A_Wo, A_seg_len, B_x, B_w1, B_w3, B_w2,
):
    del A_seg_len, B_x
    batch, seq, d_model = A_x.shape
    _, n_heads, d_head = A_Wq.shape
    n_mem = A_mem0.shape[1]
    d_ff = B_w1.shape[1]
    assert batch == 1 and seq % 128 == 0 and d_ff % (4 * LANES) == 0
    rows = 2 * SEG + 2 * n_mem

    def kernel(*refs):
        _kernel(*refs, n_heads=n_heads, d_head=d_head, n_mem=n_mem)

    hbm = pl.BlockSpec(memory_space=pl.ANY)
    vmem = pl.BlockSpec(memory_space=pltpu.VMEM)
    out_t = pl.pallas_call(
        kernel,
        out_shape=jax.ShapeDtypeStruct((d_model, seq), A_x.dtype),
        in_specs=[hbm, vmem, hbm, hbm, hbm, hbm, hbm, hbm, hbm],
        out_specs=hbm,
        scratch_shapes=[
            pltpu.VMEM((d_model, seq), BF16),
            pltpu.VMEM((3 * QKV_PARTS, (d_model // QKV_PARTS + 1) * n_heads, d_head), BF16),
            pltpu.VMEM((d_model, 3 * n_heads * d_head), BF16),
            pltpu.VMEM((d_model, n_heads * d_head), BF16),
            pltpu.VMEM((2, d_model, d_ff // 2), BF16),
            pltpu.VMEM((2, d_model, d_ff // 2), BF16),
            pltpu.VMEM((2, d_model, d_ff // 2), BF16),
            pltpu.VMEM((2, 5, K_BLOCK // 2, d_ff // 2), jnp.uint32),
            pltpu.VMEM((2, 5, K_BLOCK // 2, d_ff // 4), jnp.uint32),
            pltpu.VMEM((3 * seq + 2 * SEG, d_model), F32),
            pltpu.VMEM((2 * seq, d_model), F32),
            pltpu.VMEM((rows, d_model), BF16),
            pltpu.VMEM((4 * SEG, d_model), F32),
            pltpu.VMEM((seq // LANES, d_model, LANES), A_x.dtype),
            pltpu.SemaphoreType.DMA((9,)),
            pltpu.SemaphoreType.DMA((3 * QKV_PARTS,)),
            pltpu.SemaphoreType.DMA((seq // LANES,)),
        ],
        compiler_params=pltpu.CompilerParams(vmem_limit_bytes=126 * 1024 * 1024),
    )(
        A_x[0].T,
        A_mem0[0],
        A_Wq.reshape(d_model * n_heads, d_head),
        A_Wk.reshape(d_model * n_heads, d_head),
        A_Wv.reshape(d_model * n_heads, d_head),
        jnp.transpose(A_Wo, (0, 2, 1)),
        B_w1,
        B_w3,
        B_w2.T,
    )
    return out_t.T[None]
```

```python
import functools

import jax
import jax.numpy as jnp
from jax import lax
import jax.experimental.pallas as pl
import jax.experimental.pallas.tpu as pltpu

SEG = 32
EPS = 1e-5
LOG2_E = 1.4426950408889634
MASK_FILL = -1000000000.0
LANES = 128
LAG = 4
SPLIT_ROWS = 48
QKV_PARTS = 4
K_BLOCK = 256
PLAIN_CHUNK = 384
SUM_ROWS = 32
STAGE_LAG = 5
BF16 = jnp.bfloat16
F32 = jnp.float32
NT_DIMS = (((1,), (1,)), ((), ()))


def _layernorm(x):
    inv_n = 1.0 / x.shape[-1]
    c = x - jnp.sum(x, axis=-1, keepdims=True) * inv_n
    v = jnp.sum(c * c, axis=-1, keepdims=True) * inv_n
    return c * lax.rsqrt(v + EPS)


def _strassen_lhs(a11, a12, a21, a22):
    return [a.astype(BF16) for a in (a11 + a22, a21 + a22, a11, a22, a11 + a12, a21 - a11, a12 - a22)]


def _strassen_rhs_sums(*blocks):
    words = [pltpu.bitcast(b, jnp.uint32) for b in blocks]
    halves = []
    for index in range(2):
        b11, b12, b21, b22 = (
            pltpu.unpack_elementwise(w, index=index, packed_dtype=BF16, unpacked_dtype=F32) for w in words)
        halves.append((b11 + b22, b12 - b22, b21 - b11, b11 + b12, b21 + b22))
    return [pltpu.pack_elementwise(list(pair), packed_dtype=BF16) for pair in zip(*halves)]


def _strassen_out(m1, m2, m3, m4, m5, m6, m7):
    return m1 + m4 - m5 + m7, m3 + m5, m2 + m4, m1 - m2 + m3 + m6


def _attention_mask(n_x, n_mem):
    rows = n_x + 2 * n_mem
    r = lax.broadcasted_iota(jnp.int32, (rows, rows), 0)
    c = lax.broadcasted_iota(jnp.int32, (rows, rows), 1)
    r_mem, c_mem = r >= n_x, c >= n_x
    r_stream = jnp.where(r_mem, (r - n_x) // n_mem, r // SEG)
    c_stream = jnp.where(c_mem, (c - n_x) // n_mem, c // SEG)
    same = r_stream == c_stream
    visible = same & (r_mem | c_mem | (c <= r))
    fill = jnp.where(same, MASK_FILL, -jnp.inf).astype(F32)
    return visible, fill


def _kernel(xt_hbm, mem0_ref, wq_hbm, wk_hbm, wv_hbm, wot_hbm, w1_hbm, w3_hbm, w2t_hbm,
            out_hbm,
            xt_v, stage, wqkv, wot, w1, w3, w2t, up_sums, down_sums,
            acts, ys, h_a, acc, out_v, sems, qkv_sems, out_sems,
            *, n_heads, d_head, n_mem):
    d_model, seq = xt_hbm.shape
    n_seg = seq // SEG
    n_chunks = seq // LANES
    segs_per_chunk = LANES // SEG
    f_half = w1.shape[2]
    f_quarter = f_half // 2
    k_lo, k_hi, k_rest = slice(0, K_BLOCK), slice(K_BLOCK, 2 * K_BLOCK), slice(2 * K_BLOCK, d_model)
    scale = d_head ** -0.5

    def seg_rows(base, s):
        return pl.ds(pl.multiple_of(base + s * SEG, SEG), SEG)

    def dot(a, b):
        return jnp.dot(a, b, preferred_element_type=F32)

    def dot_nt(a, b):
        return lax.dot_general(a, b, NT_DIMS, preferred_element_type=F32)

    def trailing_features(w_t, act):
        n, rows = w_t.shape[0], act.shape[0]
        out_t = dot_nt(w_t, act)
        if rows < LANES:
            out_t = jnp.concatenate([out_t, jnp.zeros((n, LANES - rows), F32)], axis=1)
        out_t = jnp.concatenate([out_t, jnp.zeros((LANES - n, LANES), F32)], axis=0)
        return out_t.T[:rows, :n]

    def pair_rows(start):
        return pl.ds(pl.multiple_of(start, 2 * SEG), 2 * SEG)

    def mixer_stages(h, n_x):
        rows = n_x + 2 * n_mem
        visible, fill = _attention_mask(n_x, n_mem)
        fill = fill / scale

        qkv, probs, mixed = {}, {}, {}

        def project(i):
            qkv[i] = dot(h, wqkv[:, 3 * i * d_head:3 * (i + 1) * d_head]).astype(BF16)

        def scores(i):
            s = dot_nt(qkv[i][:, 0:d_head], qkv[i][:, d_head:2 * d_head])
            s = jnp.where(visible, s, fill)
            e = jnp.exp2((s - jnp.max(s, axis=-1, keepdims=True)) * (scale * LOG2_E))
            total = jnp.sum(e, axis=-1, keepdims=True)
            inv = pl.reciprocal(total, approx=True)
            probs[i] = (e * (inv * (2.0 - total * inv))).astype(BF16)

        def mix(i):
            mixed[i] = dot(probs[i], qkv[i][:, 2 * d_head:]).astype(BF16)

        def output():
            o = jnp.concatenate([mixed[i] for i in range(n_heads)], axis=1)
            rest = trailing_features(wot[k_rest, :], o)
            return jnp.concatenate([dot_nt(o, wot[0:2 * K_BLOCK, :]), rest], axis=1)

        return project, scores, mix, output

    def swiglu(gate, up):
        half_gate = 0.5 * gate
        return (half_gate + half_gate * jnp.tanh(half_gate)) * up

    def ffn_stages(src0, src1, dst0, dst1):
        y = jnp.concatenate([ys[pair_rows(src0), :], ys[pair_rows(src1), :]], axis=0)
        h = _layernorm(y)
        top, bot = slice(0, 2 * SEG), slice(2 * SEG, 4 * SEG)
        lhs = _strassen_lhs(h[top, k_lo], h[top, k_hi], h[bot, k_lo], h[bot, k_hi])
        rest = h[:, k_rest].astype(BF16)

        tiles = {}

        def hidden_tile(half, cols):
            rhs = (pltpu.bitcast(up_sums[half, 0, :, cols], BF16), w1[half, k_lo, cols], pltpu.bitcast(up_sums[half, 1, :, cols], BF16),
                   pltpu.bitcast(up_sums[half, 2, :, cols], BF16), w3[half, k_hi, cols], pltpu.bitcast(up_sums[half, 3, :, cols], BF16),
                   pltpu.bitcast(up_sums[half, 4, :, cols], BF16))
            gate_top, up_top, gate_bot, up_bot = _strassen_out(*(dot(a, b) for a, b in zip(lhs, rhs)))
            gate_rest = dot(rest, w1[half, k_rest, cols])
            gate_top, gate_bot = gate_top + gate_rest[top], gate_bot + gate_rest[bot]
            up_rest = dot(rest, w3[half, k_rest, cols])
            g_top = swiglu(gate_top, up_top + up_rest[top])
            g_bot = swiglu(gate_bot, up_bot + up_rest[bot])
            return g_top, g_bot

        def hidden(half, f):
            cols = slice(f * LANES, (f + 1) * LANES)
            g11, g21 = hidden_tile(half, cols)
            g12, g22 = hidden_tile(half, slice(f_quarter + f * LANES, f_quarter + (f + 1) * LANES))
            tiles[f] = _strassen_lhs(g11, g12, g21, g22) + [g12.astype(BF16), g21.astype(BF16)]

        def output(half):
            f_lo, f_hi = slice(0, f_quarter), slice(f_quarter, f_half)
            g = [jnp.concatenate([tiles[f][k] for f in range(f_quarter // LANES)], axis=1) for k in range(9)]
            plain = jnp.concatenate([jnp.concatenate([g[2], g[7]], axis=1),
                                     jnp.concatenate([g[8], g[3]], axis=1)], axis=0)
            rhs = (pltpu.bitcast(down_sums[half, 0], BF16), w2t[half, k_lo, f_lo], pltpu.bitcast(down_sums[half, 1], BF16), pltpu.bitcast(down_sums[half, 2], BF16),
                   w2t[half, k_hi, f_hi], pltpu.bitcast(down_sums[half, 3], BF16), pltpu.bitcast(down_sums[half, 4], BF16))
            c11, c12, c21, c22 = _strassen_out(*(dot_nt(a, b) for a, b in zip(g, rhs)))
            part = jnp.concatenate(
                [jnp.concatenate([c11, c21], axis=0), jnp.concatenate([c12, c22], axis=0),
                 trailing_features(w2t[half, k_rest, :], plain)], axis=1)
            return part

        def finish(update):
            z = y + update
            acts[pair_rows(dst0), :] = z[top]
            acts[pair_rows(dst1), :] = z[bot]

        def half_stages(half):
            return ([functools.partial(hidden, half, f) for f in range(f_quarter // LANES)],
                    functools.partial(output, half))

        return half_stages, finish

    def first_ffn():
        y = ys[0:2 * SEG, :]
        h = _layernorm(y).astype(BF16)

        def quarter_pass(n, z):
            half, first = n // 2, (n % 2) * f_quarter
            g = []
            for f in range(f_quarter // PLAIN_CHUNK):
                cols = pl.ds(pl.multiple_of(first + f * PLAIN_CHUNK, LANES), PLAIN_CHUNK)
                g.append(swiglu(dot(h, w1[half, :, cols]), dot(h, w3[half, :, cols])).astype(BF16))
            g = jnp.concatenate(g, axis=1)
            cols = pl.ds(pl.multiple_of(first, LANES), f_quarter)
            trailing = trailing_features(w2t[half, k_rest, cols], g)
            return z + jnp.concatenate([dot_nt(g, w2t[half, 0:2 * K_BLOCK, cols]), trailing], axis=1)

        acts[seq:seq + 2 * SEG, :] = lax.fori_loop(0, 4, quarter_pass, y)

    def form_weight_sums(i, carry):
        per_half = K_BLOCK // SUM_ROWS
        half = i // per_half
        r0 = pl.multiple_of((i % per_half) * SUM_ROWS, SUM_ROWS)
        lo, hi = pl.ds(r0, SUM_ROWS), pl.ds(r0 + K_BLOCK, SUM_ROWS)
        packed = pl.ds(pl.multiple_of(r0 // 2, SUM_ROWS // 2), SUM_ROWS // 2)
        for c in range(f_half // LANES):
            cols = slice(c * LANES, (c + 1) * LANES)
            blocks = (w1[half, lo, cols], w3[half, lo, cols], w1[half, hi, cols], w3[half, hi, cols])
            for k, b in enumerate(_strassen_rhs_sums(*blocks)):
                up_sums[half, k, packed, cols] = b
        for c in range(f_quarter // LANES):
            cols = slice(c * LANES, (c + 1) * LANES)
            cols_hi = slice(f_quarter + c * LANES, f_quarter + (c + 1) * LANES)
            blocks = (w2t[half, lo, cols], w2t[half, hi, cols], w2t[half, lo, cols_hi], w2t[half, hi, cols_hi])
            for k, b in enumerate(_strassen_rhs_sums(*blocks)):
                down_sums[half, k, packed, cols] = b
        return carry

    def emit(matmul_work, scores, mix):
        for i in range(max(len(matmul_work), n_heads + 2 * STAGE_LAG)):
            if i < len(matmul_work):
                matmul_work[i]()
            if 0 <= i - STAGE_LAG < n_heads:
                scores(i - STAGE_LAG)
            if 0 <= i - 2 * STAGE_LAG < n_heads:
                mix(i - 2 * STAGE_LAG)

    def stage_segment(layer, s):
        h_a[0:SEG, :] = _layernorm(acts[seg_rows(layer * seq, s), :]).astype(BF16)

    def mixer_only(layer, s, mem):
        x = acts[seg_rows(layer * seq, s), :]
        tail = jnp.concatenate([mem, jnp.zeros_like(mem)], axis=0)
        h = jnp.concatenate([h_a[0:SEG, :], tail.astype(BF16)], axis=0)
        project, scores, mix, output = mixer_stages(h, SEG)
        emit([functools.partial(project, i) for i in range(n_heads)], scores, mix)

        @pl.when(s == 0)
        def _():
            for cp in cp_wo:
                cp.wait()

        stage_segment(layer, jnp.minimum(s + 1, layer * (n_seg - LAG) + LAG - 1))
        att = output()
        ys[seg_rows(layer * seq, s), :] = x + att[0:SEG]
        return att[SEG:SEG + n_mem]

    def stage_tokens(t):
        h_a[0:SEG, :] = _layernorm(acts[seg_rows(0, t), :]).astype(BF16)
        h_a[SEG:2 * SEG, :] = _layernorm(acts[seg_rows(seq, t - LAG), :]).astype(BF16)

    def transpose_out(c):
        rows = pl.ds(pl.multiple_of(2 * seq + c * LANES, LANES), LANES)
        out_v[c] = acts[rows, :].T.astype(out_v.dtype)

    def out_copy(c):
        return pltpu.make_async_copy(out_v.at[c], out_hbm.at[:, pl.ds(pl.multiple_of(c * LANES, LANES), LANES)],
                                     out_sems.at[c])

    cp_x0 = pltpu.make_async_copy(xt_hbm.at[:, 0:LANES], xt_v.at[:, 0:LANES], sems.at[8])
    cp_x = pltpu.make_async_copy(xt_hbm.at[:, LANES:], xt_v.at[:, LANES:], sems.at[0])
    part_rows = d_model // QKV_PARTS
    cp_qkv = [pltpu.make_async_copy(w.at[pl.ds(p * part_rows * n_heads, part_rows * n_heads)],
                                    stage.at[i * QKV_PARTS + p, pl.ds(0, part_rows * n_heads)],
                                    qkv_sems.at[i * QKV_PARTS + p])
              for i, w in enumerate((wq_hbm, wk_hbm, wv_hbm)) for p in range(QKV_PARTS)]
    cp_wo = [pltpu.make_async_copy(wot_hbm.at[i], wot.at[:, pl.ds(i * d_head, d_head)], sems.at[4])
             for i in range(n_heads)]
    cp_ff = [pltpu.make_async_copy(src.at[:, pl.ds(half * f_half, f_half)], dst.at[half], sems.at[5])
             for src, dst in ((w1_hbm, w1), (w3_hbm, w3), (w2t_hbm, w2t)) for half in range(2)]

    def transpose_in(c, carry):
        chunk = pl.ds(pl.multiple_of(c * LANES, LANES), LANES)
        acts[chunk, :] = xt_v[:, chunk].astype(F32).T
        return carry

    cp_x0.start()
    cp_qkv[0].start()
    cp_qkv[1].start()
    cp_x0.wait()
    acts[0:LANES, :] = xt_v[:, 0:LANES].astype(F32).T
    acts[2 * seq:2 * seq + LANES, :] = jnp.zeros((LANES, d_model), F32)
    acc[...] = jnp.zeros(acc.shape, F32)

    pairs = n_heads // 2

    def split_heads(n, b, carry):
        i, p = n // QKV_PARTS, n % QKV_PARTS
        first = pl.multiple_of(b * SPLIT_ROWS * pairs, SPLIT_ROWS * pairs)
        block = stage.at[n].bitcast(jnp.uint32).at[pl.ds(first, (SPLIT_ROWS + 1) * pairs)]
        features = pl.ds(pl.multiple_of(p * part_rows + b * SPLIT_ROWS, SPLIT_ROWS), SPLIT_ROWS)
        for j in range(pairs):
            w = block[pl.ds(j, SPLIT_ROWS, stride=pairs), :]
            even = pl.ds(pl.multiple_of((2 * j * 3 + i) * d_head, d_head), d_head)
            odd = pl.ds(pl.multiple_of(((2 * j + 1) * 3 + i) * d_head, d_head), d_head)
            wqkv[features, even] = pltpu.bitcast(w << 16, F32).astype(BF16)
            wqkv[features, odd] = pltpu.bitcast(w & jnp.uint32(0xFFFF0000), F32).astype(BF16)
        return carry

    def split_part(n, carry):
        landed = stage.at[n, pl.ds(0, part_rows * n_heads)]
        pltpu.make_async_copy(landed, landed, qkv_sems.at[n]).wait()
        for m in range(2, len(cp_qkv)):
            pl.when(n + 2 == m)(cp_qkv[m].start)

        @pl.when(n + 2 == len(cp_qkv))
        def _():
            for cp in cp_wo:
                cp.start()

        return lax.fori_loop(0, part_rows // SPLIT_ROWS, functools.partial(split_heads, n), carry)

    lax.fori_loop(0, len(cp_qkv), split_part, 0)
    for cp in cp_ff:
        cp.start()

    def step_pair(i, carry):
        t0 = 2 * i
        src0 = (t0 - 2) * SEG
        lagged = (t0 - LAG - 2) * SEG
        ready = lagged >= 0
        half_stages, finish = ffn_stages(
            src0, jnp.where(ready, seq + lagged, 0), seq + src0, jnp.where(ready, 2 * seq + lagged, 3 * seq))
        for half in range(2):
            t = t0 + half
            hidden, ffn_output = half_stages(half)
            project, scores, mix, mixer_output = mixer_stages(h_a[...], 2 * SEG)
            for work in hidden[:half]:
                work()
            emit([functools.partial(project, i) for i in range(n_heads)] + hidden[half:], scores, mix)
            if half == 0:
                transpose_out(jnp.maximum(t - out_delay, 0) // segs_per_chunk)
                first_half = ffn_output()
            else:
                finish(first_half + ffn_output())
            stage_tokens(jnp.minimum(t + 1, n_seg - 1))
            att = mixer_output()
            h_a[2 * SEG:, :] = att[2 * SEG:].astype(BF16)
            ys[seg_rows(0, t), :] = acts[seg_rows(0, t), :] + att[0:SEG]
            ys[seg_rows(seq, t - LAG), :] = acts[seg_rows(seq, t - LAG), :] + att[SEG:2 * SEG]
        return carry

    out_delay = LAG + 2 + segs_per_chunk
    done = (n_seg - 2 - out_delay) // segs_per_chunk + 1
    mem0 = mem0_ref[...].astype(F32)
    h_a[2 * SEG:, :] = jnp.concatenate([mem0, mem0], axis=0).astype(BF16)

    def schedule_round(layer, carry):
        first = layer * (n_seg - LAG)
        mem = h_a[2 * SEG:, :].astype(F32)[n_mem:]
        stage_segment(layer, first)
        mem = lax.fori_loop(first, first + LAG, functools.partial(mixer_only, layer), mem)

        @pl.when(layer == 0)
        def _():
            for cp in cp_ff:
                cp.wait()
            cp_x.start()
            lax.fori_loop(0, 2 * K_BLOCK // SUM_ROWS, form_weight_sums, 0)
            first_ffn()
            cp_x.wait()
            lax.fori_loop(1, n_chunks, transpose_in, 0, unroll=5)
            stage_tokens(LAG)
            h_a[2 * SEG:, :] = jnp.concatenate([mem, mem0], axis=0).astype(BF16)
            lax.fori_loop(LAG // 2, n_seg // 2, step_pair, 0)
            for c in range(done):
                out_copy(c).start()

        src0 = jnp.where(layer == 0, (n_seg - 2) * SEG, seq + (n_seg - 4) * SEG)
        src1 = jnp.where(layer == 0, seq + (n_seg - LAG - 2) * SEG, seq + (n_seg - 2) * SEG)

        def ffn_half(half, inner):
            half_stages, finish = ffn_stages(src0, src1, seq + src0, seq + src1)
            hidden, output = half_stages(half)
            for work in hidden:
                work()
            total = output() + jnp.where(half == 1, acc[...], 0.0)
            acc[...] = total
            finish(total)
            return inner

        lax.fori_loop(0, 2, ffn_half, 0)
        transpose_out(done + layer)
        out_copy(done + layer).start()
        return carry

    lax.fori_loop(0, 2, schedule_round, 0)
    for c in range(n_chunks):
        out_copy(c).wait()


@jax.jit
def pallas_interleave_layers__memory_aug_recurrent_mem_tr__glu_gated_swiglu__prompt_kernel(
    A_x, A_mem0, A_Wq, A_Wk, A_Wv, A_Wo, A_seg_len, B_x, B_w1, B_w3, B_w2,
):
    del A_seg_len, B_x
    batch, seq, d_model = A_x.shape
    _, n_heads, d_head = A_Wq.shape
    n_mem = A_mem0.shape[1]
    d_ff = B_w1.shape[1]
    assert batch == 1 and seq % 128 == 0 and d_ff % (4 * LANES) == 0
    rows = 2 * SEG + 2 * n_mem

    def kernel(*refs):
        _kernel(*refs, n_heads=n_heads, d_head=d_head, n_mem=n_mem)

    hbm = pl.BlockSpec(memory_space=pl.ANY)
    vmem = pl.BlockSpec(memory_space=pltpu.VMEM)
    out_t = pl.pallas_call(
        kernel,
        out_shape=jax.ShapeDtypeStruct((d_model, seq), A_x.dtype),
        in_specs=[hbm, vmem, hbm, hbm, hbm, hbm, hbm, hbm, hbm],
        out_specs=hbm,
        scratch_shapes=[
            pltpu.VMEM((d_model, seq), BF16),
            pltpu.VMEM((3 * QKV_PARTS, (d_model // QKV_PARTS + 1) * n_heads, d_head), BF16),
            pltpu.VMEM((d_model, 3 * n_heads * d_head), BF16),
            pltpu.VMEM((d_model, n_heads * d_head), BF16),
            pltpu.VMEM((2, d_model, d_ff // 2), BF16),
            pltpu.VMEM((2, d_model, d_ff // 2), BF16),
            pltpu.VMEM((2, d_model, d_ff // 2), BF16),
            pltpu.VMEM((2, 5, K_BLOCK // 2, d_ff // 2), jnp.uint32),
            pltpu.VMEM((2, 5, K_BLOCK // 2, d_ff // 4), jnp.uint32),
            pltpu.VMEM((3 * seq + 2 * SEG, d_model), F32),
            pltpu.VMEM((2 * seq, d_model), F32),
            pltpu.VMEM((rows, d_model), BF16),
            pltpu.VMEM((4 * SEG, d_model), F32),
            pltpu.VMEM((seq // LANES, d_model, LANES), A_x.dtype),
            pltpu.SemaphoreType.DMA((9,)),
            pltpu.SemaphoreType.DMA((3 * QKV_PARTS,)),
            pltpu.SemaphoreType.DMA((seq // LANES,)),
        ],
        compiler_params=pltpu.CompilerParams(vmem_limit_bytes=116 * 1024 * 1024),
    )(
        A_x[0].T,
        A_mem0[0],
        A_Wq.reshape(d_model * n_heads, d_head),
        A_Wk.reshape(d_model * n_heads, d_head),
        A_Wv.reshape(d_model * n_heads, d_head),
        jnp.transpose(A_Wo, (0, 2, 1)),
        B_w1,
        B_w3,
        B_w2.T,
    )
    return out_t.T[None]
```

```python
import functools

import jax
import jax.numpy as jnp
from jax import lax
import jax.experimental.pallas as pl
import jax.experimental.pallas.tpu as pltpu

SEG = 32
EPS = 1e-5
LOG2_E = 1.4426950408889634
MASK_FILL = -1000000000.0
LANES = 128
LAG = 4
SPLIT_ROWS = 48
QKV_PARTS = 4
K_BLOCK = 256
PLAIN_CHUNK = 384
SUM_ROWS = 32
STAGE_LAG = 5
BF16 = jnp.bfloat16
F32 = jnp.float32
NT_DIMS = (((1,), (1,)), ((), ()))


def _layernorm(x):
    inv_n = 1.0 / x.shape[-1]
    c = x - jnp.sum(x, axis=-1, keepdims=True) * inv_n
    v = jnp.sum(c * c, axis=-1, keepdims=True) * inv_n
    return c * lax.rsqrt(v + EPS)


def _strassen_lhs(a11, a12, a21, a22):
    return [a.astype(BF16) for a in (a11 + a22, a21 + a22, a11, a22, a11 + a12, a21 - a11, a12 - a22)]


def _strassen_rhs_sums(*blocks):
    b11, b12, b21, b22 = (b.astype(F32) for b in blocks)
    return [b.astype(BF16) for b in (b11 + b22, b12 - b22, b21 - b11, b11 + b12, b21 + b22)]


def _strassen_out(m1, m2, m3, m4, m5, m6, m7):
    return m1 + m4 - m5 + m7, m3 + m5, m2 + m4, m1 - m2 + m3 + m6


def _attention_mask(n_x, n_mem):
    rows = n_x + 2 * n_mem
    r = lax.broadcasted_iota(jnp.int32, (rows, rows), 0)
    c = lax.broadcasted_iota(jnp.int32, (rows, rows), 1)
    r_mem, c_mem = r >= n_x, c >= n_x
    r_stream = jnp.where(r_mem, (r - n_x) // n_mem, r // SEG)
    c_stream = jnp.where(c_mem, (c - n_x) // n_mem, c // SEG)
    same = r_stream == c_stream
    visible = same & (r_mem | c_mem | (c <= r))
    fill = jnp.where(same, MASK_FILL, -jnp.inf).astype(F32)
    return visible, fill


def _kernel(xt_hbm, mem0_ref, wq_hbm, wk_hbm, wv_hbm, wot_hbm, w1_hbm, w3_hbm, w2t_hbm,
            out_hbm,
            xt_v, stage, words, wqkv, wot, w1, w3, w2t, up_sums, down_sums,
            acts, ys, h_a, acc, out_v, sems, qkv_sems, out_sems,
            *, n_heads, d_head, n_mem):
    d_model, seq = xt_hbm.shape
    n_seg = seq // SEG
    n_chunks = seq // LANES
    segs_per_chunk = LANES // SEG
    f_half = w1.shape[2]
    f_quarter = f_half // 2
    k_lo, k_hi, k_rest = slice(0, K_BLOCK), slice(K_BLOCK, 2 * K_BLOCK), slice(2 * K_BLOCK, d_model)
    scale = d_head ** -0.5

    def seg_rows(base, s):
        return pl.ds(pl.multiple_of(base + s * SEG, SEG), SEG)

    def dot(a, b):
        return jnp.dot(a, b, preferred_element_type=F32)

    def dot_nt(a, b):
        return lax.dot_general(a, b, NT_DIMS, preferred_element_type=F32)

    def trailing_features(w_t, act):
        n, rows = w_t.shape[0], act.shape[0]
        out_t = dot_nt(w_t, act)
        if rows < LANES:
            out_t = jnp.concatenate([out_t, jnp.zeros((n, LANES - rows), F32)], axis=1)
        out_t = jnp.concatenate([out_t, jnp.zeros((LANES - n, LANES), F32)], axis=0)
        return out_t.T[:rows, :n]

    def pair_rows(start):
        return pl.ds(pl.multiple_of(start, 2 * SEG), 2 * SEG)

    def mixer_stages(h, n_x):
        rows = n_x + 2 * n_mem
        visible, fill = _attention_mask(n_x, n_mem)
        fill = fill / scale

        qkv, probs, mixed = {}, {}, {}

        def project(i):
            qkv[i] = dot(h, wqkv[:, 3 * i * d_head:3 * (i + 1) * d_head]).astype(BF16)

        def scores(i):
            s = dot_nt(qkv[i][:, 0:d_head], qkv[i][:, d_head:2 * d_head])
            s = jnp.where(visible, s, fill)
            e = jnp.exp2((s - jnp.max(s, axis=-1, keepdims=True)) * (scale * LOG2_E))
            total = jnp.sum(e, axis=-1, keepdims=True)
            inv = pl.reciprocal(total, approx=True)
            probs[i] = (e * (inv * (2.0 - total * inv))).astype(BF16)

        def mix(i):
            mixed[i] = dot(probs[i], qkv[i][:, 2 * d_head:]).astype(BF16)

        def output():
            o = jnp.concatenate([mixed[i] for i in range(n_heads)], axis=1)
            rest = trailing_features(wot[k_rest, :], o)
            return jnp.concatenate([dot_nt(o, wot[0:2 * K_BLOCK, :]), rest], axis=1)

        return project, scores, mix, output

    def swiglu(gate, up):
        half_gate = 0.5 * gate
        return (half_gate + half_gate * jnp.tanh(half_gate)) * up

    def ffn_stages(src0, src1, dst0, dst1):
        y = jnp.concatenate([ys[pair_rows(src0), :], ys[pair_rows(src1), :]], axis=0)
        h = _layernorm(y)
        top, bot = slice(0, 2 * SEG), slice(2 * SEG, 4 * SEG)
        lhs = _strassen_lhs(h[top, k_lo], h[top, k_hi], h[bot, k_lo], h[bot, k_hi])
        rest = h[:, k_rest].astype(BF16)

        tiles = {}

        def hidden_tile(half, cols):
            rhs = (up_sums[half, 0, :, cols], w1[half, k_lo, cols], up_sums[half, 1, :, cols],
                   up_sums[half, 2, :, cols], w3[half, k_hi, cols], up_sums[half, 3, :, cols],
                   up_sums[half, 4, :, cols])
            gate_top, up_top, gate_bot, up_bot = _strassen_out(*(dot(a, b) for a, b in zip(lhs, rhs)))
            gate_rest = dot(rest, w1[half, k_rest, cols])
            gate_top, gate_bot = gate_top + gate_rest[top], gate_bot + gate_rest[bot]
            up_rest = dot(rest, w3[half, k_rest, cols])
            g_top = swiglu(gate_top, up_top + up_rest[top])
            g_bot = swiglu(gate_bot, up_bot + up_rest[bot])
            return g_top, g_bot

        def hidden(half, f):
            cols = slice(f * LANES, (f + 1) * LANES)
            g11, g21 = hidden_tile(half, cols)
            g12, g22 = hidden_tile(half, slice(f_quarter + f * LANES, f_quarter + (f + 1) * LANES))
            tiles[f] = _strassen_lhs(g11, g12, g21, g22) + [g12.astype(BF16), g21.astype(BF16)]

        def output(half):
            f_lo, f_hi = slice(0, f_quarter), slice(f_quarter, f_half)
            g = [jnp.concatenate([tiles[f][k] for f in range(f_quarter // LANES)], axis=1) for k in range(9)]
            plain = jnp.concatenate([jnp.concatenate([g[2], g[7]], axis=1),
                                     jnp.concatenate([g[8], g[3]], axis=1)], axis=0)
            rhs = (down_sums[half, 0], w2t[half, k_lo, f_lo], down_sums[half, 1], down_sums[half, 2],
                   w2t[half, k_hi, f_hi], down_sums[half, 3], down_sums[half, 4])
            c11, c12, c21, c22 = _strassen_out(*(dot_nt(a, b) for a, b in zip(g, rhs)))
            part = jnp.concatenate(
                [jnp.concatenate([c11, c21], axis=0), jnp.concatenate([c12, c22], axis=0),
                 trailing_features(w2t[half, k_rest, :], plain)], axis=1)
            return part

        def finish(update):
            z = y + update
            acts[pair_rows(dst0), :] = z[top]
            acts[pair_rows(dst1), :] = z[bot]

        def half_stages(half):
            return ([functools.partial(hidden, half, f) for f in range(f_quarter // LANES)],
                    functools.partial(output, half))

        return half_stages, finish

    def first_ffn():
        y = ys[0:2 * SEG, :]
        h = _layernorm(y).astype(BF16)

        def quarter_pass(n, z):
            half, first = n // 2, (n % 2) * f_quarter
            g = []
            for f in range(f_quarter // PLAIN_CHUNK):
                cols = pl.ds(pl.multiple_of(first + f * PLAIN_CHUNK, LANES), PLAIN_CHUNK)
                g.append(swiglu(dot(h, w1[half, :, cols]), dot(h, w3[half, :, cols])).astype(BF16))
            g = jnp.concatenate(g, axis=1)
            cols = pl.ds(pl.multiple_of(first, LANES), f_quarter)
            trailing = trailing_features(w2t[half, k_rest, cols], g)
            return z + jnp.concatenate([dot_nt(g, w2t[half, 0:2 * K_BLOCK, cols]), trailing], axis=1)

        acts[seq:seq + 2 * SEG, :] = lax.fori_loop(0, 4, quarter_pass, y)

    def form_weight_sums(i, carry):
        per_half = K_BLOCK // SUM_ROWS
        half = i // per_half
        r0 = pl.multiple_of((i % per_half) * SUM_ROWS, SUM_ROWS)
        lo, hi = pl.ds(r0, SUM_ROWS), pl.ds(r0 + K_BLOCK, SUM_ROWS)
        for c in range(f_half // LANES):
            cols = slice(c * LANES, (c + 1) * LANES)
            blocks = (w1[half, lo, cols], w3[half, lo, cols], w1[half, hi, cols], w3[half, hi, cols])
            for k, b in enumerate(_strassen_rhs_sums(*blocks)):
                up_sums[half, k, lo, cols] = b
        for c in range(f_quarter // LANES):
            cols = slice(c * LANES, (c + 1) * LANES)
            cols_hi = slice(f_quarter + c * LANES, f_quarter + (c + 1) * LANES)
            blocks = (w2t[half, lo, cols], w2t[half, hi, cols], w2t[half, lo, cols_hi], w2t[half, hi, cols_hi])
            for k, b in enumerate(_strassen_rhs_sums(*blocks)):
                down_sums[half, k, lo, cols] = b
        return carry

    def emit(matmul_work, scores, mix):
        for i in range(max(len(matmul_work), n_heads + 2 * STAGE_LAG)):
            if i < len(matmul_work):
                matmul_work[i]()
            if 0 <= i - STAGE_LAG < n_heads:
                scores(i - STAGE_LAG)
            if 0 <= i - 2 * STAGE_LAG < n_heads:
                mix(i - 2 * STAGE_LAG)

    def stage_segment(layer, s):
        h_a[0:SEG, :] = _layernorm(acts[seg_rows(layer * seq, s), :]).astype(BF16)

    def mixer_only(layer, s, mem):
        x = acts[seg_rows(layer * seq, s), :]
        tail = jnp.concatenate([mem, jnp.zeros_like(mem)], axis=0)
        h = jnp.concatenate([h_a[0:SEG, :], tail.astype(BF16)], axis=0)
        project, scores, mix, output = mixer_stages(h, SEG)
        emit([functools.partial(project, i) for i in range(n_heads)], scores, mix)

        @pl.when(s == 0)
        def _():
            for cp in cp_wo:
                cp.wait()

        stage_segment(layer, jnp.minimum(s + 1, layer * (n_seg - LAG) + LAG - 1))
        att = output()
        ys[seg_rows(layer * seq, s), :] = x + att[0:SEG]
        return att[SEG:SEG + n_mem]

    def stage_tokens(t):
        h_a[0:SEG, :] = _layernorm(acts[seg_rows(0, t), :]).astype(BF16)
        h_a[SEG:2 * SEG, :] = _layernorm(acts[seg_rows(seq, t - LAG), :]).astype(BF16)

    def transpose_out(c):
        rows = pl.ds(pl.multiple_of(2 * seq + c * LANES, LANES), LANES)
        out_v[c] = acts[rows, :].T.astype(out_v.dtype)

    def out_copy(c):
        return pltpu.make_async_copy(out_v.at[c], out_hbm.at[:, pl.ds(pl.multiple_of(c * LANES, LANES), LANES)],
                                     out_sems.at[c])

    cp_x0 = pltpu.make_async_copy(xt_hbm.at[:, 0:LANES], xt_v.at[:, 0:LANES], sems.at[8])
    cp_x = pltpu.make_async_copy(xt_hbm.at[:, LANES:], xt_v.at[:, LANES:], sems.at[0])
    part_rows = d_model // QKV_PARTS
    cp_qkv = [pltpu.make_async_copy(w.at[pl.ds(p * part_rows * n_heads, part_rows * n_heads)],
                                    stage.at[i * QKV_PARTS + p], qkv_sems.at[i * QKV_PARTS + p])
              for i, w in enumerate((wq_hbm, wk_hbm, wv_hbm)) for p in range(QKV_PARTS)]
    cp_wo = [pltpu.make_async_copy(wot_hbm.at[i], wot.at[:, pl.ds(i * d_head, d_head)], sems.at[4])
             for i in range(n_heads)]
    cp_ff = [pltpu.make_async_copy(src.at[:, pl.ds(half * f_half, f_half)], dst.at[half], sems.at[5])
             for src, dst in ((w1_hbm, w1), (w3_hbm, w3), (w2t_hbm, w2t)) for half in range(2)]

    def transpose_in(c, carry):
        chunk = pl.ds(pl.multiple_of(c * LANES, LANES), LANES)
        acts[chunk, :] = xt_v[:, chunk].astype(F32).T
        return carry

    cp_x0.start()
    cp_qkv[0].start()
    cp_qkv[1].start()
    cp_x0.wait()
    acts[0:LANES, :] = xt_v[:, 0:LANES].astype(F32).T
    acts[2 * seq:2 * seq + LANES, :] = jnp.zeros((LANES, d_model), F32)
    acc[...] = jnp.zeros(acc.shape, F32)

    pairs = n_heads // 2

    def split_heads(n, b, carry):
        i, p = n // QKV_PARTS, n % QKV_PARTS
        first = pl.multiple_of(b * SPLIT_ROWS * n_heads, SPLIT_ROWS * n_heads)
        words[0:SPLIT_ROWS * pairs, :] = pltpu.bitcast(
            stage[n, pl.ds(first, SPLIT_ROWS * n_heads), :], jnp.uint32)
        features = pl.ds(pl.multiple_of(p * part_rows + b * SPLIT_ROWS, SPLIT_ROWS), SPLIT_ROWS)
        for j in range(pairs):
            w = words[pl.ds(j, SPLIT_ROWS, stride=pairs), :]
            even = pl.ds(pl.multiple_of((2 * j * 3 + i) * d_head, d_head), d_head)
            odd = pl.ds(pl.multiple_of(((2 * j + 1) * 3 + i) * d_head, d_head), d_head)
            wqkv[features, even] = pltpu.bitcast(w << 16, F32).astype(BF16)
            wqkv[features, odd] = pltpu.bitcast(w & jnp.uint32(0xFFFF0000), F32).astype(BF16)
        return carry

    def split_part(n, carry):
        pltpu.make_async_copy(stage.at[n], stage.at[n], qkv_sems.at[n]).wait()
        for m in range(2, len(cp_qkv)):
            pl.when(n + 2 == m)(cp_qkv[m].start)

        @pl.when(n + 2 == len(cp_qkv))
        def _():
            for cp in cp_wo:
                cp.start()

        return lax.fori_loop(0, part_rows // SPLIT_ROWS, functools.partial(split_heads, n), carry)

    lax.fori_loop(0, len(cp_qkv), split_part, 0)
    for cp in cp_ff:
        cp.start()

    def step_pair(i, carry):
        t0 = 2 * i
        src0 = (t0 - 2) * SEG
        lagged = (t0 - LAG - 2) * SEG
        ready = lagged >= 0
        half_stages, finish = ffn_stages(
            src0, jnp.where(ready, seq + lagged, 0), seq + src0, jnp.where(ready, 2 * seq + lagged, 3 * seq))
        for half in range(2):
            t = t0 + half
            hidden, ffn_output = half_stages(half)
            project, scores, mix, mixer_output = mixer_stages(h_a[...], 2 * SEG)
            for work in hidden[:half]:
                work()
            emit([functools.partial(project, i) for i in range(n_heads)] + hidden[half:], scores, mix)
            if half == 0:
                transpose_out(jnp.maximum(t - out_delay, 0) // segs_per_chunk)
                first_half = ffn_output()
            else:
                finish(first_half + ffn_output())
            stage_tokens(jnp.minimum(t + 1, n_seg - 1))
            att = mixer_output()
            h_a[2 * SEG:, :] = att[2 * SEG:].astype(BF16)
            ys[seg_rows(0, t), :] = acts[seg_rows(0, t), :] + att[0:SEG]
            ys[seg_rows(seq, t - LAG), :] = acts[seg_rows(seq, t - LAG), :] + att[SEG:2 * SEG]
        return carry

    out_delay = LAG + 2 + segs_per_chunk
    done = (n_seg - 2 - out_delay) // segs_per_chunk + 1
    mem0 = mem0_ref[...].astype(F32)
    h_a[2 * SEG:, :] = jnp.concatenate([mem0, mem0], axis=0).astype(BF16)

    def schedule_round(layer, carry):
        first = layer * (n_seg - LAG)
        mem = h_a[2 * SEG:, :].astype(F32)[n_mem:]
        stage_segment(layer, first)
        mem = lax.fori_loop(first, first + LAG, functools.partial(mixer_only, layer), mem)

        @pl.when(layer == 0)
        def _():
            for cp in cp_ff:
                cp.wait()
            cp_x.start()
            lax.fori_loop(0, 2 * K_BLOCK // SUM_ROWS, form_weight_sums, 0)
            first_ffn()
            cp_x.wait()
            lax.fori_loop(1, n_chunks, transpose_in, 0, unroll=5)
            stage_tokens(LAG)
            h_a[2 * SEG:, :] = jnp.concatenate([mem, mem0], axis=0).astype(BF16)
            lax.fori_loop(LAG // 2, n_seg // 2, step_pair, 0)
            for c in range(done):
                out_copy(c).start()

        src0 = jnp.where(layer == 0, (n_seg - 2) * SEG, seq + (n_seg - 4) * SEG)
        src1 = jnp.where(layer == 0, seq + (n_seg - LAG - 2) * SEG, seq + (n_seg - 2) * SEG)

        def ffn_half(half, inner):
            half_stages, finish = ffn_stages(src0, src1, seq + src0, seq + src1)
            hidden, output = half_stages(half)
            for work in hidden:
                work()
            total = output() + jnp.where(half == 1, acc[...], 0.0)
            acc[...] = total
            finish(total)
            return inner

        lax.fori_loop(0, 2, ffn_half, 0)
        transpose_out(done + layer)
        out_copy(done + layer).start()
        return carry

    lax.fori_loop(0, 2, schedule_round, 0)
    for c in range(n_chunks):
        out_copy(c).wait()


@jax.jit
def pallas_interleave_layers__memory_aug_recurrent_mem_tr__glu_gated_swiglu__prompt_kernel(
    A_x, A_mem0, A_Wq, A_Wk, A_Wv, A_Wo, A_seg_len, B_x, B_w1, B_w3, B_w2,
):
    del A_seg_len, B_x
    batch, seq, d_model = A_x.shape
    _, n_heads, d_head = A_Wq.shape
    n_mem = A_mem0.shape[1]
    d_ff = B_w1.shape[1]
    assert batch == 1 and seq % 128 == 0 and d_ff % (4 * LANES) == 0
    rows = 2 * SEG + 2 * n_mem

    def kernel(*refs):
        _kernel(*refs, n_heads=n_heads, d_head=d_head, n_mem=n_mem)

    hbm = pl.BlockSpec(memory_space=pl.ANY)
    vmem = pl.BlockSpec(memory_space=pltpu.VMEM)
    out_t = pl.pallas_call(
        kernel,
        out_shape=jax.ShapeDtypeStruct((d_model, seq), A_x.dtype),
        in_specs=[hbm, vmem, hbm, hbm, hbm, hbm, hbm, hbm, hbm],
        out_specs=hbm,
        scratch_shapes=[
            pltpu.VMEM((d_model, seq), BF16),
            pltpu.VMEM((3 * QKV_PARTS, d_model // QKV_PARTS * n_heads, d_head), BF16),
            pltpu.VMEM(((SPLIT_ROWS + 1) * n_heads // 2, d_head), jnp.uint32),
            pltpu.VMEM((d_model, 3 * n_heads * d_head), BF16),
            pltpu.VMEM((d_model, n_heads * d_head), BF16),
            pltpu.VMEM((2, d_model, d_ff // 2), BF16),
            pltpu.VMEM((2, d_model, d_ff // 2), BF16),
            pltpu.VMEM((2, d_model, d_ff // 2), BF16),
            pltpu.VMEM((2, 5, K_BLOCK, d_ff // 2), BF16),
            pltpu.VMEM((2, 5, K_BLOCK, d_ff // 4), BF16),
            pltpu.VMEM((3 * seq + 2 * SEG, d_model), F32),
            pltpu.VMEM((2 * seq, d_model), F32),
            pltpu.VMEM((rows, d_model), BF16),
            pltpu.VMEM((4 * SEG, d_model), F32),
            pltpu.VMEM((seq // LANES, d_model, LANES), A_x.dtype),
            pltpu.SemaphoreType.DMA((9,)),
            pltpu.SemaphoreType.DMA((3 * QKV_PARTS,)),
            pltpu.SemaphoreType.DMA((seq // LANES,)),
        ],
        compiler_params=pltpu.CompilerParams(vmem_limit_bytes=116 * 1024 * 1024),
    )(
        A_x[0].T,
        A_mem0[0],
        A_Wq.reshape(d_model * n_heads, d_head),
        A_Wk.reshape(d_model * n_heads, d_head),
        A_Wv.reshape(d_model * n_heads, d_head),
        jnp.transpose(A_Wo, (0, 2, 1)),
        B_w1,
        B_w3,
        B_w2.T,
    )
    return out_t.T[None]
```
